```python
import jax
import jax.numpy as jnp

def _softmax(x, axis=-1):
    return jax.nn.softmax(x, axis=axis)
def _gelu(x):
    return jax.nn.gelu(x, approximate=True)
def _silu(x):
    return jax.nn.silu(x)
def _sigmoid(x):
    return jax.nn.sigmoid(x)
def _layernorm(x, axis=-1, eps=1e-5):
    m = jnp.mean(x, axis=axis, keepdims=True)
    v = jnp.var(x, axis=axis, keepdims=True)
    return (x - m) / jnp.sqrt(v + eps)
def _scatter_add(tgt, idx, src, axis=0):
    return tgt.at[idx].add(src)
def _segment_sum(src, seg, n):
    return jax.ops.segment_sum(src, seg, n)
class _Rng:
    def __init__(self, key):
        self._k = key
    def _next(self):
        self._k, sub = jax.random.split(self._k)
        return sub
    def normal(self, shape):
        return jax.random.normal(self._next(), shape, dtype=jnp.bfloat16)
    def randint(self, lo, hi, shape):
        return jax.random.randint(self._next(), shape, lo, hi, dtype=jnp.int32)
    def uniform(self, shape, lo=0.0, hi=1.0):
        return jax.random.uniform(self._next(), shape, jnp.bfloat16, lo, hi)
    def permutation(self, n):
        return jax.random.permutation(self._next(), n)


kernel_name = 'gated_mix__ssm_conv_h3__sliding_local_dilated__prompt'

def setup_inputs():
    _rng = _Rng(jax.random.key(int.from_bytes(__import__("os").urandom(4), "little")))
    _w = (lambda a: (lambda t: t.astype(jnp.bfloat16) if jnp.issubdtype(t.dtype, jnp.floating) else t)(jnp.asarray(a)))
    def _A_setup():
        B, S, D = 1, 2048, 640
        ks = 4
        return {
            "q": _w((lambda *s: _rng.normal(s) * 0.05)(B, S, D)),
            "k": _w((lambda *s: _rng.normal(s) * 0.05)(B, S, D)),
            "v": _w((lambda *s: _rng.normal(s) * 0.05)(B, S, D)),
            "shift_k": _w((lambda *s: _rng.normal(s) * 0.05)(D, ks) * 0.5),
            "ssm_k": _w((lambda *s: _rng.normal(s) * 0.05)(D, S) * (1.0 / S ** 0.5)),
            "ssm_D": _w((lambda *s: _rng.normal(s) * 0.05)(D)),
        }
    _A_in = _A_setup()

    def _B_setup():
        B, S, D = 1, 2048, 640
        return {
            "x": _w((lambda *s: _rng.normal(s) * 0.05)(B, S, D)),
            "wqkv": _w((lambda *s: _rng.normal(s) * 0.05)(D, 3 * D)),
            "wo": _w((lambda *s: _rng.normal(s) * 0.05)(D, D)),
        }
    _B_in = _B_setup()

    return {
        "A_q": _A_in["q"],
        "A_k": _A_in["k"],
        "A_v": _A_in["v"],
        "A_shift_k": _A_in["shift_k"],
        "A_ssm_k": _A_in["ssm_k"],
        "A_ssm_D": _A_in["ssm_D"],
        "B_x": _B_in["x"],
        "B_wqkv": _B_in["wqkv"],
        "B_wo": _B_in["wo"],
        "gate_w": _w((lambda *s: _rng.normal(s) * 0.05)(640)),
    }

def reference(A_q, A_k, A_v, A_shift_k, A_ssm_k, A_ssm_D, B_x, B_wqkv, B_wo, gate_w):
    def _A_ref(q, k, v, shift_k, ssm_k, ssm_D):
        B, S, D = q.shape
        ks = shift_k.shape[-1]
        k_pad = jnp.pad(k, ((0, 0), (ks - 1, 0), (0, 0)))
        k_shift = jnp.zeros_like(k)
        for t in range(ks):
            k_shift = k_shift + k_pad[:, t:t + S, :] * shift_k[:, ks - 1 - t][None, None, :]
        kv = k_shift * v
        L = 2 * S
        kv_pad = jnp.pad(kv, ((0, 0), (0, S), (0, 0)))
        kf_pad = jnp.pad(ssm_k, ((0, 0), (0, S)))
        kv_f = (lambda x, axes=(-2,-1): jnp.fft.rfft2(x.astype(jnp.float32), axes=axes))(kv_pad[:, None, :, :], axes=(1, 2))
        kf_f = (lambda x, axes=(-2,-1): jnp.fft.rfft2(x.astype(jnp.float32), axes=axes))(kf_pad[:, None, :], axes=(1, 2))
        kf_f = (lambda x, *d: x.transpose(*d))(kf_f, 1, 2, 0)
        y_f = kv_f * kf_f[None, :, :, :]
        y = (lambda x, s, axes=(-2,-1): jnp.fft.irfft2(x, s=s, axes=axes).astype(jnp.bfloat16))(y_f, (1, L), axes=(1, 2))[:, 0, :S, :]
        y = y + kv * ssm_D[None, None, :]
        return q * y

    def _B_ref(x, wqkv, wo):
        B, S, D = x.shape
        H = 32; Dh = D // H
        W, dil = 8, 2
        qkv = (lambda x, *d: x.transpose(*d))((x @ wqkv).reshape(B, S, 3, H, Dh), 2, 0, 3, 1, 4)
        q, k, v = qkv[0], qkv[1], qkv[2]
        scale = Dh ** -0.5
        pos = jnp.arange(S)
        off = jnp.arange(W) * dil
        idx = pos[:, None] - off[None, :]
        mask = idx >= 0
        idx_c = jnp.where(mask, idx, 0).reshape(-1)
        kg = k[:, :, idx_c, :].reshape(B, H, S, W, Dh)
        vg = v[:, :, idx_c, :].reshape(B, H, S, W, Dh)
        logits = jnp.einsum("bhsd,bhswd->bhsw", q, kg) * scale
        logits = jnp.where(mask[None, None, :, :], logits, -1e9)
        attn = _softmax(logits, axis=-1)
        o = jnp.einsum("bhsw,bhswd->bhsd", attn, vg)
        return (lambda x, *d: x.transpose(*d))(o, 0, 2, 1, 3).reshape(B, S, D) @ wo

    x = A_q
    g = _sigmoid((x * gate_w).sum(-1, keepdims=True))
    a = _A_ref(x, A_k, A_v, A_shift_k, A_ssm_k, A_ssm_D)
    b = _B_ref(x, B_wqkv, B_wo)
    return g * a + (1 - g) * b
```

```python
import functools
import numpy as np
import jax
import jax.numpy as jnp
from jax.experimental import pallas as pl
from jax.experimental.pallas import tpu as pltpu

S, D = 2048, 640
ND = 5
L = 128
NA = S // L
T = 256
NT = S // T
H, DH = 32, 20
HALO = 16
GR = 16
NG = T // GR
LOG2E = 1.4426950408889634
QSCALE = float(DH ** -0.5) * LOG2E
MASKED = -1e9 * LOG2E
F32, BF16, U32 = jnp.float32, jnp.bfloat16, jnp.uint32


def _dft_constants():
    forder = np.concatenate([np.arange(0, 128, 2), np.arange(1, 128, 2)])
    th = np.pi * (2 * forder + 1) / 256.0
    b = np.arange(128)
    fwd = np.concatenate([np.cos(np.outer(th, b)), -np.sin(np.outer(th, b))], 0)
    gre = np.cos(np.outer(b, th)) / 128
    gim = -np.sin(np.outer(b, th)) / 128
    inv = np.stack([gre, gim], -1).reshape(128, 256)
    return fwd.astype(np.float32), inv.astype(np.float32), np.eye(128, dtype=np.float32)


def _bf(x):
    return pltpu.bitcast(x, BF16)


def _u32(x):
    return pltpu.bitcast(x, U32)


def _dot(a, b):
    return jnp.dot(a, b, preferred_element_type=F32)


def _dot_nt(a, b):
    return jax.lax.dot_general(a, b, (((1,), (1,)), ((), ())), preferred_element_type=F32)


def _kernel(q_hbm, k_hbm, v_hbm, shk_ref, sk_hbm, dvec_ref, wqkv_hbm, wo_hbm, gw_ref,
            fwd_ref, inv_ref, eye_ref,
            out_hbm,
            kbuf, vbuf, skbuf, qbuf, wqkv_v, wo_v, par, fwdp, invp,
            kf, kvp, ubuf, kpbuf, ybuf, y2, wt, wtp, wof, wop,
            qp, kp, vp, lbuf, op, bres, obuf,
            sem_a, sem_q, sem_w, sem_o):

    def slab_copies(j):
        return (
            pltpu.make_async_copy(k_hbm.at[0, :, pl.ds(j * 128, 128)], kbuf.at[j], sem_a.at[3 * j]),
            pltpu.make_async_copy(v_hbm.at[0, :, pl.ds(j * 128, 128)], vbuf.at[j], sem_a.at[3 * j + 1]),
            pltpu.make_async_copy(sk_hbm.at[pl.ds(j * 128, 128), :], skbuf.at[j], sem_a.at[3 * j + 2]),
        )

    def q_copy(b):
        return pltpu.make_async_copy(q_hbm.at[0, pl.ds(b * T, T), :], qbuf.at[pl.ds(b * T, T), :], sem_q.at[b])

    def out_copy(b, slot):
        return pltpu.make_async_copy(obuf.at[slot], out_hbm.at[0, pl.ds(b * T, T), :], sem_o.at[slot])

    wqkv_copy = pltpu.make_async_copy(wqkv_hbm, wqkv_v, sem_w.at[0])
    wo_copy = pltpu.make_async_copy(wo_hbm, wo_v, sem_w.at[1])

    for j in range(ND):
        for c in slab_copies(j):
            c.start()
        if j == 1:
            wqkv_copy.start()
        if j == 2:
            wo_copy.start()
    for b in range(NT):
        q_copy(b).start()

    taps = shk_ref[...].astype(F32).T
    dv = dvec_ref[...].astype(F32)
    gw = gw_ref[...].astype(F32)
    for j in range(ND):
        par[j, 0:4, :] = taps[:, j * 128:(j + 1) * 128]
        par[j, 4:5, :] = dv[:, j * 128:(j + 1) * 128]
        par[j, 5:6, :] = gw[:, j * 128:(j + 1) * 128]
        par[j, 6:8, :] = jnp.zeros((2, 128), F32)
    fwdp[...] = _u32(fwd_ref[...])
    invp[...] = _u32(inv_ref[...])
    kf[0:8, :] = jnp.zeros((8, 128), F32)
    ybuf[...] = jnp.zeros(ybuf.shape, U32)
    for j in range(ND):
        kp[j, 0:HALO, :] = jnp.zeros((HALO, 128), F32)
        vp[j, 0:HALO, :] = jnp.zeros((HALO, 128), F32)

    def kvprep(j):
        for c in range(NA):
            kf[8 + c * L:8 + (c + 1) * L, :] = kbuf[j, c * L:(c + 1) * L, :].astype(F32)
        t = [par[j, i:i + 1, :] for i in range(4)]
        for c in range(S // 32):
            r = c * 32
            ks = kf[8 + r:8 + r + 32, :] * t[0]
            for i in range(1, 4):
                ks = ks + kf[8 + r - i:8 + r - i + 32, :] * t[i]
            kv = ks * vbuf[j, r:r + 32, :].astype(F32)
            kvp[j, r // 2:r // 2 + 16, :] = _u32(kv.astype(BF16))

    def dft_u(j, slot):
        f = _bf(fwdp[...])
        for c in range(NA):
            ubuf[slot, c] = _dot(f, _bf(kvp[j, c * 64:(c + 1) * 64, :]))

    def dft_k(j, slot):
        f = _bf(fwdp[...])
        for m in range(NA):
            kpbuf[slot, m] = _dot_nt(f, skbuf[j, :, m * L:(m + 1) * L])

    def aconv(slot):
        for p in range(16):
            r, i = p * 8, 128 + p * 8
            pr = [kpbuf[slot, m, r:r + 8, :] for m in range(NA)]
            pi = [kpbuf[slot, m, i:i + 8, :] for m in range(NA)]
            if p < 8:
                kr = [pr[0]] + [pr[m] - pi[m - 1] for m in range(1, NA)]
                ki = [pi[0]] + [pi[m] + pr[m - 1] for m in range(1, NA)]
            else:
                kr = [pr[0]] + [pr[m] + pi[m - 1] for m in range(1, NA)]
                ki = [pi[0]] + [pi[m] - pr[m - 1] for m in range(1, NA)]
            for a in range(NA):
                accr = acci = None
                for c in range(a + 1):
                    m = a - c
                    ur = ubuf[slot, c, r:r + 8, :]
                    ui = ubuf[slot, c, i:i + 8, :]
                    tr = kr[m] * ur - ki[m] * ui
                    ti = kr[m] * ui + ki[m] * ur
                    accr = tr if accr is None else accr + tr
                    acci = ti if acci is None else acci + ti
                ybuf[slot, a, r:r + 8, :] = pltpu.pack_elementwise([accr, acci], packed_dtype=BF16)

    def idft(j, slot):
        g0 = _bf(invp[:, 0:128])
        g1 = _bf(invp[:, 128:256])
        for a in range(NA):
            y2[0, j, a * L:(a + 1) * L, :] = _dot(g0, _bf(ybuf[slot, a, 0:64, :]))
            y2[1, j, a * L:(a + 1) * L, :] = _dot(g1, _bf(ybuf[slot, a, 64:128, :]))

    def wait_slab(j):
        for c in slab_copies(j):
            c.wait()

    def w_transpose():
        eye = eye_ref[...]
        for n in range(15):
            r = _dot_nt(eye, wqkv_v[:, n * 128:(n + 1) * 128])
            for kt in range(ND):
                wt[kt, n * 128:(n + 1) * 128, :] = r[:, kt * 128:(kt + 1) * 128]

    def w_permute():
        for p in range(3):
            for dh in range(DH):
                for kt in range(ND):
                    rows = wt[kt, pl.ds(p * D + dh, H, stride=DH), :]
                    r0 = (p * D + dh * H) // 2
                    wtp[r0:r0 + H // 2, kt * 128:(kt + 1) * 128] = _u32(rows.astype(BF16))
        for j in range(ND):
            wof[j] = wo_v[:, j * 128:(j + 1) * 128].astype(F32)
        for dh in range(DH):
            for j in range(ND):
                rows = wof[j, pl.ds(dh, H, stride=DH), :]
                r0 = dh * H // 2
                wop[r0:r0 + H // 2, j * 128:(j + 1) * 128] = _u32(rows.astype(BF16))

    def qkv(b):
        r0 = pl.multiple_of(b * T, T)
        r = _dot_nt(qbuf[pl.ds(r0, T), :], _bf(wtp[...]))
        slot = b % 2
        for j in range(ND):
            qp[slot, j] = r[:, j * 128:(j + 1) * 128]
            kp[j, pl.ds(HALO + r0, T), :] = r[:, D + j * 128:D + (j + 1) * 128]
            vp[j, pl.ds(HALO + r0, T), :] = r[:, 2 * D + j * 128:2 * D + (j + 1) * 128]

    def attention(b):
        r0 = pl.multiple_of(b * T, T)
        slot = b % 2
        P, Sx = {}, {}
        for g in range(NG + 3):
            if g < NG:
                row = r0 + g * GR
                q = [qp[slot, j, g * GR:(g + 1) * GR, :] * QSCALE for j in range(ND)]
                P[g] = []
                for w in range(8):
                    p = None
                    for j in range(ND):
                        t = q[j] * kp[j, pl.ds(row + HALO - 2 * w, GR), :]
                        p = t if p is None else p + t
                    P[g].append((p, pltpu.roll(p, 64, 1)))
            if 0 <= g - 1 < NG:
                Sx[g - 1] = []
                for (p, r) in P.pop(g - 1):
                    s = p + r
                    Sx[g - 1].append((s, pltpu.roll(s, 32, 1)))
            if 0 <= g - 2 < NG:
                gg = g - 2
                for w, (s, r) in enumerate(Sx.pop(gg)):
                    l = s + r
                    if gg == 0 and w > 0:
                        t = r0 + jax.lax.broadcasted_iota(jnp.int32, (GR, 128), 0)
                        l = jnp.where(t >= 2 * w, l, MASKED)
                    lbuf[w, gg * GR:(gg + 1) * GR, :] = l
            if 0 <= g - 3 < NG:
                gg = g - 3
                row = r0 + gg * GR
                lg = [lbuf[w, gg * GR:(gg + 1) * GR, :] for w in range(8)]
                m = lg[0]
                for w in range(1, 8):
                    m = jnp.maximum(m, lg[w])
                es = [jnp.exp2(l - m) for l in lg]
                s = es[0]
                for w in range(1, 8):
                    s = s + es[w]
                inv = 1.0 / s
                for j in range(ND):
                    acc = None
                    for w in range(8):
                        t = es[w] * vp[j, pl.ds(row + HALO - 2 * w, GR), :]
                        acc = t if acc is None else acc + t
                    op[gg * GR // 2:(gg + 1) * GR // 2, j * 128:(j + 1) * 128] = _u32((acc * inv).astype(BF16))

    def outproj(b):
        bres[b % 2] = _dot(_bf(op[...]), _bf(wop[...]))

    def epilogue(b):
        r0 = pl.multiple_of(b * T, T)
        slot = b % 2
        for g in range(NG):
            row = r0 + g * GR
            rowh = pl.multiple_of(b * (T // 2), T // 2) + g * (GR // 2)
            q = [qbuf[pl.ds(row, GR), j * 128:(j + 1) * 128].astype(F32) for j in range(ND)]
            s = None
            for j in range(ND):
                t = q[j] * par[j, 5:6, :]
                s = t if s is None else s + t
            gate = jax.nn.sigmoid(jnp.sum(s, axis=-1, keepdims=True))
            for j in range(ND):
                kv = _bf(kvp[j, pl.ds(rowh, GR // 2), :]).astype(F32)
                z = y2[0, j, pl.ds(row, GR), :] + y2[1, j, pl.ds(row, GR), :] + kv * par[j, 4:5, :]
                bb = bres[slot, g * GR:(g + 1) * GR, j * 128:(j + 1) * 128]
                o = bb + gate * (q[j] * z - bb)
                obuf[slot, g * GR:(g + 1) * GR, j * 128:(j + 1) * 128] = o.astype(BF16)

    wait_slab(0)
    kvprep(0)
    dft_k(0, 0)
    dft_u(0, 0)

    def body_a(j, carry):
        slot = j % 2
        wait_slab(j + 1)
        kvprep(j + 1)
        aconv(slot)
        dft_k(j + 1, 1 - slot)
        idft(jnp.maximum(j - 1, 0), 1 - slot)
        dft_u(j + 1, 1 - slot)
        return carry

    jax.lax.fori_loop(0, ND - 1, body_a, 0)

    wqkv_copy.wait()
    wo_copy.wait()
    aconv((ND - 1) % 2)
    idft(ND - 2, (ND - 2) % 2)
    w_transpose()
    w_permute()

    q_copy(0).wait()
    idft(ND - 1, (ND - 1) % 2)
    qkv(0)

    q_copy(1).wait()
    attention(0)
    qkv(1)
    outproj(0)

    def body_b(b, carry):
        q_copy(b).wait()

        @pl.when(b >= 4)
        def _():
            out_copy(b - 4, b % 2).wait()
        epilogue(b - 2)
        out_copy(b - 2, b % 2).start()
        attention(b - 1)
        qkv(b)
        outproj(b - 1)
        return carry

    jax.lax.fori_loop(2, NT, body_b, 0)

    out_copy(NT - 4, 0).wait()
    epilogue(NT - 2)
    out_copy(NT - 2, 0).start()
    attention(NT - 1)
    outproj(NT - 1)
    out_copy(NT - 3, 1).wait()
    epilogue(NT - 1)
    out_copy(NT - 1, 1).start()
    out_copy(NT - 2, 0).wait()
    out_copy(NT - 1, 1).wait()


@jax.jit
def pallas_gated_mix__ssm_conv_h3__sliding_local_dilated__prompt_kernel(A_q, A_k, A_v, A_shift_k, A_ssm_k, A_ssm_D, B_x, B_wqkv, B_wo, gate_w):
    fwd, inv, eye = _dft_constants()
    hbm = pl.BlockSpec(memory_space=pl.ANY)
    vm = pl.BlockSpec(memory_space=pltpu.VMEM)
    return pl.pallas_call(
        _kernel,
        out_shape=jax.ShapeDtypeStruct((1, S, D), BF16),
        in_specs=[hbm, hbm, hbm, vm, hbm, vm, hbm, hbm, vm, vm, vm, vm],
        out_specs=hbm,
        scratch_shapes=[
            pltpu.VMEM((ND, S, 128), BF16),
            pltpu.VMEM((ND, S, 128), BF16),
            pltpu.VMEM((ND, 128, S), BF16),
            pltpu.VMEM((S, D), BF16),
            pltpu.VMEM((D, 3 * D), BF16),
            pltpu.VMEM((D, D), BF16),
            pltpu.VMEM((ND, 8, 128), F32),
            pltpu.VMEM((128, 128), U32),
            pltpu.VMEM((64, 256), U32),
            pltpu.VMEM((8 + S, 128), F32),
            pltpu.VMEM((ND, S // 2, 128), U32),
            pltpu.VMEM((2, NA, 256, 128), F32),
            pltpu.VMEM((2, NA, 256, 128), F32),
            pltpu.VMEM((2, NA, 128, 128), U32),
            pltpu.VMEM((2, ND, S, 128), F32),
            pltpu.VMEM((ND, 3 * D, 128), F32),
            pltpu.VMEM((3 * D // 2, D), U32),
            pltpu.VMEM((ND, D, 128), F32),
            pltpu.VMEM((D // 2, D), U32),
            pltpu.VMEM((2, ND, T, 128), F32),
            pltpu.VMEM((ND, HALO + S, 128), F32),
            pltpu.VMEM((ND, HALO + S, 128), F32),
            pltpu.VMEM((8, T, 128), F32),
            pltpu.VMEM((T // 2, D), U32),
            pltpu.VMEM((2, T, D), F32),
            pltpu.VMEM((2, T, D), BF16),
            pltpu.SemaphoreType.DMA((3 * ND,)),
            pltpu.SemaphoreType.DMA((NT,)),
            pltpu.SemaphoreType.DMA((2,)),
            pltpu.SemaphoreType.DMA((2,)),
        ],
        compiler_params=pltpu.CompilerParams(vmem_limit_bytes=100 * 2 ** 20),
    )(A_q, A_k, A_v, A_shift_k, A_ssm_k, A_ssm_D.reshape(1, D), B_wqkv, B_wo, gate_w.reshape(1, D),
      jnp.asarray(fwd, BF16), jnp.asarray(inv, BF16), jnp.asarray(eye, BF16))
```

```python
import contextlib
import functools
import numpy as np
import jax
import jax.numpy as jnp
from jax.experimental import pallas as pl
from jax.experimental.pallas import tpu as pltpu


def E(key, default):
    return default


ONLY = E('ONLY', '')
SCOPES = int(E('SCOPES', '0'))
AN, EN, GN, PACE = int(E('AN', '13')), int(E('EN', '14')), int(E('GN', '10')), int(E('PACE', '4'))
D1, D2, D3 = int(E('D1', '2')), int(E('D2', '4')), int(E('D3', '5'))
DYNZ = int(E('DYNZ', '0'))
AB = int(E('AB', '4'))
ATOK = int(E('ATOK', '0'))
AOFF = int(E('AOFF', '1'))
ARATE = int(E('ARATE', '100'))
AORD = E('AORD', 'cf')
FR = int(E('FR', '100'))
USM = int(E('USM', '1'))
MERGE = int(E('MERGE', '0'))
KVFIRST = int(E('KVFIRST', '1'))
KSPLIT = int(E('KSPLIT', '8'))

WT_AT = int(E('WT_AT', '2'))
LN = int(E('LN', '14'))
EPI = E('EPI', 'late')
GATEP = int(E('GATEP', '1'))
NNW = int(E('NNW', '0'))
NCH = int(E('NCH', '4'))
Q0 = int(E('Q0', '1'))
S, D = 2048, 640
ND = 5
L = 128
NA = S // L
T = 256
NT = S // T
H, DH = 32, 20
HALO = 16
GR = 16
GE = 8
NG = T // GR
LOG2E = 1.4426950408889634
QSCALE = float(DH ** -0.5) * LOG2E
MASKED = -1e9 * LOG2E
F32, BF16, U32 = jnp.float32, jnp.bfloat16, jnp.uint32


def _scope(name):
    return jax.named_scope(name) if SCOPES else contextlib.nullcontext()


def _dft_constants():
    forder = np.concatenate([np.arange(0, 128, 2), np.arange(1, 128, 2)])
    th = np.pi * (2 * forder + 1) / 256.0
    b = np.arange(128)
    fre, fim = np.cos(np.outer(th, b)), -np.sin(np.outer(th, b))
    fwd = np.concatenate([fre, fim, fre + fim], 0)
    gre = np.cos(np.outer(b, th)) / 128
    gim = -np.sin(np.outer(b, th)) / 128
    inv = np.stack([gre, gim], -1).reshape(128, 256)
    return fwd.astype(np.float32), inv.astype(np.float32), np.eye(128, dtype=np.float32)


def _bf(x):
    return pltpu.bitcast(x, BF16)


def _u32(x):
    return pltpu.bitcast(x, U32)


def _bmul(x, t8):
    return (x.reshape(-1, 8, 128) * t8).reshape(x.shape)


def _badd(x, t8):
    return (x.reshape(-1, 8, 128) + t8).reshape(x.shape)


def _dot(a, b):
    return jnp.dot(a, b, preferred_element_type=F32)


def _dot_nt(a, b):
    return jax.lax.dot_general(a, b, (((1,), (1,)), ((), ())), preferred_element_type=F32)


class _Copies:
    def __init__(self, cs):
        self.cs = list(cs)

    def start(self):
        for c in self.cs:
            c.start()

    def wait(self):
        for c in self.cs:
            c.wait()


def _kernel(q_hbm, k_hbm, v_hbm, shk_hbm, sk_hbm, dvec_hbm, wqkv_hbm, wo_hbm, gw_hbm,
            fwd_hbm, inv_hbm, eye_hbm,
            out_hbm,
            shk_ref, dvec_ref, gw_ref, fwd_ref, inv_ref, eye_ref,
            kbuf, vbuf, skbuf, qbuf, wqkv_v, wo_v, par, zvec, zsm, fwdp, invp, onesp, eyep,
            kf, kvp, ubuf0, ubuf1, kpbuf0, kpbuf1, ybuf0, ybuf1, kst0, kst1, y2, wt, wtp, wnn, wof, wop,
            qp0, qp1, kp0, kp1, vp0, vp1, pbuf, sbuf, lbuf, op, bres0, bres1, obuf0, obuf1, gsp, glog0, glog1,
            sem_a, sem_q, sem_w, sem_o, sem_s, sem_f):
    ubuf, kpbuf, ybuf, kstb = (ubuf0, ubuf1), (kpbuf0, kpbuf1), (ybuf0, ybuf1), (kst0, kst1)
    qp, kp, vp = (qp0, qp1), (kp0, kp1), (vp0, vp1)
    bres, obuf, glog = (bres0, bres1), (obuf0, obuf1), (glog0, glog1)
    skw, qw, wqkvw = skbuf.bitcast(U32), qbuf.bitcast(U32), wqkv_v.bitcast(U32)

    def kv_copy(j):
        return _Copies(
            [pltpu.make_async_copy(k_hbm.at[0, :, pl.ds(j * 128, 128)], kbuf.at[j], sem_a.at[3 * j]),
             pltpu.make_async_copy(v_hbm.at[0, :, pl.ds(j * 128, 128)], vbuf.at[j], sem_a.at[3 * j + 1])])

    def sk_copy(j):
        return _Copies(pltpu.make_async_copy(sk_hbm.at[pl.ds(j * 128, 128), pl.ds(m * L, L)], skbuf.at[j, m],
                                             sem_a.at[3 * j + 2]) for m in range(NA))

    def slab_copy(j):
        return _Copies(kv_copy(j).cs + sk_copy(j).cs)

    def first_copy(ch):
        rows = pl.ds(ch * (S // NCH), S // NCH)
        ms = range(ch * (NA // NCH), (ch + 1) * (NA // NCH))
        return _Copies(
            [pltpu.make_async_copy(k_hbm.at[0, rows, pl.ds(0, 128)], kbuf.at[0, rows], sem_f.at[ch]),
             pltpu.make_async_copy(v_hbm.at[0, rows, pl.ds(0, 128)], vbuf.at[0, rows], sem_f.at[ch])]
            + [pltpu.make_async_copy(sk_hbm.at[pl.ds(0, 128), pl.ds(m * L, L)], skbuf.at[0, m], sem_f.at[ch])
               for m in ms])

    small_copy = _Copies(pltpu.make_async_copy(a, b, sem_s.at[i]) for i, (a, b) in enumerate(
        [(shk_hbm, shk_ref), (dvec_hbm, dvec_ref), (gw_hbm, gw_ref), (fwd_hbm, fwd_ref), (inv_hbm, inv_ref),
         (eye_hbm, eye_ref)]))
    def q_copy(b):
        rows = pl.ds(b * T, T)
        return _Copies(pltpu.make_async_copy(q_hbm.at[0, rows, pl.ds(j * 128, 128)], qbuf.at[j, rows], sem_q.at[b])
                       for j in range(ND))

    wqkv_copy = _Copies(pltpu.make_async_copy(wqkv_hbm.at[:, pl.ds(n * 128, 128)], wqkv_v.at[n], sem_w.at[0])
                        for n in range(15))
    wo_copy = _Copies(pltpu.make_async_copy(wo_hbm.at[:, pl.ds(n * 128, 128)], wo_v.at[n], sem_w.at[1])
                      for n in range(ND))

    def out_copy(b, s):
        return _Copies(pltpu.make_async_copy(obuf[s].at[j], out_hbm.at[0, pl.ds(b * T, T), pl.ds(j * 128, 128)],
                                             sem_o.at[s]) for j in range(ND))

    with _scope("s_issue"):
        small_copy.start()
        if ONLY != 'B':
            first_copy(0).start()
    with _scope("s_wait"):
        small_copy.wait()
    if ONLY != 'B':
        for ch in range(1, NCH):
            first_copy(ch).start()

    with _scope("s_setup"):
        taps = shk_ref[...].astype(F32)
        dv = dvec_ref[...].astype(F32).reshape(1, D)
        gw = gw_ref[...].astype(F32).reshape(1, D)
        for j in range(ND):
            for i in range(4):
                par[j, i] = jnp.broadcast_to(taps[i:i + 1, j * 128:(j + 1) * 128], (8, 128))
            par[j, 4] = jnp.broadcast_to(dv[:, j * 128:(j + 1) * 128], (8, 128))
            par[j, 5] = jnp.broadcast_to(gw[:, j * 128:(j + 1) * 128], (8, 128))
        zvec[...] = jnp.zeros((8, 128), F32)
        for i in range(64):
            zsm[i] = 0
        fwdp[...] = _u32(fwd_ref[...])
        invp[...] = _u32(inv_ref[...])
        eyep[...] = _u32(eye_ref[...])
        onesp[...] = _u32(jnp.ones((128, 128), BF16))
        kf[0:8, :] = jnp.zeros((8, 128), F32)
        for j in range(ND):
            kp0[j, 0:HALO, :] = jnp.zeros((HALO, 128), F32)
            vp0[j, 0:HALO, :] = jnp.zeros((HALO, 128), F32)

    def fresh(i):
        return pl.multiple_of(zsm[i] * 8, 8)

    def kvprep(j, blks=range(NA)):
        for c in blks:
            kf[8 + c * L:8 + (c + 1) * L, :] = kbuf[j, c * L:(c + 1) * L, :].astype(F32)
        t = [par[j, i] for i in range(4)]
        for c in [4 * cc + q for cc in blks for q in range(4)]:
            r = c * 32
            ks = _bmul(kf[8 + r:8 + r + 32, :], t[0])
            for i in range(1, 4):
                ks = ks + _bmul(kf[8 + r - i:8 + r - i + 32, :], t[i])
            kv = ks * vbuf[j, r:r + 32, :].astype(F32)
            kvp[j, r // 2:r // 2 + 16, :] = _u32(kv.astype(BF16))

    def dft_u(j, s, cs=range(NA)):
        toks = []
        for c in cs:
            f = _bf(fwdp[pl.ds(fresh(16 + c), 192 if USM else 128), :])
            r = _dot(f, _bf(kvp[j, c * 64:(c + 1) * 64, :]))
            for i in range(3 if USM else 2):
                ubuf[s][i, c] = r[i * 128:(i + 1) * 128]
            toks.append(r[0:8])
        return toks

    def dft_k(j, s, ms=range(NA)):
        toks = []
        for m in ms:
            f = _bf(fwdp[pl.ds(fresh(32 + m), 128), :])
            r = _dot_nt(f, _bf(skw[j, m]))
            kpbuf[s][m] = r
            toks.append(r[0:8])
        return toks

    def aconv(s, plist=range(16), toks=None, mode=None, tz=True):
        ub, kb, yb = ubuf[s], kpbuf[s], ybuf[s]

        def kprep(p):
            r, im = p * 8, 128 + p * 8
            kst = kstb[p % 2]
            pr = [kb[m, r:r + 8, :] for m in range(NA)]
            pi = [kb[m, im:im + 8, :] for m in range(NA)]
            for m in range(NA):
                if m == 0:
                    kr, ki = pr[0], pi[0]
                    if toks is not None and toks[p] is not None:
                        kr = kr + (toks[p] * zvec[...] if tz else toks[p])
                elif p < 8:
                    kr, ki = pr[m] - pi[m - 1], pi[m] + pr[m - 1]
                else:
                    kr, ki = pr[m] + pi[m - 1], pi[m] - pr[m - 1]
                kst[m * 8:m * 8 + 8, :] = kr
                kst[128 + m * 8:128 + m * 8 + 8, :] = kr + ki
                kst[256 + m * 8:256 + m * 8 + 8, :] = ki - kr

        def macs(p):
            r = p * 8
            kst = kstb[p % 2]
            for bi, a0 in enumerate(range(0, NA, AB)):
                z = fresh(bi)
                acc = [[None] * AB for _ in range(3)]
                for c in range(a0 + AB):
                    if USM:
                        uu = [ub[i, c, pl.ds(z + r, 8), :] for i in (2, 1, 0)]
                    else:
                        u_i, u_r = ub[1, c, pl.ds(z + r, 8), :], ub[0, c, pl.ds(z + r, 8), :]
                        uu = [u_r + u_i, u_i, u_r]
                    for i in range(AB):
                        m = a0 + i - c
                        if m < 0:
                            continue
                        for t in range(3):
                            x = kst[pl.ds(z + t * 128 + m * 8, 8), :] * uu[t]
                            acc[t][i] = x if acc[t][i] is None else acc[t][i] + x
                for i in range(AB):
                    yb[a0 + i, r:r + 8, :] = pltpu.pack_elementwise(
                        [acc[0][i] - acc[1][i], acc[0][i] + acc[2][i]], packed_dtype=BF16)

        if mode == 'begin':
            kprep(0)
            return
        if mode == 'step':
            p = plist
            if p + 1 < 16:
                kprep(p + 1)
            macs(p)
            return
        plist = list(plist)
        kprep(plist[0])
        for n, p in enumerate(plist):
            if n + 1 < len(plist):
                kprep(plist[n + 1])
            macs(p)

    def aconv_begin(s):
        aconv(s, mode='begin')

    def aconv_step(s, p):
        aconv(s, p, mode='step')

    def idft(j, s, as_=range(NA)):
        toks = []
        for a in as_:
            z = fresh(48 + a)
            g0 = _bf(invp[pl.ds(z, 64), 0:128])
            g1 = _bf(invp[pl.ds(z, 64), 128:256])
            r0 = _dot(g0, _bf(ybuf[s][a, 0:64, :]))
            r1 = _dot(g1, _bf(ybuf[s][a, 64:128, :]))
            y2[0, j, a * L:(a + 1) * L, :] = r0
            y2[1, j, a * L:(a + 1) * L, :] = r1
            toks.append(r1[0:8])
        return toks

    def w_transpose():
        eye = _bf(eyep[...])
        for n in range(15):
            r = _dot_nt(eye, _bf(wqkvw[n]))
            for kt in range(ND):
                wt[kt, n * 128:(n + 1) * 128, :] = r[:, kt * 128:(kt + 1) * 128]

    def w_permute():
        for p in range(3):
            for dh in range(DH):
                for kt in range(ND):
                    rows = wt[kt, pl.ds(p * D + dh, H, stride=DH), :]
                    r0 = (p * D + dh * H) // 2
                    wtp[r0:r0 + H // 2, kt * 128:(kt + 1) * 128] = _u32(rows.astype(BF16))

    def wo_permute():
        for j in range(ND):
            wof[j] = wo_v[j].astype(F32)
        for dh in range(DH):
            for j in range(ND):
                rows = wof[j, pl.ds(dh, H, stride=DH), :]
                r0 = dh * H // 2
                wop[r0:r0 + H // 2, j * 128:(j + 1) * 128] = _u32(rows.astype(BF16))

    def qkv(b, s):
        r0 = pl.multiple_of(b * (T // 2), T // 2)
        x = jnp.concatenate([_bf(qw[j, pl.ds(r0, T // 2), :]) for j in range(ND)], axis=1)
        r = _dot(x, _bf(wnn[...])) if NNW else _dot_nt(x, _bf(wtp[...]))
        for j in range(ND):
            qp[s][j] = r[:, j * 128:(j + 1) * 128]
            kp[s][j, HALO:HALO + T, :] = r[:, D + j * 128:D + (j + 1) * 128]
            vp[s][j, HALO:HALO + T, :] = r[:, 2 * D + j * 128:2 * D + (j + 1) * 128]
        return [r[0:8, n * 128:(n + 1) * 128] * zvec[...] for n in range(15)]

    def gate(b, s, mt=None):
        r0 = pl.multiple_of(b * T, T)
        for g in range(NG):
            sm = None if mt is None else jnp.concatenate([mt[(g * GN) // NG]] * (GR // 8), axis=0)
            for j in range(ND):
                t = _bmul(qbuf[j, pl.ds(r0 + g * GR, GR), :].astype(F32), par[j, 5])
                sm = t if sm is None else sm + t
            hi = sm.astype(BF16)
            lo = (sm - hi.astype(F32)).astype(BF16)
            gsp[0, g * GR // 2:(g + 1) * GR // 2, :] = _u32(hi)
            gsp[1, g * GR // 2:(g + 1) * GR // 2, :] = _u32(lo)
        ones = _bf(onesp[...])
        glog[s][0] = _dot(_bf(gsp[0]), ones)
        glog[s][1] = _dot(_bf(gsp[1]), ones)

    def halo(s):
        for j in range(ND):
            kp[1 - s][j, 0:HALO, :] = kp[s][j, T:T + HALO, :]
            vp[1 - s][j, 0:HALO, :] = vp[s][j, T:T + HALO, :]

    def softmax_pv(vv, row):
        lg = [lbuf[w, row:row + GR, :] for w in range(8)]
        m = lg[0]
        for w in range(1, 8):
            m = jnp.maximum(m, lg[w])
        es = [jnp.exp2(l - m) for l in lg]
        sm = es[0]
        for w in range(1, 8):
            sm = sm + es[w]
        inv = 1.0 / sm
        for j in range(ND):
            acc = None
            for w in range(8):
                o = row + HALO - 2 * w
                t = es[w] * vv[j, o:o + GR, :]
                acc = t if acc is None else acc + t
            res = acc * inv
            op[row // 2:(row + GR) // 2, j * 128:(j + 1) * 128] = _u32(res.astype(BF16))
        return res[0:8]

    def qk(qq, kk, row, tok):
        if tok is None:
            q = [qq[j, row:row + GE, :] * QSCALE for j in range(ND)]
        else:
            sc = tok + QSCALE
            q = [qq[j, row:row + GE, :] * sc for j in range(ND)]
        out = []
        for w in range(8):
            p = None
            o = row + HALO - 2 * w
            for j in range(ND):
                t = q[j] * kk[j, o:o + GE, :]
                p = t if p is None else p + t
            out.append(p)
        return out

    def attention(b, s, mt=None):
        qq, kk, vv = qp[s], kp[s], vp[s]
        n1 = T // GE
        per = GR // GE
        r1, r2, done = {}, {}, {}
        for g in range(n1 + D3 + per):
            if g < n1:
                row = g * GE
                tok = None
                if mt is not None:
                    tok = mt[(g * AN) // n1]
                    prev = done.get(row // GR - PACE) if PACE else None
                    if prev is not None:
                        tok = tok + prev * zvec[...]
                r1[g] = []
                for w, p in enumerate(qk(qq, kk, row, tok)):
                    pbuf[w, row:row + GE, :] = p
                    r1[g].append(pltpu.roll(p, 64, 1))
            gg = g - D1
            if 0 <= gg < n1:
                row = gg * GE
                r2[gg] = []
                for w, r in enumerate(r1.pop(gg)):
                    sm = pbuf[w, row:row + GE, :] + r
                    sbuf[w, row:row + GE, :] = sm
                    r2[gg].append(pltpu.roll(sm, 32, 1))
            gg = g - D2
            if 0 <= gg < n1:
                row = gg * GE
                for w, r in enumerate(r2.pop(gg)):
                    l = sbuf[w, row:row + GE, :] + r
                    if row < HALO and w > 0:
                        t = b * T + row + jax.lax.broadcasted_iota(jnp.int32, (GE, 128), 0)
                        l = jnp.where(t >= 2 * w, l, MASKED)
                    lbuf[w, row:row + GE, :] = l
            gg = g - D3
            if 0 <= gg < n1 and (gg + 1) % per == 0:
                row = (gg + 1 - per) * GE
                done[row // GR] = softmax_pv(vv, row)

    def outproj(s):
        r = _dot(_bf(op[...]), _bf(wop[...]))
        bres[s][...] = r
        return [r[0:8, n * 128:(n + 1) * 128] * zvec[...] for n in range(ND)]

    def epilogue(b, s, mt=None):
        r0 = pl.multiple_of(b * T, T)
        for g in range(NG):
            row = r0 + g * GR
            rowh = pl.multiple_of(b * (T // 2), T // 2) + g * (GR // 2)
            gl = glog[s][0, g * GR:(g + 1) * GR, :] + glog[s][1, g * GR:(g + 1) * GR, :]
            if mt is not None:
                gl = _badd(gl, mt[(g * EN) // NG])
            gt = jax.nn.sigmoid(gl)
            for j in range(ND):
                q = qbuf[j, pl.ds(row, GR), :].astype(F32)
                kv = _bf(kvp[j, pl.ds(rowh, GR // 2), :]).astype(F32)
                z = y2[0, j, pl.ds(row, GR), :] + y2[1, j, pl.ds(row, GR), :] + _bmul(kv, par[j, 4])
                bb = bres[s][g * GR:(g + 1) * GR, j * 128:(j + 1) * 128]
                o = bb + gt * (q * z - bb)
                obuf[s][j, g * GR:(g + 1) * GR, :] = o.astype(BF16)

    def region(k, f):
        pl.when(zsm[k % 64] == 0)(f)

    P = functools.partial

    wq_a, wq_b = _Copies(wqkv_copy.cs[:8]), _Copies(wqkv_copy.cs[8:])

    def block_x(j):
        s = j % 2
        with _scope("waitX%d" % j):
            sk_copy(j + 1).wait()
            if j == WT_AT:
                wqkv_copy.wait()
        if j + 2 < ND:
            sk_copy(j + 2).start()
        if j == 0:
            wq_a.start()
        if j == 1:
            wq_b.start()
        if j == 2:
            wo_copy.start()
        if j == 3:
            q_copy(1).start()
        with _scope("X%d" % j):
            aconv(s)
            if j >= 1:
                idft(j - 1, 1 - s)
            dft_k(j + 1, 1 - s)
            if j == WT_AT:
                w_transpose()

    def block_y(j):
        s = j % 2
        with _scope("waitY%d" % j):
            kv_copy(j + 1).wait()
            if j == WT_AT:
                wo_copy.wait()
        if j + 2 < ND:
            kv_copy(j + 2).start()
        if j == 2:
            q_copy(0).start()
        if j == 3:
            q_copy(2).start()
        with _scope("Y%d" % j):
            kvprep(j + 1)
            if j == WT_AT:
                w_permute()
                wo_permute()
            dft_u(j + 1, 1 - s)

    def body_a(j, carry):
        return carry

    def block_b(b, s):
        if ONLY == '':
            q_copy(b).wait()

        @pl.when(b >= 4)
        def _():
            out_copy(b - 4, s).wait()
        with _scope("B"):
            halo(1 - s)
            mt = qkv(b, s)
            if EPI == 'paced':
                epilogue(b - 2, s, mt)
            elif EPI == 'free':
                epilogue(b - 2, s)
            elif EPI == 'late':
                epilogue(b - 2, s, [mt[14]] * 15)
            if EPI != 'after':
                out_copy(b - 2, s).start()
            if E('NOATT', '0') != '1':
                attention(b - 1, 1 - s, mt)
            if E('NOGATE', '0') != '1':
                gate(b - 1, 1 - s, mt if GATEP else None)
            if EPI == 'after':
                ot = outproj(1 - s)
                epilogue(b - 2, s, [ot[(g * 5) // 15] for g in range(15)])
                out_copy(b - 2, s).start()
            else:
                outproj(1 - s)

    def body_b(b, carry):
        if E('ONEPAR', '0') == '1':
            block_b(b, 0)
            return carry
        for s in range(2):
            pl.when(b % 2 == s)(functools.partial(block_b, b, s))
        return carry

    if ONLY != 'B':
        nb = NA // NCH
        for ch in range(NCH):
            with _scope("wait0"):
                first_copy(ch).wait()
            if ch == 1:
                sk_copy(1).start()
            if ch == NCH - 1:
                kv_copy(1).start()
            with _scope("pro"):
                blks = range(ch * nb, (ch + 1) * nb)
                kvprep(0, blks)
                dft_k(0, 0, blks)
                dft_u(0, 0, blks)

        for j in range(ND - 1):
            region(2 * j, P(block_x, j))
            region(2 * j + 1, P(block_y, j))

    if ONLY == '':
        def block_alast():
            q_copy(0).wait()
            for b in range(3, NT):
                q_copy(b).start()
            with _scope("Alast"):
                if Q0 == 2:
                    idft(ND - 2, (ND - 2) % 2)
                    mt = qkv(0, 0)
                    toks = [None] + [mt[min(14, ((p - 1) * LN) // 16)] for p in range(1, 16)]
                    aconv((ND - 1) % 2, range(16), toks, tz=False)
                else:
                    aconv((ND - 1) % 2)
                    idft(ND - 2, (ND - 2) % 2)
                    if Q0:
                        qkv(0, 0)

        region(10, block_alast)

        def block_b1():
            q_copy(1).wait()
            with _scope("B1"):
                if not Q0:
                    qkv(0, 0)
                idft(ND - 1, (ND - 1) % 2)
                halo(0)
                mt = qkv(1, 1)
                attention(0, 0, mt)
                gate(0, 0, mt)
                outproj(0)

        region(11, block_b1)

    if ONLY != 'A':
        jax.lax.fori_loop(2, NT, body_b, 0)

    if ONLY == '':
        with _scope("fin1"):
            out_copy(NT - 4, 0).wait()
            epilogue(NT - 2, 0)
            out_copy(NT - 2, 0).start()
            attention(NT - 1, 1)
            gate(NT - 1, 1)
            outproj(1)
        with _scope("fin2"):
            out_copy(NT - 3, 1).wait()
            epilogue(NT - 1, 1)
            out_copy(NT - 1, 1).start()
        with _scope("fin3"):
            out_copy(NT - 2, 0).wait()
            out_copy(NT - 1, 1).wait()
    elif ONLY == 'B':
        out_copy(NT - 4, 0).wait()
        out_copy(NT - 3, 0 if E('ONEPAR', '0') == '1' else 1).wait()
    else:
        for b in range(3):
            q_copy(b).wait()


@jax.jit
def pallas_gated_mix__ssm_conv_h3__sliding_local_dilated__prompt_kernel(A_q, A_k, A_v, A_shift_k, A_ssm_k, A_ssm_D, B_x, B_wqkv, B_wo, gate_w):
    fwd, inv, eye = _dft_constants()
    hbm = pl.BlockSpec(memory_space=pl.ANY)
    vm = pl.BlockSpec(memory_space=pltpu.VMEM)
    two = lambda shape, dt: [pltpu.VMEM(shape, dt), pltpu.VMEM(shape, dt)]
    return pl.pallas_call(
        _kernel,
        out_shape=jax.ShapeDtypeStruct((1, S, D), BF16),
        in_specs=[hbm] * 12,
        out_specs=hbm,
        scratch_shapes=[
            pltpu.VMEM((4, D), BF16),
            pltpu.VMEM((D,), BF16),
            pltpu.VMEM((D,), BF16),
            pltpu.VMEM((384, 128), BF16),
            pltpu.VMEM((128, 256), BF16),
            pltpu.VMEM((128, 128), BF16),
            pltpu.VMEM((ND, S, 128), BF16),
            pltpu.VMEM((ND, S, 128), BF16),
            pltpu.VMEM((ND, NA, 128, L), BF16),
            pltpu.VMEM((ND, S, 128), BF16),
            pltpu.VMEM((15, D, 128), BF16),
            pltpu.VMEM((ND, D, 128), BF16),
            pltpu.VMEM((ND, 6, 8, 128), F32),
            pltpu.VMEM((8, 128), F32),
            pltpu.SMEM((64,), jnp.int32),
            pltpu.VMEM((192, 128), U32),
            pltpu.VMEM((64, 256), U32),
            pltpu.VMEM((64, 128), U32),
            pltpu.VMEM((64, 128), U32),
            pltpu.VMEM((8 + S, 128), F32),
            pltpu.VMEM((ND, S // 2, 128), U32),
            *two((3, NA, 128, 128), F32),
            *two((NA, 256, 128), F32),
            *two((NA, 128, 128), U32),
            *two((384, 128), F32),
            pltpu.VMEM((2, ND, S, 128), F32),
            pltpu.VMEM((ND, 3 * D, 128), F32),
            pltpu.VMEM((3 * D // 2, D), U32),
            pltpu.VMEM((D // 2, 3 * D), U32),
            pltpu.VMEM((ND, D, 128), F32),
            pltpu.VMEM((D // 2, D), U32),
            *two((ND, T, 128), F32),
            *two((ND, HALO + T, 128), F32),
            *two((ND, HALO + T, 128), F32),
            pltpu.VMEM((8, T, 128), F32),
            pltpu.VMEM((8, T, 128), F32),
            pltpu.VMEM((8, T, 128), F32),
            pltpu.VMEM((T // 2, D), U32),
            *two((T, D), F32),
            *two((ND, T, 128), BF16),
            pltpu.VMEM((2, T // 2, 128), U32),
            *two((2, T, 128), F32),
            pltpu.SemaphoreType.DMA((3 * ND,)),
            pltpu.SemaphoreType.DMA((NT,)),
            pltpu.SemaphoreType.DMA((2,)),
            pltpu.SemaphoreType.DMA((2,)),
            pltpu.SemaphoreType.DMA((6,)),
            pltpu.SemaphoreType.DMA((NCH,)),
        ],
        compiler_params=pltpu.CompilerParams(vmem_limit_bytes=100 * 2 ** 20),
    )(A_q, A_k, A_v, A_shift_k.T, A_ssm_k, A_ssm_D, B_wqkv, B_wo, gate_w,
      jnp.asarray(fwd, BF16), jnp.asarray(inv, BF16), jnp.asarray(eye, BF16))
```

```python
import contextlib
import functools
import numpy as np
import jax
import jax.numpy as jnp
from jax.experimental import pallas as pl
from jax.experimental.pallas import tpu as pltpu


def E(key, default):
    return default


ONLY = E('ONLY', '')
SCOPES = int(E('SCOPES', '0'))
AN, EN, GN, PACE = int(E('AN', '13')), int(E('EN', '14')), int(E('GN', '10')), int(E('PACE', '4'))
D1, D2, D3 = int(E('D1', '2')), int(E('D2', '4')), int(E('D3', '5'))
DYNZ = int(E('DYNZ', '0'))
AB = int(E('AB', '4'))
ATOK = int(E('ATOK', '0'))
AOFF = int(E('AOFF', '1'))
ARATE = int(E('ARATE', '100'))
AORD = E('AORD', 'cf')
FR = int(E('FR', '100'))
USM = int(E('USM', '0'))
MERGE = int(E('MERGE', '0'))
KVFIRST = int(E('KVFIRST', '1'))
KSPLIT = int(E('KSPLIT', '8'))

WT_AT = int(E('WT_AT', '2'))
LN = int(E('LN', '15'))
EPI = E('EPI', 'late')
GATEP = int(E('GATEP', '1'))
NNW = int(E('NNW', '0'))
LOFF = int(E('LOFF', '0'))
LAB = int(E('LAB', '2'))
KVPOS = E('KVPOS', 'post')
TFIRST = int(E('TFIRST', '0'))
KVT = [int(x) for x in E('KVT', '-1,-1,-1').split(',')]
GATE = E('GATE', 'mem')
BIG = int(E('BIG', '0'))
KSPREAD = int(E('KSPREAD', '1'))
NCH = int(E('NCH', '4'))
Q0 = int(E('Q0', '1'))
S, D = 2048, 640
ND = 5
L = 128
NA = S // L
T = 256
NT = S // T
H, DH = 32, 20
HALO = 16
KH = 8
GR = 16
GE = 8
NG = T // GR
LOG2E = 1.4426950408889634
QSCALE = float(DH ** -0.5) * LOG2E
MASKED = -1e9 * LOG2E
F32, BF16, U32 = jnp.float32, jnp.bfloat16, jnp.uint32


def _scope(name):
    return jax.named_scope(name) if SCOPES else contextlib.nullcontext()


def _dft_constants():
    forder = np.concatenate([np.arange(0, 128, 2), np.arange(1, 128, 2)])
    th = np.pi * (2 * forder + 1) / 256.0
    b = np.arange(128)
    fre, fim = np.cos(np.outer(th, b)), -np.sin(np.outer(th, b))
    fwd = np.concatenate([fre, fim, fre + fim], 0)
    gre = np.cos(np.outer(b, th)) / 128
    gim = -np.sin(np.outer(b, th)) / 128
    inv = np.stack([gre, gim], -1).reshape(128, 256)
    return fwd.astype(np.float32), inv.astype(np.float32), np.eye(128, dtype=np.float32)


def _bf(x):
    return pltpu.bitcast(x, BF16)


def _u32(x):
    return pltpu.bitcast(x, U32)


def _bmul(x, t8):
    return (x.reshape(-1, 8, 128) * t8).reshape(x.shape)


def _badd(x, t8):
    return (x.reshape(-1, 8, 128) + t8).reshape(x.shape)


def _dot(a, b):
    return jnp.dot(a, b, preferred_element_type=F32)


def _dot_nt(a, b):
    return jax.lax.dot_general(a, b, (((1,), (1,)), ((), ())), preferred_element_type=F32)


class _Copies:
    def __init__(self, cs):
        self.cs = list(cs)

    def start(self):
        for c in self.cs:
            c.start()

    def wait(self):
        for c in self.cs:
            c.wait()


def _kernel(q_hbm, k_hbm, v_hbm, shk_hbm, sk_hbm, dvec_hbm, wqkv_hbm, wo_hbm, gw_hbm,
            fwd_hbm, inv_hbm, eye_hbm,
            out_hbm,
            shk_ref, dvec_ref, gw_ref, fwd_ref, inv_ref, eye_ref,
            kbuf, vbuf, skbuf, qbuf, wqkv_v, wo_v, par, zvec, zsm, fwdp, invp, onesp, eyep,
            kvp, ubuf0, ubuf1, kpbuf0, kpbuf1, ybuf0, ybuf1, kst0, kst1, y2, wt, wtp, wnn, wof, wop,
            qp0, qp1, kp0, kp1, vp0, vp1, pbuf, sbuf, lbuf, op, bres0, bres1, obuf0, obuf1, gsp, glog0, glog1,
            sem_a, sem_q, sem_w, sem_o, sem_s, sem_f):
    ubuf, kpbuf, ybuf, kstb = (ubuf0, ubuf1), (kpbuf0, kpbuf1), (ybuf0, ybuf1), (kst0, kst1)
    qp, kp, vp = (qp0, qp1), (kp0, kp1), (vp0, vp1)
    bres, obuf, glog = (bres0, bres1), (obuf0, obuf1), (glog0, glog1)
    skw, qw, wqkvw = skbuf.bitcast(U32), qbuf.bitcast(U32), wqkv_v.bitcast(U32)
    kw, vw = kbuf.bitcast(U32), vbuf.bitcast(U32)

    def kv_copy(j):
        return _Copies(
            [pltpu.make_async_copy(k_hbm.at[0, :, pl.ds(j * 128, 128)], kbuf.at[j, pl.ds(2 * KH, S)], sem_a.at[3 * j]),
             pltpu.make_async_copy(v_hbm.at[0, :, pl.ds(j * 128, 128)], vbuf.at[j], sem_a.at[3 * j + 1])])

    def sk_copy(j):
        return _Copies(pltpu.make_async_copy(sk_hbm.at[pl.ds(j * 128, 128), pl.ds(m * L, L)], skbuf.at[j, m],
                                             sem_a.at[3 * j + 2]) for m in range(NA))

    def slab_copy(j):
        return _Copies(kv_copy(j).cs + sk_copy(j).cs)

    def first_copy(ch):
        rows = pl.ds(ch * (S // NCH), S // NCH)
        ms = range(ch * (NA // NCH), (ch + 1) * (NA // NCH))
        return _Copies(
            [pltpu.make_async_copy(k_hbm.at[0, rows, pl.ds(0, 128)],
                                   kbuf.at[0, pl.ds(2 * KH + ch * (S // NCH), S // NCH)], sem_f.at[ch]),
             pltpu.make_async_copy(v_hbm.at[0, rows, pl.ds(0, 128)], vbuf.at[0, rows], sem_f.at[ch])]
            + [pltpu.make_async_copy(sk_hbm.at[pl.ds(0, 128), pl.ds(m * L, L)], skbuf.at[0, m], sem_f.at[ch])
               for m in ms])

    small_copy = _Copies(pltpu.make_async_copy(a, b, sem_s.at[i]) for i, (a, b) in enumerate(
        [(shk_hbm, shk_ref), (dvec_hbm, dvec_ref), (gw_hbm, gw_ref), (fwd_hbm, fwd_ref), (inv_hbm, inv_ref),
         (eye_hbm, eye_ref)]))
    def q_copy(b):
        rows = pl.ds(b * T, T)
        return _Copies(pltpu.make_async_copy(q_hbm.at[0, rows, pl.ds(j * 128, 128)], qbuf.at[j, rows], sem_q.at[b])
                       for j in range(ND))

    wqkv_copy = _Copies(pltpu.make_async_copy(wqkv_hbm.at[:, pl.ds(n * 128, 128)], wqkv_v.at[n], sem_w.at[0])
                        for n in range(15))
    wo_copy = _Copies(pltpu.make_async_copy(wo_hbm.at[:, pl.ds(n * 128, 128)], wo_v.at[n], sem_w.at[1])
                      for n in range(ND))

    def out_copy(b, s):
        return _Copies(pltpu.make_async_copy(obuf[s].at[j], out_hbm.at[0, pl.ds(b * T, T), pl.ds(j * 128, 128)],
                                             sem_o.at[s]) for j in range(ND))

    with _scope("s_issue"):
        small_copy.start()
        if ONLY != 'B':
            first_copy(0).start()
    with _scope("s_wait"):
        small_copy.wait()
    if ONLY != 'B':
        for ch in range(1, NCH):
            first_copy(ch).start()

    with _scope("s_setup"):
        taps = shk_ref[...].astype(F32)
        dv = dvec_ref[...].astype(F32).reshape(1, D)
        gw = gw_ref[...].astype(F32).reshape(1, D)
        for j in range(ND):
            for i in range(4):
                par[j, i] = jnp.broadcast_to(taps[i:i + 1, j * 128:(j + 1) * 128], (8, 128))
            par[j, 4] = jnp.broadcast_to(dv[:, j * 128:(j + 1) * 128], (8, 128))
            par[j, 5] = jnp.broadcast_to(gw[:, j * 128:(j + 1) * 128], (8, 128))
        zvec[...] = jnp.zeros((8, 128), F32)
        for i in range(64):
            zsm[i] = 0
        fwdp[...] = _u32(fwd_ref[...])
        invp[...] = _u32(inv_ref[...])
        eyep[...] = _u32(eye_ref[...])
        onesp[...] = _u32(jnp.ones((128, 128), BF16))
        for j in range(ND):
            kw[j, 0:KH, :] = jnp.zeros((KH, 128), U32)
        for j in range(ND):
            kp0[j, 0:HALO, :] = jnp.zeros((HALO, 128), F32)
            vp0[j, 0:HALO, :] = jnp.zeros((HALO, 128), F32)

    def fresh(i):
        return pl.multiple_of(zsm[i] * 8, 8)

    def gated(tok):
        i = tok[0, 0].astype(jnp.int32)
        return pl.multiple_of(jnp.minimum(jnp.maximum(i, zsm[62]), zsm[63]) * 8, 8)

    def kvprep(j, blks=range(NA), tok=None):
        t = [par[j, i] if tok is None else par[j, i] + tok * zvec[...] for i in range(4)]
        even = lambda w: pltpu.bitcast(w << 16, F32)
        odd = lambda w: pltpu.bitcast(w & jnp.uint32(0xFFFF0000), F32)
        for c in blks:
            for q in range(L // 32):
                r = c * (L // 2) + q * 16
                w0 = kw[j, KH + r:KH + r + 16, :]
                w1 = kw[j, KH + r - 1:KH + r + 15, :]
                w2 = kw[j, KH + r - 2:KH + r + 14, :]
                e0, o0, e1, o1, o2 = even(w0), odd(w0), even(w1), odd(w1), odd(w2)
                ks_e = _bmul(e0, t[0]) + _bmul(o1, t[1]) + _bmul(e1, t[2]) + _bmul(o2, t[3])
                ks_o = _bmul(o0, t[0]) + _bmul(e0, t[1]) + _bmul(o1, t[2]) + _bmul(e1, t[3])
                wv = vw[j, r:r + 16, :]
                kvp[j, r:r + 16, :] = pltpu.pack_elementwise([ks_e * even(wv), ks_o * odd(wv)], packed_dtype=BF16)

    def dft_u(j, s, cs=range(NA)):
        cs = list(cs)
        if BIG:
            f = _bf(fwdp[pl.ds(fresh(16), 192 if USM else 128), :])
            rhs = jnp.concatenate([_bf(kvp[j, c * 64:(c + 1) * 64, :]) for c in cs], axis=1)
            r = _dot(f, rhs)
            for n, c in enumerate(cs):
                for i in range(3 if USM else 2):
                    ubuf[s][i, c] = r[i * 128:(i + 1) * 128, n * 128:(n + 1) * 128]
            return [r[0:8, n * 128:(n + 1) * 128] for n in range(len(cs))]
        toks = []
        for c in cs:
            f = _bf(fwdp[pl.ds(fresh(16 + c), 192 if USM else 128), :])
            r = _dot(f, _bf(kvp[j, c * 64:(c + 1) * 64, :]))
            for i in range(3 if USM else 2):
                ubuf[s][i, c] = r[i * 128:(i + 1) * 128]
            toks.append(r[0:8])
        return toks

    def dft_k(j, s, ms=range(NA)):
        ms = list(ms)
        if BIG:
            f = _bf(fwdp[pl.ds(fresh(32), 128), :])
            rhs = jnp.concatenate([_bf(skw[j, m]) for m in ms], axis=0)
            r = _dot_nt(f, rhs)
            for n, m in enumerate(ms):
                kpbuf[s][m] = r[:, n * 128:(n + 1) * 128]
            return [r[0:8, n * 128:(n + 1) * 128] for n in range(len(ms))]
        toks = []
        for m in ms:
            f = _bf(fwdp[pl.ds(fresh(32 + m), 128), :])
            r = _dot_nt(f, _bf(skw[j, m]))
            kpbuf[s][m] = r
            toks.append(r[0:8])
        return toks

    def aconv(s, plist=range(16), toks=None, mode=None, tz=True, btoks=None, ab=AB):
        ub, kb, yb = ubuf[s], kpbuf[s], ybuf[s]

        def kprep(p, ms=range(NA)):
            r, im = p * 8, 128 + p * 8
            kst = kstb[p % 2]
            for m in ms:
                pr, pi = kb[m, r:r + 8, :], kb[m, im:im + 8, :]
                if m == 0:
                    kr, ki = pr, pi
                    if toks is not None and toks[p] is not None:
                        kr = kr + (toks[p] * zvec[...] if tz else toks[p])
                elif p < 8:
                    kr, ki = pr - kb[m - 1, im:im + 8, :], pi + kb[m - 1, r:r + 8, :]
                else:
                    kr, ki = pr + kb[m - 1, im:im + 8, :], pi - kb[m - 1, r:r + 8, :]
                kst[m * 8:m * 8 + 8, :] = kr
                kst[128 + m * 8:128 + m * 8 + 8, :] = kr + ki
                kst[256 + m * 8:256 + m * 8 + 8, :] = ki - kr

        def macs(p, nxt=None):
            r = p * 8
            kst = kstb[p % 2]
            nb = NA // ab
            for bi, a0 in enumerate(range(0, NA, ab)):
                z = fresh(bi)
                if btoks is not None and btoks[p][bi] is not None:
                    z = gated(btoks[p][bi])
                acc = [[None] * ab for _ in range(3)]
                ncs = a0 + ab
                todo = []
                if nxt is not None and KSPREAD:
                    if bi >= nb - 2:
                        half = bi - (nb - 2)
                        todo = list(range(half * 8, half * 8 + 8))
                for c in range(ncs):
                    if USM:
                        uu = [ub[i, c, pl.ds(z + r, 8), :] for i in (2, 1, 0)]
                    else:
                        u_i, u_r = ub[1, c, pl.ds(z + r, 8), :], ub[0, c, pl.ds(z + r, 8), :]
                        uu = [u_r + u_i, u_i, u_r]
                    for i in range(ab):
                        m = a0 + i - c
                        if m < 0:
                            continue
                        for t in range(3):
                            x = kst[pl.ds(z + t * 128 + m * 8, 8), :] * uu[t]
                            acc[t][i] = x if acc[t][i] is None else acc[t][i] + x
                    if todo and c < 8:
                        kprep(nxt, [todo[c]])
                for i in range(ab):
                    yb[a0 + i, r:r + 8, :] = pltpu.pack_elementwise(
                        [acc[0][i] - acc[1][i], acc[0][i] + acc[2][i]], packed_dtype=BF16)

        plist = list(plist)
        kprep(plist[0])
        for n, p in enumerate(plist):
            nxt = plist[n + 1] if n + 1 < len(plist) else None
            if nxt is not None and not KSPREAD:
                kprep(nxt)
            macs(p, nxt)

    def idft(j, s, as_=range(NA)):
        as_ = list(as_)
        if BIG:
            z = fresh(48)
            toks = []
            for h in range(2):
                g = _bf(invp[pl.ds(z, 64), h * 128:(h + 1) * 128])
                rhs = jnp.concatenate([_bf(ybuf[s][a, h * 64:(h + 1) * 64, :]) for a in as_], axis=1)
                r = _dot(g, rhs)
                for n, a in enumerate(as_):
                    y2[h, j, a * L:(a + 1) * L, :] = r[:, n * 128:(n + 1) * 128]
                toks += [r[0:8, n * 128:(n + 1) * 128] for n in range(len(as_))]
            return toks
        toks = []
        for a in as_:
            z = fresh(48 + a)
            g0 = _bf(invp[pl.ds(z, 64), 0:128])
            g1 = _bf(invp[pl.ds(z, 64), 128:256])
            r0 = _dot(g0, _bf(ybuf[s][a, 0:64, :]))
            r1 = _dot(g1, _bf(ybuf[s][a, 64:128, :]))
            y2[0, j, a * L:(a + 1) * L, :] = r0
            y2[1, j, a * L:(a + 1) * L, :] = r1
            toks.append(r1[0:8])
        return toks

    def w_transpose(ns=range(15)):
        toks = []
        for n in ns:
            eye = _bf(eyep[pl.ds(fresh(n), 64), :])
            r = _dot_nt(eye, _bf(wqkvw[n]))
            for kt in range(ND):
                wt[kt, n * 128:(n + 1) * 128, :] = r[:, kt * 128:(kt + 1) * 128]
            toks.append(r[0:8, 0:128])
        return toks

    def w_permute():
        for p in range(3):
            for dh in range(DH):
                for kt in range(ND):
                    rows = wt[kt, pl.ds(p * D + dh, H, stride=DH), :]
                    r0 = (p * D + dh * H) // 2
                    wtp[r0:r0 + H // 2, kt * 128:(kt + 1) * 128] = _u32(rows.astype(BF16))

    def wo_permute():
        for j in range(ND):
            wof[j] = wo_v[j].astype(F32)
        for dh in range(DH):
            for j in range(ND):
                rows = wof[j, pl.ds(dh, H, stride=DH), :]
                r0 = dh * H // 2
                wop[r0:r0 + H // 2, j * 128:(j + 1) * 128] = _u32(rows.astype(BF16))

    def qkv(b, s, fine=False):
        r0 = pl.multiple_of(b * (T // 2), T // 2)
        x = jnp.concatenate([_bf(qw[j, pl.ds(r0, T // 2), :]) for j in range(ND)], axis=1)
        r = _dot(x, _bf(wnn[...])) if NNW else _dot_nt(x, _bf(wtp[...]))
        for j in range(ND):
            qp[s][j] = r[:, j * 128:(j + 1) * 128]
            kp[s][j, HALO:HALO + T, :] = r[:, D + j * 128:D + (j + 1) * 128]
            vp[s][j, HALO:HALO + T, :] = r[:, 2 * D + j * 128:2 * D + (j + 1) * 128]
        if fine:
            return [r[64 * i:64 * i + 8, n * 128:(n + 1) * 128] * zvec[...] for n in range(15) for i in range(4)]
        return [r[0:8, n * 128:(n + 1) * 128] * zvec[...] for n in range(15)]

    def gate(b, s, mt=None):
        r0 = pl.multiple_of(b * T, T)
        for g in range(NG):
            sm = None if mt is None else jnp.concatenate([mt[(g * GN) // NG]] * (GR // 8), axis=0)
            for j in range(ND):
                t = _bmul(qbuf[j, pl.ds(r0 + g * GR, GR), :].astype(F32), par[j, 5])
                sm = t if sm is None else sm + t
            hi = sm.astype(BF16)
            lo = (sm - hi.astype(F32)).astype(BF16)
            gsp[0, g * GR // 2:(g + 1) * GR // 2, :] = _u32(hi)
            gsp[1, g * GR // 2:(g + 1) * GR // 2, :] = _u32(lo)
        ones = _bf(onesp[...])
        glog[s][0] = _dot(_bf(gsp[0]), ones)
        glog[s][1] = _dot(_bf(gsp[1]), ones)

    def halo(s):
        for j in range(ND):
            kp[1 - s][j, 0:HALO, :] = kp[s][j, T:T + HALO, :]
            vp[1 - s][j, 0:HALO, :] = vp[s][j, T:T + HALO, :]

    def softmax_pv(vv, row):
        lg = [lbuf[w, row:row + GR, :] for w in range(8)]
        m = lg[0]
        for w in range(1, 8):
            m = jnp.maximum(m, lg[w])
        es = [(l - m) if E('NOEXP', '0') == '1' else jnp.exp2(l - m) for l in lg]
        sm = es[0]
        for w in range(1, 8):
            sm = sm + es[w]
        inv = 1.0 / sm
        for j in range(ND):
            acc = None
            for w in range(8):
                o = row + HALO - 2 * w
                t = es[w] * vv[j, o:o + GR, :]
                acc = t if acc is None else acc + t
            res = acc * inv
            op[row // 2:(row + GR) // 2, j * 128:(j + 1) * 128] = _u32(res.astype(BF16))
        return res[0:8]

    def qk(qq, kk, row, tok):
        if tok is None:
            q = [qq[j, row:row + GE, :] * QSCALE for j in range(ND)]
        else:
            sc = tok + QSCALE
            q = [qq[j, row:row + GE, :] * sc for j in range(ND)]
        out = []
        for w in range(8):
            p = None
            o = row + HALO - 2 * w
            for j in range(ND):
                t = q[j] * kk[j, o:o + GE, :]
                p = t if p is None else p + t
            out.append(p)
        return out

    def attention(b, s, mt=None):
        qq, kk, vv = qp[s], kp[s], vp[s]
        n1 = T // GE
        per = GR // GE
        r1, r2, done = {}, {}, {}
        for g in range(n1 + D3 + per):
            if g < n1:
                row = g * GE
                tok = None
                if mt is not None:
                    tok = mt[(g * AN) // n1]
                    prev = done.get(row // GR - PACE) if PACE else None
                    if prev is not None:
                        tok = tok + prev * zvec[...]
                r1[g] = []
                for w, p in enumerate(qk(qq, kk, row, tok)):
                    pbuf[w, row:row + GE, :] = p
                    r1[g].append(p * 2.0 if E('NOROLL', '0') == '1' else pltpu.roll(p, 64, 1))
            gg = g - D1
            if 0 <= gg < n1:
                row = gg * GE
                r2[gg] = []
                for w, r in enumerate(r1.pop(gg)):
                    sm = pbuf[w, row:row + GE, :] + r
                    sbuf[w, row:row + GE, :] = sm
                    r2[gg].append(sm * 2.0 if E('NOROLL', '0') == '1' else pltpu.roll(sm, 32, 1))
            gg = g - D2
            if 0 <= gg < n1:
                row = gg * GE
                for w, r in enumerate(r2.pop(gg)):
                    l = sbuf[w, row:row + GE, :] + r
                    if row < HALO and w > 0:
                        t = b * T + row + jax.lax.broadcasted_iota(jnp.int32, (GE, 128), 0)
                        l = jnp.where(t >= 2 * w, l, MASKED)
                    lbuf[w, row:row + GE, :] = l
            gg = g - D3
            if 0 <= gg < n1 and (gg + 1) % per == 0:
                row = (gg + 1 - per) * GE
                done[row // GR] = softmax_pv(vv, row)

    def outproj(s):
        r = _dot(_bf(op[...]), _bf(wop[...]))
        bres[s][...] = r
        return [r[0:8, n * 128:(n + 1) * 128] * zvec[...] for n in range(ND)]

    def epilogue(b, s, mt=None):
        r0 = pl.multiple_of(b * T, T)
        for g in range(NG):
            row = r0 + g * GR
            rowh = pl.multiple_of(b * (T // 2), T // 2) + g * (GR // 2)
            gl = glog[s][0, g * GR:(g + 1) * GR, :] + glog[s][1, g * GR:(g + 1) * GR, :]
            if mt is not None:
                gl = _badd(gl, mt[(g * EN) // NG])
            gt = jax.nn.sigmoid(gl)
            for j in range(ND):
                q = qbuf[j, pl.ds(row, GR), :].astype(F32)
                kv = _bf(kvp[j, pl.ds(rowh, GR // 2), :]).astype(F32)
                z = y2[0, j, pl.ds(row, GR), :] + y2[1, j, pl.ds(row, GR), :] + _bmul(kv, par[j, 4])
                bb = bres[s][g * GR:(g + 1) * GR, j * 128:(j + 1) * 128]
                o = bb + gt * (q * z - bb)
                obuf[s][j, g * GR:(g + 1) * GR, :] = o.astype(BF16)

    def region(k, f):
        pl.when(zsm[k % 64] == 0)(f)

    P = functools.partial

    wq_a, wq_b = _Copies(wqkv_copy.cs[:8]), _Copies(wqkv_copy.cs[8:])

    def x_dma(j):
        with _scope("waitX%d" % j):
            sk_copy(j + 1).wait()
            if j == 2:
                wq_a.wait()
            if j == 3:
                wq_b.wait()
        if j == 0:
            kv_copy(2).start()
            sk_copy(2).start()
        if j == 1:
            kv_copy(3).start()
            sk_copy(3).start()
            wq_a.start()
        if j == 2:
            kv_copy(4).start()
            sk_copy(4).start()
            wq_b.start()
        if j == 3:
            q_copy(0).start()
            wo_copy.start()
            q_copy(1).start()

    def block_x(j):
        s = j % 2
        with _scope("X%d" % j):
            aconv(s)
            if j >= 1:
                idft(j - 1, 1 - s)
                dft_u(j + 1, 1 - s)
            dft_k(j + 1, 1 - s)
            if j == 2:
                w_transpose(range(0, 8))
            if j == 3:
                w_transpose(range(8, 15))
        if j == 0:
            with _scope("waitK1"):
                kv_copy(1).wait()
            with _scope("Y0"):
                kvprep(1)
                dft_u(1, 1)
        if j + 2 < ND:
            with _scope("waitK%d" % (j + 2)):
                kv_copy(j + 2).wait()
            with _scope("KV%d" % (j + 2)):
                kvprep(j + 2)

    def body_a(j, carry):
        return carry

    def block_b(b, s):
        if ONLY == '':
            q_copy(b).wait()

        @pl.when(b >= 4)
        def _():
            out_copy(b - 4, s).wait()
        with _scope("B"):
            halo(1 - s)
            mt = qkv(b, s)
            if EPI == 'paced':
                epilogue(b - 2, s, mt)
            elif EPI == 'free':
                epilogue(b - 2, s)
            elif EPI == 'late':
                epilogue(b - 2, s, [mt[14]] * 15)
            if EPI != 'after':
                out_copy(b - 2, s).start()
            if E('NOATT', '0') != '1':
                attention(b - 1, 1 - s, mt)
            if E('NOGATE', '0') != '1':
                gate(b - 1, 1 - s, mt if GATEP else None)
            if EPI == 'after':
                ot = outproj(1 - s)
                epilogue(b - 2, s, [ot[(g * 5) // 15] for g in range(15)])
                out_copy(b - 2, s).start()
            else:
                outproj(1 - s)

    def body_b(b, carry):
        if E('ONEPAR', '0') == '1':
            block_b(b, 0)
            return carry
        for s in range(2):
            pl.when(b % 2 == s)(functools.partial(block_b, b, s))
        return carry

    if ONLY != 'B':
        nb = NA // NCH
        for ch in range(NCH):
            with _scope("wait0"):
                first_copy(ch).wait()
            if ch == 1:
                sk_copy(1).start()
            if ch == NCH - 1:
                kv_copy(1).start()
            with _scope("pro"):
                blks = range(ch * nb, (ch + 1) * nb)
                kvprep(0, blks)
                dft_k(0, 0, blks)
                dft_u(0, 0, blks)

        for j in range(ND - 1):
            x_dma(j)
            region(2 * j, P(block_x, j))

    if ONLY == '':
        q_copy(0).wait()
        wo_copy.wait()
        for b in range(2, NT):
            q_copy(b).start()

        def block_alast():
            with _scope("Alast"):
                w_permute()
                wo_permute()
                if Q0 == 3:
                    idft(ND - 2, (ND - 2) % 2)
                    mt = qkv(0, 0, True)
                    wts = [sum(a + 1 for a in range(a0, a0 + LAB)) for a0 in range(0, NA, LAB)]
                    tot = 136 * 16
                    bt, cum = [], 0
                    for p in range(16):
                        row = []
                        for bi in range(len(wts)):
                            k = (cum * LN * len(mt)) // (tot * 16) - LOFF
                            row.append(mt[min(k, len(mt) - 1)] if k >= 0 else None)
                            cum += wts[bi]
                        bt.append(row)
                    aconv((ND - 1) % 2, range(16), btoks=bt, ab=LAB)
                elif Q0 == 2:
                    idft(ND - 2, (ND - 2) % 2)
                    mt = qkv(0, 0)
                    toks = [None] + [mt[min(14, ((p - 1) * LN) // 16)] for p in range(1, 16)]
                    aconv((ND - 1) % 2, range(16), toks, tz=False)
                else:
                    aconv((ND - 1) % 2)
                    idft(ND - 2, (ND - 2) % 2)
                    if Q0:
                        qkv(0, 0)

        region(10, block_alast)

        def block_b1():
            q_copy(1).wait()
            with _scope("B1"):
                if not Q0:
                    qkv(0, 0)
                idft(ND - 1, (ND - 1) % 2)
                halo(0)
                mt = qkv(1, 1)
                attention(0, 0, mt)
                gate(0, 0, mt)
                outproj(0)

        region(11, block_b1)

    if ONLY != 'A':
        jax.lax.fori_loop(2, NT, body_b, 0)

    if ONLY == '':
        with _scope("fin1"):
            out_copy(NT - 4, 0).wait()
            epilogue(NT - 2, 0)
            out_copy(NT - 2, 0).start()
            attention(NT - 1, 1)
            gate(NT - 1, 1)
            outproj(1)
        with _scope("fin2"):
            out_copy(NT - 3, 1).wait()
            epilogue(NT - 1, 1)
            out_copy(NT - 1, 1).start()
        with _scope("fin3"):
            out_copy(NT - 2, 0).wait()
            out_copy(NT - 1, 1).wait()
    elif ONLY == 'B':
        out_copy(NT - 4, 0).wait()
        out_copy(NT - 3, 0 if E('ONEPAR', '0') == '1' else 1).wait()
    else:
        for b in range(2):
            q_copy(b).wait()
        wo_copy.wait()


@jax.jit
def pallas_gated_mix__ssm_conv_h3__sliding_local_dilated__prompt_kernel(A_q, A_k, A_v, A_shift_k, A_ssm_k, A_ssm_D, B_x, B_wqkv, B_wo, gate_w):
    fwd, inv, eye = _dft_constants()
    hbm = pl.BlockSpec(memory_space=pl.ANY)
    vm = pl.BlockSpec(memory_space=pltpu.VMEM)
    two = lambda shape, dt: [pltpu.VMEM(shape, dt), pltpu.VMEM(shape, dt)]
    return pl.pallas_call(
        _kernel,
        out_shape=jax.ShapeDtypeStruct((1, S, D), BF16),
        in_specs=[hbm] * 12,
        out_specs=hbm,
        scratch_shapes=[
            pltpu.VMEM((4, D), BF16),
            pltpu.VMEM((D,), BF16),
            pltpu.VMEM((D,), BF16),
            pltpu.VMEM((384, 128), BF16),
            pltpu.VMEM((128, 256), BF16),
            pltpu.VMEM((128, 128), BF16),
            pltpu.VMEM((ND, 2 * KH + S, 128), BF16),
            pltpu.VMEM((ND, S, 128), BF16),
            pltpu.VMEM((ND, NA, 128, L), BF16),
            pltpu.VMEM((ND, S, 128), BF16),
            pltpu.VMEM((15, D, 128), BF16),
            pltpu.VMEM((ND, D, 128), BF16),
            pltpu.VMEM((ND, 6, 8, 128), F32),
            pltpu.VMEM((8, 128), F32),
            pltpu.SMEM((64,), jnp.int32),
            pltpu.VMEM((192, 128), U32),
            pltpu.VMEM((64, 256), U32),
            pltpu.VMEM((64, 128), U32),
            pltpu.VMEM((64, 128), U32),
            pltpu.VMEM((ND, S // 2, 128), U32),
            *two((3, NA, 128, 128), F32),
            *two((NA, 256, 128), F32),
            *two((NA, 128, 128), U32),
            *two((384, 128), F32),
            pltpu.VMEM((2, ND, S, 128), F32),
            pltpu.VMEM((ND, 3 * D, 128), F32),
            pltpu.VMEM((3 * D // 2, D), U32),
            pltpu.VMEM((D // 2, 3 * D), U32),
            pltpu.VMEM((ND, D, 128), F32),
            pltpu.VMEM((D // 2, D), U32),
            *two((ND, T, 128), F32),
            *two((ND, HALO + T, 128), F32),
            *two((ND, HALO + T, 128), F32),
            pltpu.VMEM((8, T, 128), F32),
            pltpu.VMEM((8, T, 128), F32),
            pltpu.VMEM((8, T, 128), F32),
            pltpu.VMEM((T // 2, D), U32),
            *two((T, D), F32),
            *two((ND, T, 128), BF16),
            pltpu.VMEM((2, T // 2, 128), U32),
            *two((2, T, 128), F32),
            pltpu.SemaphoreType.DMA((3 * ND,)),
            pltpu.SemaphoreType.DMA((NT,)),
            pltpu.SemaphoreType.DMA((2,)),
            pltpu.SemaphoreType.DMA((2,)),
            pltpu.SemaphoreType.DMA((6,)),
            pltpu.SemaphoreType.DMA((NCH,)),
        ],
        compiler_params=pltpu.CompilerParams(vmem_limit_bytes=100 * 2 ** 20),
    )(A_q, A_k, A_v, A_shift_k.T, A_ssm_k, A_ssm_D, B_wqkv, B_wo, gate_w,
      jnp.asarray(fwd, BF16), jnp.asarray(inv, BF16), jnp.asarray(eye, BF16))
```

```python
import contextlib
import functools
import numpy as np
import jax
import jax.numpy as jnp
from jax.experimental import pallas as pl
from jax.experimental.pallas import tpu as pltpu


def E(key, default):
    return default


ONLY = E('ONLY', '')
SCOPES = int(E('SCOPES', '0'))
AN, EN, GN, PACE = int(E('AN', '13')), int(E('EN', '14')), int(E('GN', '10')), int(E('PACE', '4'))
D1, D2, D3 = int(E('D1', '2')), int(E('D2', '4')), int(E('D3', '5'))
DYNZ = int(E('DYNZ', '0'))
AB = int(E('AB', '4'))
ATOK = int(E('ATOK', '0'))
AOFF = int(E('AOFF', '1'))
ARATE = int(E('ARATE', '100'))
AORD = E('AORD', 'cf')
FR = int(E('FR', '100'))
USM = int(E('USM', '0'))
MERGE = int(E('MERGE', '0'))
KVFIRST = int(E('KVFIRST', '1'))
KSPLIT = int(E('KSPLIT', '8'))

WT_AT = int(E('WT_AT', '2'))
LN = int(E('LN', '15'))
EPI = E('EPI', 'late')
GATEP = int(E('GATEP', '1'))
NNW = int(E('NNW', '0'))
LOFF = int(E('LOFF', '0'))
LAB = int(E('LAB', '2'))
KVPOS = E('KVPOS', 'post')
TFIRST = int(E('TFIRST', '0'))
KVT = [int(x) for x in E('KVT', '-1,-1,-1').split(',')]
GATE = E('GATE', 'mem')
BIG = int(E('BIG', '0'))
KSPREAD = int(E('KSPREAD', '1'))
PAIR = int(E('PAIR', '0'))
NOB = 4
FSPLIT = int(E('FSPLIT', '4'))
PERM_EARLY = int(E('PERM_EARLY', '1'))
WQ0 = int(E('WQ0', '4'))
WLATE = int(E('WLATE', '1'))
NCH = int(E('NCH', '4'))
Q0 = int(E('Q0', '1'))
S, D = 2048, 640
ND = 5
L = 128
NA = S // L
T = 256
NT = S // T
H, DH = 32, 20
HALO = 16
KH = 8
GR = 16
GE = int(E('GE', '8'))
NG = T // GR
LOG2E = 1.4426950408889634
QSCALE = float(DH ** -0.5) * LOG2E
MASKED = -1e9 * LOG2E
F32, BF16, U32 = jnp.float32, jnp.bfloat16, jnp.uint32


def _scope(name):
    return jax.named_scope(name) if SCOPES else contextlib.nullcontext()


def _dft_constants():
    forder = np.concatenate([np.arange(0, 128, 2), np.arange(1, 128, 2)])
    th = np.pi * (2 * forder + 1) / 256.0
    b = np.arange(128)
    fre, fim = np.cos(np.outer(th, b)), -np.sin(np.outer(th, b))
    fwd = np.concatenate([fre, fim, fre + fim], 0)
    gre = np.cos(np.outer(b, th)) / 128
    gim = -np.sin(np.outer(b, th)) / 128
    inv = np.stack([gre, gim], -1).reshape(128, 256)
    return fwd.astype(np.float32), inv.astype(np.float32), np.eye(128, dtype=np.float32)


def _bf(x):
    return pltpu.bitcast(x, BF16)


def _u32(x):
    return pltpu.bitcast(x, U32)


def _bmul(x, t8):
    return (x.reshape(-1, 8, 128) * t8).reshape(x.shape)


def _badd(x, t8):
    return (x.reshape(-1, 8, 128) + t8).reshape(x.shape)


def _dot(a, b):
    return jnp.dot(a, b, preferred_element_type=F32)


def _dot_nt(a, b):
    return jax.lax.dot_general(a, b, (((1,), (1,)), ((), ())), preferred_element_type=F32)


class _Copies:
    def __init__(self, cs):
        self.cs = list(cs)

    def start(self):
        for c in self.cs:
            c.start()

    def wait(self):
        for c in self.cs:
            c.wait()


def _kernel(q_hbm, k_hbm, v_hbm, shk_hbm, sk_hbm, dvec_hbm, wqkv_hbm, wo_hbm, gw_hbm,
            fwd_hbm, inv_hbm, eye_hbm,
            out_hbm,
            shk_ref, dvec_ref, gw_ref, fwd_ref, inv_ref, eye_ref,
            kbuf, vbuf, skbuf, qbuf, wqkv_v, wo_v, par, zvec, zsm, fwdp, invp, onesp, eyep,
            kvp, ubuf0, ubuf1, kpbuf0, kpbuf1, ybuf0, ybuf1, kst0, kst1, y2, wt, wtp, wnn, wof, wop,
            qp0, qp1, kp0, kp1, vp0, vp1, pbuf, sbuf, lbuf, op, bres0, bres1, obuf, gsp, glog0, glog1,
            sem_a, sem_q, sem_w, sem_o, sem_s, sem_f):
    ubuf, kpbuf, ybuf, kstb = (ubuf0, ubuf1), (kpbuf0, kpbuf1), (ybuf0, ybuf1), (kst0, kst1)
    qp, kp, vp = (qp0, qp1), (kp0, kp1), (vp0, vp1)
    bres, glog = (bres0, bres1), (glog0, glog1)
    skw, qw, wqkvw = skbuf.bitcast(U32), qbuf.bitcast(U32), wqkv_v.bitcast(U32)
    kw, vw = kbuf.bitcast(U32), vbuf.bitcast(U32)

    def kv_copy(j):
        return _Copies(
            [pltpu.make_async_copy(k_hbm.at[0, :, pl.ds(j * 128, 128)], kbuf.at[j, pl.ds(2 * KH, S)], sem_a.at[3 * j]),
             pltpu.make_async_copy(v_hbm.at[0, :, pl.ds(j * 128, 128)], vbuf.at[j], sem_a.at[3 * j + 1])])

    def sk_copy(j):
        return _Copies(pltpu.make_async_copy(sk_hbm.at[pl.ds(j * 128, 128), pl.ds(m * L, L)], skbuf.at[j, m],
                                             sem_a.at[3 * j + 2]) for m in range(NA))

    def slab_copy(j):
        return _Copies(kv_copy(j).cs + sk_copy(j).cs)

    def first_copy(ch):
        rows = pl.ds(ch * (S // NCH), S // NCH)
        ms = range(ch * (NA // NCH), (ch + 1) * (NA // NCH))
        return _Copies(
            [pltpu.make_async_copy(k_hbm.at[0, rows, pl.ds(0, 128)],
                                   kbuf.at[0, pl.ds(2 * KH + ch * (S // NCH), S // NCH)], sem_f.at[ch]),
             pltpu.make_async_copy(v_hbm.at[0, rows, pl.ds(0, 128)], vbuf.at[0, rows], sem_f.at[ch])]
            + [pltpu.make_async_copy(sk_hbm.at[pl.ds(0, 128), pl.ds(m * L, L)], skbuf.at[0, m], sem_f.at[ch])
               for m in ms])

    small_copy = _Copies(pltpu.make_async_copy(a, b, sem_s.at[i]) for i, (a, b) in enumerate(
        [(shk_hbm, shk_ref), (dvec_hbm, dvec_ref), (gw_hbm, gw_ref), (fwd_hbm, fwd_ref), (inv_hbm, inv_ref),
         (eye_hbm, eye_ref)]))
    def q_copy(b):
        rows = pl.ds(b * T, T)
        return _Copies(pltpu.make_async_copy(q_hbm.at[0, rows, pl.ds(j * 128, 128)], qbuf.at[j, rows], sem_q.at[b])
                       for j in range(ND))

    wqkv_copy = _Copies(pltpu.make_async_copy(wqkv_hbm.at[:, pl.ds(n * 128, 128)], wqkv_v.at[n], sem_w.at[0])
                        for n in range(15))
    wo_copy = _Copies(pltpu.make_async_copy(wo_hbm.at[:, pl.ds(n * 128, 128)], wo_v.at[n], sem_w.at[1])
                      for n in range(ND))

    def out_copy(b, r0=0, n=T):
        return _Copies(pltpu.make_async_copy(obuf.at[b % NOB, j, pl.ds(r0, n)],
                                             out_hbm.at[0, pl.ds(b * T + r0, n), pl.ds(j * 128, 128)],
                                             sem_o.at[b % NOB]) for j in range(ND))

    with _scope("s_issue"):
        small_copy.start()
        if ONLY != 'B':
            first_copy(0).start()
    with _scope("s_wait"):
        small_copy.wait()
    if ONLY != 'B':
        for ch in range(1, NCH):
            first_copy(ch).start()

    with _scope("s_setup"):
        taps = shk_ref[...].astype(F32)
        dv = dvec_ref[...].astype(F32).reshape(1, D)
        gw = gw_ref[...].astype(F32).reshape(1, D)
        for j in range(ND):
            for i in range(4):
                par[j, i] = jnp.broadcast_to(taps[i:i + 1, j * 128:(j + 1) * 128], (8, 128))
            par[j, 4] = jnp.broadcast_to(dv[:, j * 128:(j + 1) * 128], (8, 128))
            par[j, 5] = jnp.broadcast_to(gw[:, j * 128:(j + 1) * 128], (8, 128))
        zvec[...] = jnp.zeros((8, 128), F32)
        for i in range(64):
            zsm[i] = 0
        fwdp[...] = _u32(fwd_ref[...])
        invp[...] = _u32(inv_ref[...])
        eyep[...] = _u32(eye_ref[...])
        onesp[...] = _u32(jnp.ones((128, 128), BF16))
        for j in range(ND):
            kw[j, 0:KH, :] = jnp.zeros((KH, 128), U32)
        for j in range(ND):
            kp0[j, 0:HALO, :] = jnp.zeros((HALO, 128), F32)
            vp0[j, 0:HALO, :] = jnp.zeros((HALO, 128), F32)

    def fresh(i):
        return pl.multiple_of(zsm[i] * 8, 8)

    def gated(tok):
        i = tok[0, 0].astype(jnp.int32)
        return pl.multiple_of(jnp.minimum(jnp.maximum(i, zsm[62]), zsm[63]) * 8, 8)

    def kvprep(j, blks=range(NA), tok=None):
        t = [par[j, i] if tok is None else par[j, i] + tok * zvec[...] for i in range(4)]
        even = lambda w: pltpu.bitcast(w << 16, F32)
        odd = lambda w: pltpu.bitcast(w & jnp.uint32(0xFFFF0000), F32)
        for c in blks:
            for q in range(L // 32):
                r = c * (L // 2) + q * 16
                w0 = kw[j, KH + r:KH + r + 16, :]
                w1 = kw[j, KH + r - 1:KH + r + 15, :]
                w2 = kw[j, KH + r - 2:KH + r + 14, :]
                e0, o0, e1, o1, o2 = even(w0), odd(w0), even(w1), odd(w1), odd(w2)
                ks_e = _bmul(e0, t[0]) + _bmul(o1, t[1]) + _bmul(e1, t[2]) + _bmul(o2, t[3])
                ks_o = _bmul(o0, t[0]) + _bmul(e0, t[1]) + _bmul(o1, t[2]) + _bmul(e1, t[3])
                wv = vw[j, r:r + 16, :]
                kvp[j, r:r + 16, :] = pltpu.pack_elementwise([ks_e * even(wv), ks_o * odd(wv)], packed_dtype=BF16)

    def dft_u(j, s, cs=range(NA)):
        cs = list(cs)
        if BIG:
            f = _bf(fwdp[pl.ds(fresh(16), 192 if USM else 128), :])
            rhs = jnp.concatenate([_bf(kvp[j, c * 64:(c + 1) * 64, :]) for c in cs], axis=1)
            r = _dot(f, rhs)
            for n, c in enumerate(cs):
                for i in range(3 if USM else 2):
                    ubuf[s][i, c] = r[i * 128:(i + 1) * 128, n * 128:(n + 1) * 128]
            return [r[0:8, n * 128:(n + 1) * 128] for n in range(len(cs))]
        toks = []
        for c in cs:
            f = _bf(fwdp[pl.ds(fresh(16 + c), 192 if USM else 128), :])
            r = _dot(f, _bf(kvp[j, c * 64:(c + 1) * 64, :]))
            for i in range(3 if USM else 2):
                ubuf[s][i, c] = r[i * 128:(i + 1) * 128]
            toks.append(r[0:8])
        return toks

    def dft_k(j, s, ms=range(NA)):
        ms = list(ms)
        if BIG:
            f = _bf(fwdp[pl.ds(fresh(32), 128), :])
            rhs = jnp.concatenate([_bf(skw[j, m]) for m in ms], axis=0)
            r = _dot_nt(f, rhs)
            for n, m in enumerate(ms):
                kpbuf[s][m] = r[:, n * 128:(n + 1) * 128]
            return [r[0:8, n * 128:(n + 1) * 128] for n in range(len(ms))]
        toks = []
        for m in ms:
            f = _bf(fwdp[pl.ds(fresh(32 + m), 128), :])
            r = _dot_nt(f, _bf(skw[j, m]))
            kpbuf[s][m] = r
            toks.append(r[0:8])
        return toks

    def aconv(s, plist=range(16), toks=None, mode=None, tz=True, btoks=None, ab=AB):
        ub, kb, yb = ubuf[s], kpbuf[s], ybuf[s]

        def kprep(p, ms=range(NA)):
            r, im = p * 8, 128 + p * 8
            kst = kstb[p % 2]
            for m in ms:
                pr, pi = kb[m, r:r + 8, :], kb[m, im:im + 8, :]
                if m == 0:
                    kr, ki = pr, pi
                    if toks is not None and toks[p] is not None:
                        kr = kr + (toks[p] * zvec[...] if tz else toks[p])
                elif p < 8:
                    kr, ki = pr - kb[m - 1, im:im + 8, :], pi + kb[m - 1, r:r + 8, :]
                else:
                    kr, ki = pr + kb[m - 1, im:im + 8, :], pi - kb[m - 1, r:r + 8, :]
                kst[m * 8:m * 8 + 8, :] = kr
                kst[128 + m * 8:128 + m * 8 + 8, :] = kr + ki
                kst[256 + m * 8:256 + m * 8 + 8, :] = ki - kr

        def macs(p, nxt=None):
            r = p * 8
            kst = kstb[p % 2]
            nb = NA // ab
            for bi, a0 in enumerate(range(0, NA, ab)):
                z = fresh(bi)
                if btoks is not None and btoks[p][bi] is not None:
                    z = gated(btoks[p][bi])
                acc = [[None] * ab for _ in range(3)]
                ncs = a0 + ab
                todo = []
                if nxt is not None and KSPREAD:
                    if bi >= nb - 2:
                        half = bi - (nb - 2)
                        todo = list(range(half * 8, half * 8 + 8))
                for c in range(ncs):
                    if USM:
                        uu = [ub[i, c, pl.ds(z + r, 8), :] for i in (2, 1, 0)]
                    else:
                        u_i, u_r = ub[1, c, pl.ds(z + r, 8), :], ub[0, c, pl.ds(z + r, 8), :]
                        uu = [u_r + u_i, u_i, u_r]
                    for i in range(ab):
                        m = a0 + i - c
                        if m < 0:
                            continue
                        for t in range(3):
                            x = kst[pl.ds(z + t * 128 + m * 8, 8), :] * uu[t]
                            acc[t][i] = x if acc[t][i] is None else acc[t][i] + x
                    if todo and c < 8:
                        kprep(nxt, [todo[c]])
                for i in range(ab):
                    yb[a0 + i, r:r + 8, :] = pltpu.pack_elementwise(
                        [acc[0][i] - acc[1][i], acc[0][i] + acc[2][i]], packed_dtype=BF16)

        plist = list(plist)
        kprep(plist[0])
        for n, p in enumerate(plist):
            nxt = plist[n + 1] if n + 1 < len(plist) else None
            if nxt is not None and not KSPREAD:
                kprep(nxt)
            macs(p, nxt)

    def idft(j, s, as_=range(NA)):
        as_ = list(as_)
        if BIG:
            z = fresh(48)
            toks = []
            for h in range(2):
                g = _bf(invp[pl.ds(z, 64), h * 128:(h + 1) * 128])
                rhs = jnp.concatenate([_bf(ybuf[s][a, h * 64:(h + 1) * 64, :]) for a in as_], axis=1)
                r = _dot(g, rhs)
                for n, a in enumerate(as_):
                    y2[h, j, a * L:(a + 1) * L, :] = r[:, n * 128:(n + 1) * 128]
                toks += [r[0:8, n * 128:(n + 1) * 128] for n in range(len(as_))]
            return toks
        toks = []
        for a in as_:
            z = fresh(48 + a)
            g0 = _bf(invp[pl.ds(z, 64), 0:128])
            g1 = _bf(invp[pl.ds(z, 64), 128:256])
            r0 = _dot(g0, _bf(ybuf[s][a, 0:64, :]))
            r1 = _dot(g1, _bf(ybuf[s][a, 64:128, :]))
            y2[0, j, a * L:(a + 1) * L, :] = r0
            y2[1, j, a * L:(a + 1) * L, :] = r1
            toks.append(r1[0:8])
        return toks

    def w_transpose(ns=range(15)):
        toks = []
        for n in ns:
            eye = _bf(eyep[pl.ds(fresh(n), 64), :])
            r = _dot_nt(eye, _bf(wqkvw[n]))
            for kt in range(ND):
                wt[kt, n * 128:(n + 1) * 128, :] = r[:, kt * 128:(kt + 1) * 128]
            toks.append(r[0:8, 0:128])
        return toks

    def w_permute(parts=range(3)):
        for p in parts:
            for dh in range(DH):
                for kt in range(ND):
                    rows = wt[kt, pl.ds(p * D + dh, H, stride=DH), :]
                    r0 = (p * D + dh * H) // 2
                    wtp[r0:r0 + H // 2, kt * 128:(kt + 1) * 128] = _u32(rows.astype(BF16))

    def wo_permute():
        for j in range(ND):
            wof[j] = wo_v[j].astype(F32)
        for dh in range(DH):
            for j in range(ND):
                rows = wof[j, pl.ds(dh, H, stride=DH), :]
                r0 = dh * H // 2
                wop[r0:r0 + H // 2, j * 128:(j + 1) * 128] = _u32(rows.astype(BF16))

    def qkv(b, s, fine=False):
        r0 = pl.multiple_of(b * (T // 2), T // 2)
        x = jnp.concatenate([_bf(qw[j, pl.ds(r0, T // 2), :]) for j in range(ND)], axis=1)
        r = _dot(x, _bf(wnn[...])) if NNW else _dot_nt(x, _bf(wtp[...]))
        for j in range(ND):
            qp[s][j] = r[:, j * 128:(j + 1) * 128]
            kp[s][j, HALO:HALO + T, :] = r[:, D + j * 128:D + (j + 1) * 128]
            vp[s][j, HALO:HALO + T, :] = r[:, 2 * D + j * 128:2 * D + (j + 1) * 128]
        if fine:
            return [r[64 * i:64 * i + 8, n * 128:(n + 1) * 128] * zvec[...] for n in range(15) for i in range(4)]
        return [r[0:8, n * 128:(n + 1) * 128] * zvec[...] for n in range(15)]

    def gate(b, s, mt=None):
        r0 = pl.multiple_of(b * T, T)
        for g in range(NG):
            sm = None if mt is None else jnp.concatenate([mt[(g * GN) // NG]] * (GR // 8), axis=0)
            for j in range(ND):
                t = _bmul(qbuf[j, pl.ds(r0 + g * GR, GR), :].astype(F32), par[j, 5])
                sm = t if sm is None else sm + t
            hi = sm.astype(BF16)
            lo = (sm - hi.astype(F32)).astype(BF16)
            gsp[0, g * GR // 2:(g + 1) * GR // 2, :] = _u32(hi)
            gsp[1, g * GR // 2:(g + 1) * GR // 2, :] = _u32(lo)
        ones = _bf(onesp[...])
        glog[s][0] = _dot(_bf(gsp[0]), ones)
        glog[s][1] = _dot(_bf(gsp[1]), ones)

    def halo(s):
        for j in range(ND):
            kp[1 - s][j, 0:HALO, :] = kp[s][j, T:T + HALO, :]
            vp[1 - s][j, 0:HALO, :] = vp[s][j, T:T + HALO, :]

    def softmax_pv(vv, row):
        lg = [lbuf[w, row:row + GR, :] for w in range(8)]
        m = lg[0]
        for w in range(1, 8):
            m = jnp.maximum(m, lg[w])
        es = [(l - m) if E('NOEXP', '0') == '1' else jnp.exp2(l - m) for l in lg]
        sm = es[0]
        for w in range(1, 8):
            sm = sm + es[w]
        inv = 1.0 / sm
        for j in range(ND):
            acc = None
            for w in range(8):
                o = row + HALO - 2 * w
                t = es[w] * vv[j, o:o + GR, :]
                acc = t if acc is None else acc + t
            res = acc * inv
            op[row // 2:(row + GR) // 2, j * 128:(j + 1) * 128] = _u32(res.astype(BF16))
        return res[0:8]

    def qk(qq, kk, row, tok):
        if tok is None:
            q = [qq[j, row:row + GE, :] * QSCALE for j in range(ND)]
        else:
            sc = tok + QSCALE
            q = [_bmul(qq[j, row:row + GE, :], sc) for j in range(ND)]
        out = []
        for w in range(8):
            p = None
            o = row + HALO - 2 * w
            for j in range(ND):
                t = q[j] * kk[j, o:o + GE, :]
                p = t if p is None else p + t
            out.append(p)
        return out

    def attention(b, s, mt=None):
        qq, kk, vv = qp[s], kp[s], vp[s]
        n1 = T // GE
        per = GR // GE
        r1, r2, done = {}, {}, {}
        for g in range(n1 + D3 + per):
            if g < n1:
                row = g * GE
                tok = None
                if mt is not None:
                    tok = mt[(g * AN) // n1]
                    prev = done.get(row // GR - PACE) if PACE else None
                    if prev is not None:
                        tok = tok + prev * zvec[...]
                r1[g] = []
                for w, p in enumerate(qk(qq, kk, row, tok)):
                    pbuf[w, row:row + GE, :] = p
                    r1[g].append(p * 2.0 if E('NOROLL', '0') == '1' else pltpu.roll(p, 64, 1))
            gg = g - D1
            if 0 <= gg < n1:
                row = gg * GE
                r2[gg] = []
                for w, r in enumerate(r1.pop(gg)):
                    sm = pbuf[w, row:row + GE, :] + r
                    sbuf[w, row:row + GE, :] = sm
                    r2[gg].append(sm * 2.0 if E('NOROLL', '0') == '1' else pltpu.roll(sm, 32, 1))
            gg = g - D2
            if 0 <= gg < n1:
                row = gg * GE
                for w, r in enumerate(r2.pop(gg)):
                    l = sbuf[w, row:row + GE, :] + r
                    if row < HALO and w > 0:
                        t = b * T + row + jax.lax.broadcasted_iota(jnp.int32, (GE, 128), 0)
                        l = jnp.where(t >= 2 * w, l, MASKED)
                    lbuf[w, row:row + GE, :] = l
            gg = g - D3
            if 0 <= gg < n1 and (gg + 1) % per == 0:
                row = (gg + 1 - per) * GE
                done[row // GR] = softmax_pv(vv, row)

    def outproj(s, r0=0, n=T):
        r = _dot(_bf(op[r0 // 2:(r0 + n) // 2, :]), _bf(wop[...]))
        bres[s][r0:r0 + n, :] = r
        return [r[0:8, k * 128:(k + 1) * 128] * zvec[...] for k in range(ND)]

    def epilogue(b, s, mt=None, gs=range(NG)):
        r0 = pl.multiple_of(b * T, T)
        for g in gs:
            row = r0 + g * GR
            rowh = pl.multiple_of(b * (T // 2), T // 2) + g * (GR // 2)
            gl = glog[s][0, g * GR:(g + 1) * GR, :] + glog[s][1, g * GR:(g + 1) * GR, :]
            if mt is not None:
                gl = _badd(gl, mt[(g * EN) // NG])
            gt = jax.nn.sigmoid(gl)
            for j in range(ND):
                q = qbuf[j, pl.ds(row, GR), :].astype(F32)
                kv = _bf(kvp[j, pl.ds(rowh, GR // 2), :]).astype(F32)
                z = y2[0, j, pl.ds(row, GR), :] + y2[1, j, pl.ds(row, GR), :] + _bmul(kv, par[j, 4])
                bb = bres[s][g * GR:(g + 1) * GR, j * 128:(j + 1) * 128]
                o = bb + gt * (q * z - bb)
                obuf[b % NOB, j, g * GR:(g + 1) * GR, :] = o.astype(BF16)

    def region(k, f):
        pl.when(zsm[k % 64] == 0)(f)

    P = functools.partial

    wq_0, wq_1, wq_b = _Copies(wqkv_copy.cs[:WQ0]), _Copies(wqkv_copy.cs[WQ0:8]), _Copies(wqkv_copy.cs[8:])
    wq_a = _Copies(wqkv_copy.cs[:8])

    def x_dma(j):
        with _scope("waitX%d" % j):
            sk_copy(j + 1).wait()
            if j >= 1:
                kv_copy(j + 1).wait()
            if j == 2 and not WLATE:
                wq_a.wait()
            if j == 3 and not WLATE:
                wq_b.wait()
        if j == 0:
            kv_copy(2).start()
            sk_copy(2).start()
            if not WLATE:
                wq_0.start()
        if j == 1:
            kv_copy(3).start()
            sk_copy(3).start()
            if not WLATE:
                wq_1.start()
        if j == 2:
            kv_copy(4).start()
            sk_copy(4).start()
            (wq_0 if WLATE else wq_b).start()
        if j == 3 and WLATE:
            _Copies(wqkv_copy.cs[WQ0:]).start()
        if j == 3:
            q_copy(0).start()
            if not WLATE:
                wo_copy.start()
                q_copy(1).start()

    def block_x(j):
        s = j % 2
        with _scope("X%d" % j):
            if j >= 1:
                kvprep(j + 1)
            aconv(s)
            if j >= 1:
                idft(j - 1, 1 - s)
            dft_k(j + 1, 1 - s)
            if j == 2 and not WLATE:
                w_transpose(range(0, 8))
            if j == 3 and not WLATE:
                w_transpose(range(8, 15))
                if PERM_EARLY:
                    w_permute([0])
            if j >= 1:
                dft_u(j + 1, 1 - s)
        if j == 0:
            with _scope("waitK1"):
                kv_copy(1).wait()
            with _scope("Y0"):
                kvprep(1)
                dft_u(1, 1)

    def body_a(j, carry):
        return carry

    def b_dma(b, s):
        if ONLY == '':
            q_copy(b).wait()

        @pl.when(b - 2 >= NOB)
        def _():
            out_copy(b - 2 - NOB).wait()

    def epilogue_wait(t):
        if t >= NOB:
            out_copy(t - NOB).wait()

    def block_b(b, s, dma=True):
        if dma:
            b_dma(b, s)
        with _scope("B"):
            halo(1 - s)
            mt = qkv(b, s)
            if EPI == 'paced':
                epilogue(b - 2, s, mt)
            elif EPI == 'free':
                epilogue(b - 2, s)
            elif EPI == 'late':
                epilogue(b - 2, s, [mt[14]] * 15)
            if EPI != 'after':
                out_copy(b - 2).start()
            if E('NOATT', '0') != '1':
                attention(b - 1, 1 - s, mt)
            if E('NOGATE', '0') != '1':
                gate(b - 1, 1 - s, mt if GATEP else None)
            if EPI == 'after':
                ot = outproj(1 - s)
                epilogue(b - 2, s, [ot[(g * 5) // 15] for g in range(15)])
                out_copy(b - 2).start()
            else:
                outproj(1 - s)

    def body_b2(i, carry):
        b = 2 * i
        if ONLY == '':
            q_copy(b).wait()
            q_copy(b + 1).wait()

        @pl.when(b - 2 >= NOB)
        def _():
            out_copy(b - 2 - NOB).wait()
            out_copy(b - 1 - NOB).wait()
        block_b(b, 0, False)
        block_b(b + 1, 1, False)
        return carry

    def body_b(b, carry):
        if E('ONEPAR', '0') == '1':
            block_b(b, 0)
            return carry
        for s in range(2):
            pl.when(b % 2 == s)(functools.partial(block_b, b, s))
        return carry

    if ONLY != 'B':
        nb = NA // NCH
        for ch in range(NCH):
            with _scope("wait0"):
                first_copy(ch).wait()
            if ch == 1:
                sk_copy(1).start()
            if ch == NCH - 1:
                kv_copy(1).start()
            with _scope("pro"):
                blks = range(ch * nb, (ch + 1) * nb)
                kvprep(0, blks)
                dft_k(0, 0, blks)
                dft_u(0, 0, blks)

        for j in range(ND - 1):
            x_dma(j)
            region(2 * j, P(block_x, j))

    if ONLY == '':
        q_copy(0).wait()
        if WLATE:
            wqkv_copy.wait()
            wo_copy.start()
            q_copy(1).start()
        for b in range(2, NT):
            q_copy(b).start()

        def block_wlate():
            with _scope("Alast0"):
                aconv((ND - 1) % 2)
                idft(ND - 2, (ND - 2) % 2)
                w_transpose()

        if WLATE:
            region(12, block_wlate)

        def block_alast():
            if WLATE:
                with _scope("Alast"):
                    w_permute()
                    qkv(0, 0)
                return
            with _scope("Alast"):
                w_permute([1, 2] if PERM_EARLY else [0, 1, 2])
                if Q0 == 3:
                    idft(ND - 2, (ND - 2) % 2)
                    mt = qkv(0, 0, True)
                    wts = [sum(a + 1 for a in range(a0, a0 + LAB)) for a0 in range(0, NA, LAB)]
                    tot = 136 * 16
                    bt, cum = [], 0
                    for p in range(16):
                        row = []
                        for bi in range(len(wts)):
                            k = (cum * LN * len(mt)) // (tot * 16) - LOFF
                            row.append(mt[min(k, len(mt) - 1)] if k >= 0 else None)
                            cum += wts[bi]
                        bt.append(row)
                    aconv((ND - 1) % 2, range(16), btoks=bt, ab=LAB)
                elif Q0 == 2:
                    idft(ND - 2, (ND - 2) % 2)
                    mt = qkv(0, 0)
                    toks = [None] + [mt[min(14, ((p - 1) * LN) // 16)] for p in range(1, 16)]
                    aconv((ND - 1) % 2, range(16), toks, tz=False)
                else:
                    aconv((ND - 1) % 2)
                    idft(ND - 2, (ND - 2) % 2)
                    if Q0:
                        qkv(0, 0)

        region(10, block_alast)

        def block_b1():
            q_copy(1).wait()
            wo_copy.wait()
            with _scope("B1"):
                wo_permute()
                if not Q0:
                    qkv(0, 0)
                idft(ND - 1, (ND - 1) % 2)
                halo(0)
                mt = qkv(1, 1)
                attention(0, 0, mt)
                gate(0, 0, mt)
                outproj(0)

        region(11, block_b1)

    if ONLY != 'A':
        if PAIR:
            jax.lax.fori_loop(1, NT // 2, body_b2, 0)
        else:
            jax.lax.fori_loop(2, NT, body_b, 0)

    if ONLY == '':
        if FSPLIT:
            with _scope("fin1"):
                epilogue_wait(NT - 2)
                epilogue_wait(NT - 1)
                epilogue(NT - 2, 0)
                out_copy(NT - 2).start()
                gate(NT - 1, 1)
                attention(NT - 1, 1)
                nh = T // FSPLIT
                for h in range(FSPLIT):
                    outproj(1, h * nh, nh)
                for h in range(FSPLIT):
                    epilogue(NT - 1, 1, None, range(h * nh // GR, (h + 1) * nh // GR))
                    out_copy(NT - 1, h * nh, nh).start()
        else:
            with _scope("fin1"):
                epilogue_wait(NT - 2)
                epilogue(NT - 2, 0)
                out_copy(NT - 2).start()
                attention(NT - 1, 1)
                gate(NT - 1, 1)
                outproj(1)
            with _scope("fin2"):
                epilogue_wait(NT - 1)
                epilogue(NT - 1, 1)
                out_copy(NT - 1).start()
        with _scope("fin3"):
            for t in range(NT - NOB, NT):
                out_copy(t).wait()
    elif ONLY == 'B':
        for t in range(NT - 2 - NOB, NT - 2):
            out_copy(t).wait()
    else:
        for b in range(2):
            q_copy(b).wait()
        wo_copy.wait()


@jax.jit
def pallas_gated_mix__ssm_conv_h3__sliding_local_dilated__prompt_kernel(A_q, A_k, A_v, A_shift_k, A_ssm_k, A_ssm_D, B_x, B_wqkv, B_wo, gate_w):
    fwd, inv, eye = _dft_constants()
    hbm = pl.BlockSpec(memory_space=pl.ANY)
    vm = pl.BlockSpec(memory_space=pltpu.VMEM)
    two = lambda shape, dt: [pltpu.VMEM(shape, dt), pltpu.VMEM(shape, dt)]
    return pl.pallas_call(
        _kernel,
        out_shape=jax.ShapeDtypeStruct((1, S, D), BF16),
        in_specs=[hbm] * 12,
        out_specs=hbm,
        scratch_shapes=[
            pltpu.VMEM((4, D), BF16),
            pltpu.VMEM((D,), BF16),
            pltpu.VMEM((D,), BF16),
            pltpu.VMEM((384, 128), BF16),
            pltpu.VMEM((128, 256), BF16),
            pltpu.VMEM((128, 128), BF16),
            pltpu.VMEM((ND, 2 * KH + S, 128), BF16),
            pltpu.VMEM((ND, S, 128), BF16),
            pltpu.VMEM((ND, NA, 128, L), BF16),
            pltpu.VMEM((ND, S, 128), BF16),
            pltpu.VMEM((15, D, 128), BF16),
            pltpu.VMEM((ND, D, 128), BF16),
            pltpu.VMEM((ND, 6, 8, 128), F32),
            pltpu.VMEM((8, 128), F32),
            pltpu.SMEM((64,), jnp.int32),
            pltpu.VMEM((192, 128), U32),
            pltpu.VMEM((64, 256), U32),
            pltpu.VMEM((64, 128), U32),
            pltpu.VMEM((64, 128), U32),
            pltpu.VMEM((ND, S // 2, 128), U32),
            *two((3, NA, 128, 128), F32),
            *two((NA, 256, 128), F32),
            *two((NA, 128, 128), U32),
            *two((384, 128), F32),
            pltpu.VMEM((2, ND, S, 128), F32),
            pltpu.VMEM((ND, 3 * D, 128), F32),
            pltpu.VMEM((3 * D // 2, D), U32),
            pltpu.VMEM((D // 2, 3 * D), U32),
            pltpu.VMEM((ND, D, 128), F32),
            pltpu.VMEM((D // 2, D), U32),
            *two((ND, T, 128), F32),
            *two((ND, HALO + T, 128), F32),
            *two((ND, HALO + T, 128), F32),
            pltpu.VMEM((8, T, 128), F32),
            pltpu.VMEM((8, T, 128), F32),
            pltpu.VMEM((8, T, 128), F32),
            pltpu.VMEM((T // 2, D), U32),
            *two((T, D), F32),
            pltpu.VMEM((NOB, ND, T, 128), BF16),
            pltpu.VMEM((2, T // 2, 128), U32),
            *two((2, T, 128), F32),
            pltpu.SemaphoreType.DMA((3 * ND,)),
            pltpu.SemaphoreType.DMA((NT,)),
            pltpu.SemaphoreType.DMA((2,)),
            pltpu.SemaphoreType.DMA((NOB,)),
            pltpu.SemaphoreType.DMA((6,)),
            pltpu.SemaphoreType.DMA((NCH,)),
        ],
        compiler_params=pltpu.CompilerParams(vmem_limit_bytes=100 * 2 ** 20),
    )(A_q, A_k, A_v, A_shift_k.T, A_ssm_k, A_ssm_D, B_wqkv, B_wo, gate_w,
      jnp.asarray(fwd, BF16), jnp.asarray(inv, BF16), jnp.asarray(eye, BF16))
```

```python
import contextlib
import functools
import numpy as np
import jax
import jax.numpy as jnp
from jax.experimental import pallas as pl
from jax.experimental.pallas import tpu as pltpu


def E(key, default):
    return default


ONLY = E('ONLY', '')
SCOPES = int(E('SCOPES', '0'))
AN, EN, GN, PACE = int(E('AN', '13')), int(E('EN', '14')), int(E('GN', '10')), int(E('PACE', '4'))
D1, D2, D3 = int(E('D1', '2')), int(E('D2', '4')), int(E('D3', '5'))
DYNZ = int(E('DYNZ', '0'))
AB = int(E('AB', '4'))
ATOK = int(E('ATOK', '0'))
AOFF = int(E('AOFF', '1'))
ARATE = int(E('ARATE', '100'))
AORD = E('AORD', 'cf')
FR = int(E('FR', '100'))
USM = int(E('USM', '0'))
MERGE = int(E('MERGE', '0'))
KVFIRST = int(E('KVFIRST', '1'))
KSPLIT = int(E('KSPLIT', '8'))

WT_AT = int(E('WT_AT', '2'))
LN = int(E('LN', '15'))
EPI = E('EPI', 'late')
GATEP = int(E('GATEP', '1'))
NNW = int(E('NNW', '0'))
LOFF = int(E('LOFF', '0'))
LAB = int(E('LAB', '2'))
KVPOS = E('KVPOS', 'post')
TFIRST = int(E('TFIRST', '0'))
KVT = [int(x) for x in E('KVT', '-1,-1,-1').split(',')]
GATE = E('GATE', 'mem')
BIG = int(E('BIG', '0'))
KSPREAD = int(E('KSPREAD', '1'))
PAIR = int(E('PAIR', '0'))
NOB = 4
FSPLIT = int(E('FSPLIT', '4'))
PERM_EARLY = int(E('PERM_EARLY', '1'))
WQ0 = int(E('WQ0', '4'))
WLATE = int(E('WLATE', '1'))
KVFIRST2 = int(E('KVFIRST2', '0'))
NOLBUF = int(E('NOLBUF', '0'))
MSPLIT = int(E('MSPLIT', '1'))
AMERGE = int(E('AMERGE', '0'))
LASTB = int(E('LASTB', '1'))
LAN1 = int(E('LAN1', '20'))
LAN2 = int(E('LAN2', '13'))
GLO = int(E('GLO', '0'))
NCH = int(E('NCH', '4'))
Q0 = int(E('Q0', '1'))
S, D = 2048, 640
ND = 5
L = 128
NA = S // L
T = 256
NT = S // T
H, DH = 32, 20
HALO = 16
KH = 8
GR = 16
GE = int(E('GE', '8'))
NG = T // GR
LOG2E = 1.4426950408889634
QSCALE = float(DH ** -0.5) * LOG2E
MASKED = -1e9 * LOG2E
F32, BF16, U32 = jnp.float32, jnp.bfloat16, jnp.uint32


def _scope(name):
    return jax.named_scope(name) if SCOPES else contextlib.nullcontext()


def _dft_constants():
    forder = np.concatenate([np.arange(0, 128, 2), np.arange(1, 128, 2)])
    th = np.pi * (2 * forder + 1) / 256.0
    b = np.arange(128)
    fre, fim = np.cos(np.outer(th, b)), -np.sin(np.outer(th, b))
    fwd = np.concatenate([fre, fim, fre + fim], 0)
    gre = np.cos(np.outer(b, th)) / 128
    gim = -np.sin(np.outer(b, th)) / 128
    inv = np.stack([gre, gim], -1).reshape(128, 256)
    return fwd.astype(np.float32), inv.astype(np.float32), np.eye(128, dtype=np.float32)


def _bf(x):
    return pltpu.bitcast(x, BF16)


def _u32(x):
    return pltpu.bitcast(x, U32)


def _bmul(x, t8):
    return (x.reshape(-1, 8, 128) * t8).reshape(x.shape)


def _badd(x, t8):
    return (x.reshape(-1, 8, 128) + t8).reshape(x.shape)


def _dot(a, b):
    return jnp.dot(a, b, preferred_element_type=F32)


def _dot_nt(a, b):
    return jax.lax.dot_general(a, b, (((1,), (1,)), ((), ())), preferred_element_type=F32)


class _Copies:
    def __init__(self, cs):
        self.cs = list(cs)

    def start(self):
        for c in self.cs:
            c.start()

    def wait(self):
        for c in self.cs:
            c.wait()


def _kernel(q_hbm, k_hbm, v_hbm, shk_hbm, sk_hbm, dvec_hbm, wqkv_hbm, wo_hbm, gw_hbm,
            fwd_hbm, inv_hbm, eye_hbm,
            out_hbm,
            shk_ref, dvec_ref, gw_ref, fwd_ref, inv_ref, eye_ref,
            kbuf, vbuf, skbuf, qbuf, wqkv_v, wo_v, par, zvec, zsm, fwdp, invp, onesp, eyep,
            kvp, ubuf0, ubuf1, kpbuf0, kpbuf1, ybuf0, ybuf1, kst0, kst1, y2, wt, wtp, wnn, wof, wop,
            qp0, qp1, kp0, kp1, vp0, vp1, pbuf, sbuf, lbuf, op, op2, bres0, bres1, obuf, gsp, glog0, glog1,
            sem_a, sem_q, sem_w, sem_o, sem_s, sem_f):
    ubuf, kpbuf, ybuf, kstb = (ubuf0, ubuf1), (kpbuf0, kpbuf1), (ybuf0, ybuf1), (kst0, kst1)
    qp, kp, vp = (qp0, qp1), (kp0, kp1), (vp0, vp1)
    bres, glog = (bres0, bres1), (glog0, glog1)
    skw, qw, wqkvw = skbuf.bitcast(U32), qbuf.bitcast(U32), wqkv_v.bitcast(U32)
    kw, vw = kbuf.bitcast(U32), vbuf.bitcast(U32)

    def kv_copy(j):
        return _Copies(
            [pltpu.make_async_copy(k_hbm.at[0, :, pl.ds(j * 128, 128)], kbuf.at[j, pl.ds(2 * KH, S)], sem_a.at[3 * j]),
             pltpu.make_async_copy(v_hbm.at[0, :, pl.ds(j * 128, 128)], vbuf.at[j], sem_a.at[3 * j + 1])])

    def sk_copy(j):
        return _Copies(pltpu.make_async_copy(sk_hbm.at[pl.ds(j * 128, 128), pl.ds(m * L, L)], skbuf.at[j, m],
                                             sem_a.at[3 * j + 2]) for m in range(NA))

    def slab_copy(j):
        return _Copies(kv_copy(j).cs + sk_copy(j).cs)

    def first_copy(ch):
        rows = pl.ds(ch * (S // NCH), S // NCH)
        ms = range(ch * (NA // NCH), (ch + 1) * (NA // NCH))
        return _Copies(
            [pltpu.make_async_copy(k_hbm.at[0, rows, pl.ds(0, 128)],
                                   kbuf.at[0, pl.ds(2 * KH + ch * (S // NCH), S // NCH)], sem_f.at[ch]),
             pltpu.make_async_copy(v_hbm.at[0, rows, pl.ds(0, 128)], vbuf.at[0, rows], sem_f.at[ch])]
            + [pltpu.make_async_copy(sk_hbm.at[pl.ds(0, 128), pl.ds(m * L, L)], skbuf.at[0, m], sem_f.at[ch])
               for m in ms])

    small_copy = _Copies(pltpu.make_async_copy(a, b, sem_s.at[i]) for i, (a, b) in enumerate(
        [(shk_hbm, shk_ref), (dvec_hbm, dvec_ref), (gw_hbm, gw_ref), (fwd_hbm, fwd_ref), (inv_hbm, inv_ref),
         (eye_hbm, eye_ref)]))
    def q_copy(b):
        rows = pl.ds(b * T, T)
        return _Copies(pltpu.make_async_copy(q_hbm.at[0, rows, pl.ds(j * 128, 128)], qbuf.at[j, rows], sem_q.at[b])
                       for j in range(ND))

    wqkv_copy = _Copies(pltpu.make_async_copy(wqkv_hbm.at[:, pl.ds(n * 128, 128)], wqkv_v.at[n], sem_w.at[0])
                        for n in range(15))
    wo_copy = _Copies(pltpu.make_async_copy(wo_hbm.at[:, pl.ds(n * 128, 128)], wo_v.at[n], sem_w.at[1])
                      for n in range(ND))

    def out_copy(b, r0=0, n=T):
        return _Copies(pltpu.make_async_copy(obuf.at[b % NOB, j, pl.ds(r0, n)],
                                             out_hbm.at[0, pl.ds(b * T + r0, n), pl.ds(j * 128, 128)],
                                             sem_o.at[b % NOB]) for j in range(ND))

    with _scope("s_issue"):
        small_copy.start()
        if ONLY != 'B':
            first_copy(0).start()
    with _scope("s_wait"):
        small_copy.wait()
    if ONLY != 'B':
        for ch in range(1, NCH):
            first_copy(ch).start()

    with _scope("s_setup"):
        taps = shk_ref[...].astype(F32)
        dv = dvec_ref[...].astype(F32).reshape(1, D)
        gw = gw_ref[...].astype(F32).reshape(1, D)
        for j in range(ND):
            for i in range(4):
                par[j, i] = jnp.broadcast_to(taps[i:i + 1, j * 128:(j + 1) * 128], (8, 128))
            par[j, 4] = jnp.broadcast_to(dv[:, j * 128:(j + 1) * 128], (8, 128))
            par[j, 5] = jnp.broadcast_to(gw[:, j * 128:(j + 1) * 128], (8, 128))
        zvec[...] = jnp.zeros((8, 128), F32)
        for i in range(64):
            zsm[i] = 0
        fwdp[...] = _u32(fwd_ref[...])
        invp[...] = _u32(inv_ref[...])
        eyep[...] = _u32(eye_ref[...])
        onesp[...] = _u32(jnp.ones((128, 128), BF16))
        for j in range(ND):
            kw[j, 0:KH, :] = jnp.zeros((KH, 128), U32)
        for j in range(ND):
            kp0[j, 0:HALO, :] = jnp.zeros((HALO, 128), F32)
            vp0[j, 0:HALO, :] = jnp.zeros((HALO, 128), F32)

    def fresh(i):
        return pl.multiple_of(zsm[i] * 8, 8)

    def gated(tok):
        i = tok[0, 0].astype(jnp.int32)
        return pl.multiple_of(jnp.minimum(jnp.maximum(i, zsm[62]), zsm[63]) * 8, 8)

    def kvprep(j, blks=range(NA), tok=None):
        t = [par[j, i] if tok is None else par[j, i] + tok * zvec[...] for i in range(4)]
        even = lambda w: pltpu.bitcast(w << 16, F32)
        odd = lambda w: pltpu.bitcast(w & jnp.uint32(0xFFFF0000), F32)
        for c in blks:
            for q in range(L // 32):
                r = c * (L // 2) + q * 16
                w0 = kw[j, KH + r:KH + r + 16, :]
                w1 = kw[j, KH + r - 1:KH + r + 15, :]
                w2 = kw[j, KH + r - 2:KH + r + 14, :]
                e0, o0, e1, o1, o2 = even(w0), odd(w0), even(w1), odd(w1), odd(w2)
                ks_e = _bmul(e0, t[0]) + _bmul(o1, t[1]) + _bmul(e1, t[2]) + _bmul(o2, t[3])
                ks_o = _bmul(o0, t[0]) + _bmul(e0, t[1]) + _bmul(o1, t[2]) + _bmul(e1, t[3])
                wv = vw[j, r:r + 16, :]
                pe = ks_e * even(wv)
                kvp[j, r:r + 16, :] = pltpu.pack_elementwise([pe, ks_o * odd(wv)], packed_dtype=BF16)
        return pe[0:8]

    def dft_u(j, s, cs=range(NA)):
        cs = list(cs)
        if BIG:
            f = _bf(fwdp[pl.ds(fresh(16), 192 if USM else 128), :])
            rhs = jnp.concatenate([_bf(kvp[j, c * 64:(c + 1) * 64, :]) for c in cs], axis=1)
            r = _dot(f, rhs)
            for n, c in enumerate(cs):
                for i in range(3 if USM else 2):
                    ubuf[s][i, c] = r[i * 128:(i + 1) * 128, n * 128:(n + 1) * 128]
            return [r[0:8, n * 128:(n + 1) * 128] for n in range(len(cs))]
        toks = []
        for c in cs:
            f = _bf(fwdp[pl.ds(fresh(16 + c), 192 if USM else 128), :])
            r = _dot(f, _bf(kvp[j, c * 64:(c + 1) * 64, :]))
            for i in range(3 if USM else 2):
                ubuf[s][i, c] = r[i * 128:(i + 1) * 128]
            toks.append(r[0:8])
        return toks

    def dft_k(j, s, ms=range(NA)):
        ms = list(ms)
        if BIG:
            f = _bf(fwdp[pl.ds(fresh(32), 128), :])
            rhs = jnp.concatenate([_bf(skw[j, m]) for m in ms], axis=0)
            r = _dot_nt(f, rhs)
            for n, m in enumerate(ms):
                kpbuf[s][m] = r[:, n * 128:(n + 1) * 128]
            return [r[0:8, n * 128:(n + 1) * 128] for n in range(len(ms))]
        toks = []
        for m in ms:
            f = _bf(fwdp[pl.ds(fresh(32 + m), 128), :])
            r = _dot_nt(f, _bf(skw[j, m]))
            kpbuf[s][m] = r
            toks.append(r[0:8])
        return toks

    def aconv(s, plist=range(16), toks=None, mode=None, tz=True, btoks=None, ab=AB):
        ub, kb, yb = ubuf[s], kpbuf[s], ybuf[s]

        def kprep(p, ms=range(NA)):
            r, im = p * 8, 128 + p * 8
            kst = kstb[p % 2]
            for m in ms:
                pr, pi = kb[m, r:r + 8, :], kb[m, im:im + 8, :]
                if m == 0:
                    kr, ki = pr, pi
                    if toks is not None and toks[p] is not None:
                        kr = kr + (toks[p] * zvec[...] if tz else toks[p])
                elif p < 8:
                    kr, ki = pr - kb[m - 1, im:im + 8, :], pi + kb[m - 1, r:r + 8, :]
                else:
                    kr, ki = pr + kb[m - 1, im:im + 8, :], pi - kb[m - 1, r:r + 8, :]
                kst[m * 8:m * 8 + 8, :] = kr
                kst[128 + m * 8:128 + m * 8 + 8, :] = kr + ki
                kst[256 + m * 8:256 + m * 8 + 8, :] = ki - kr

        def macs(p, nxt=None):
            r = p * 8
            kst = kstb[p % 2]
            nb = NA // ab
            for bi, a0 in enumerate(range(0, NA, ab)):
                z = fresh(bi)
                if btoks is not None and btoks[p][bi] is not None:
                    z = gated(btoks[p][bi])
                acc = [[None] * ab for _ in range(3)]
                ncs = a0 + ab
                todo = []
                if nxt is not None and KSPREAD:
                    if bi >= nb - 2:
                        half = bi - (nb - 2)
                        todo = list(range(half * 8, half * 8 + 8))
                for c in range(ncs):
                    if USM:
                        uu = [ub[i, c, pl.ds(z + r, 8), :] for i in (2, 1, 0)]
                    else:
                        u_i, u_r = ub[1, c, pl.ds(z + r, 8), :], ub[0, c, pl.ds(z + r, 8), :]
                        uu = [u_r + u_i, u_i, u_r]
                    for i in range(ab):
                        m = a0 + i - c
                        if m < 0:
                            continue
                        for t in range(3):
                            x = kst[pl.ds(z + t * 128 + m * 8, 8), :] * uu[t]
                            acc[t][i] = x if acc[t][i] is None else acc[t][i] + x
                    if todo and c < 8:
                        kprep(nxt, [todo[c]])
                for i in range(ab):
                    yb[a0 + i, r:r + 8, :] = pltpu.pack_elementwise(
                        [acc[0][i] - acc[1][i], acc[0][i] + acc[2][i]], packed_dtype=BF16)

        plist = list(plist)
        kprep(plist[0])
        for n, p in enumerate(plist):
            nxt = plist[n + 1] if n + 1 < len(plist) else None
            if nxt is not None and not KSPREAD:
                kprep(nxt)
            macs(p, nxt)

    def idft(j, s, as_=range(NA)):
        as_ = list(as_)
        if BIG:
            z = fresh(48)
            toks = []
            for h in range(2):
                g = _bf(invp[pl.ds(z, 64), h * 128:(h + 1) * 128])
                rhs = jnp.concatenate([_bf(ybuf[s][a, h * 64:(h + 1) * 64, :]) for a in as_], axis=1)
                r = _dot(g, rhs)
                for n, a in enumerate(as_):
                    y2[h, j, a * L:(a + 1) * L, :] = r[:, n * 128:(n + 1) * 128]
                toks += [r[0:8, n * 128:(n + 1) * 128] for n in range(len(as_))]
            return toks
        toks = []
        for a in as_:
            z = fresh(48 + a)
            g0 = _bf(invp[pl.ds(z, 64), 0:128])
            g1 = _bf(invp[pl.ds(z, 64), 128:256])
            r0 = _dot(g0, _bf(ybuf[s][a, 0:64, :]))
            r1 = _dot(g1, _bf(ybuf[s][a, 64:128, :]))
            y2[0, j, a * L:(a + 1) * L, :] = r0
            y2[1, j, a * L:(a + 1) * L, :] = r1
            toks.append(r1[0:8])
        return toks

    def w_transpose(ns=range(15)):
        toks = []
        for n in ns:
            eye = _bf(eyep[pl.ds(fresh(n), 64), :])
            r = _dot_nt(eye, _bf(wqkvw[n]))
            for kt in range(ND):
                wt[kt, n * 128:(n + 1) * 128, :] = r[:, kt * 128:(kt + 1) * 128]
            toks.append(r[0:8, 0:128])
        return toks

    def w_permute(parts=range(3)):
        for p in parts:
            for dh in range(DH):
                for kt in range(ND):
                    rows = wt[kt, pl.ds(p * D + dh, H, stride=DH), :]
                    r0 = (p * D + dh * H) // 2
                    wtp[r0:r0 + H // 2, kt * 128:(kt + 1) * 128] = _u32(rows.astype(BF16))

    def wo_permute():
        for j in range(ND):
            wof[j] = wo_v[j].astype(F32)
        for dh in range(DH):
            for j in range(ND):
                rows = wof[j, pl.ds(dh, H, stride=DH), :]
                r0 = dh * H // 2
                wop[r0:r0 + H // 2, j * 128:(j + 1) * 128] = _u32(rows.astype(BF16))

    def qkv(b, s, fine=False):
        r0 = pl.multiple_of(b * (T // 2), T // 2)
        if MSPLIT > 1:
            h = T // MSPLIT
            rs = []
            for i in range(MSPLIT):
                x = jnp.concatenate([_bf(qw[j, pl.ds(r0 + i * h // 2, h // 2), :]) for j in range(ND)], axis=1)
                r = _dot_nt(x, _bf(wtp[pl.ds(fresh(20 + i), 3 * D // 2), :]))
                for j in range(ND):
                    qp[s][j, i * h:(i + 1) * h, :] = r[:, j * 128:(j + 1) * 128]
                    kp[s][j, HALO + i * h:HALO + (i + 1) * h, :] = r[:, D + j * 128:D + (j + 1) * 128]
                    vp[s][j, HALO + i * h:HALO + (i + 1) * h, :] = r[:, 2 * D + j * 128:2 * D + (j + 1) * 128]
                rs.append(r)
            allt = [rs[i][0:8, n * 128:(n + 1) * 128] * zvec[...] for i in range(MSPLIT) for n in range(15)]
            return [allt[(k * len(allt)) // 15] for k in range(15)]
        x = jnp.concatenate([_bf(qw[j, pl.ds(r0, T // 2), :]) for j in range(ND)], axis=1)
        r = _dot(x, _bf(wnn[...])) if NNW else _dot_nt(x, _bf(wtp[...]))
        for j in range(ND):
            qp[s][j] = r[:, j * 128:(j + 1) * 128]
            kp[s][j, HALO:HALO + T, :] = r[:, D + j * 128:D + (j + 1) * 128]
            vp[s][j, HALO:HALO + T, :] = r[:, 2 * D + j * 128:2 * D + (j + 1) * 128]
        if fine:
            return [r[64 * i:64 * i + 8, n * 128:(n + 1) * 128] * zvec[...] for n in range(15) for i in range(4)]
        return [r[0:8, n * 128:(n + 1) * 128] * zvec[...] for n in range(15)]

    def qkv_half(b, s, i):
        h = T // 2
        r0 = b * (T // 2) + i * (h // 2)
        x = jnp.concatenate([_bf(qw[j, r0:r0 + h // 2, :]) for j in range(ND)], axis=1)
        r = _dot_nt(x, _bf(wtp[pl.ds(fresh(20 + i), 3 * D // 2), :]))
        for j in range(ND):
            qp[s][j, i * h:(i + 1) * h, :] = r[:, j * 128:(j + 1) * 128]
            kp[s][j, HALO + i * h:HALO + (i + 1) * h, :] = r[:, D + j * 128:D + (j + 1) * 128]
            vp[s][j, HALO + i * h:HALO + (i + 1) * h, :] = r[:, 2 * D + j * 128:2 * D + (j + 1) * 128]
        return [r[0:8, n * 128:(n + 1) * 128] * zvec[...] for n in range(15)]

    def gate(b, s, mt=None):
        r0 = pl.multiple_of(b * T, T)
        for g in range(NG):
            sm = None if mt is None else jnp.concatenate([mt[(g * GN) // NG]] * (GR // 8), axis=0)
            for j in range(ND):
                t = _bmul(qbuf[j, pl.ds(r0 + g * GR, GR), :].astype(F32), par[j, 5])
                sm = t if sm is None else sm + t
            hi = sm.astype(BF16)
            gsp[0, g * GR // 2:(g + 1) * GR // 2, :] = _u32(hi)
            if GLO:
                lo = (sm - hi.astype(F32)).astype(BF16)
                gsp[1, g * GR // 2:(g + 1) * GR // 2, :] = _u32(lo)
        ones = _bf(onesp[...])
        glog[s][0] = _dot(_bf(gsp[0]), ones)
        if GLO:
            glog[s][1] = _dot(_bf(gsp[1]), ones)

    def halo(s):
        for j in range(ND):
            kp[1 - s][j, 0:HALO, :] = kp[s][j, T:T + HALO, :]
            vp[1 - s][j, 0:HALO, :] = vp[s][j, T:T + HALO, :]

    def softmax_pv(vv, row, ob, lg=None):
        if lg is None:
            lg = [lbuf[w, row:row + GR, :] for w in range(8)]
        m = lg[0]
        for w in range(1, 8):
            m = jnp.maximum(m, lg[w])
        es = [(l - m) if E('NOEXP', '0') == '1' else jnp.exp2(l - m) for l in lg]
        sm = es[0]
        for w in range(1, 8):
            sm = sm + es[w]
        inv = 1.0 / sm
        for j in range(ND):
            acc = None
            for w in range(8):
                o = row + HALO - 2 * w
                t = es[w] * vv[j, o:o + GR, :]
                acc = t if acc is None else acc + t
            res = acc * inv
            ob[row // 2:(row + GR) // 2, j * 128:(j + 1) * 128] = _u32(res.astype(BF16))
        return res[0:8]

    def qk(qq, kk, row, tok):
        if tok is None:
            q = [qq[j, row:row + GE, :] * QSCALE for j in range(ND)]
        else:
            sc = tok + QSCALE
            q = [_bmul(qq[j, row:row + GE, :], sc) for j in range(ND)]
        out = []
        for w in range(8):
            p = None
            o = row + HALO - 2 * w
            for j in range(ND):
                t = q[j] * kk[j, o:o + GE, :]
                p = t if p is None else p + t
            out.append(p)
        return out

    def attention(b, s, mt=None, row0=0, nrows=T, an=AN, ob=None):
        qq, kk, vv = qp[s], kp[s], vp[s]
        ob = op if ob is None else ob
        g0 = row0 // GE
        n1 = g0 + nrows // GE
        per = GR // GE
        r1, r2, done = {}, {}, {}
        for g in range(g0, n1 + D3 + per):
            if g < n1:
                row = g * GE
                tok = None
                if mt is not None:
                    tok = mt[((g - g0) * an) // (n1 - g0)]
                    prev = done.get(row // GR - PACE) if PACE else None
                    if prev is not None:
                        tok = tok + prev * zvec[...]
                r1[g] = []
                for w, p in enumerate(qk(qq, kk, row, tok)):
                    pbuf[w, row:row + GE, :] = p
                    r1[g].append(p * 2.0 if E('NOROLL', '0') == '1' else pltpu.roll(p, 64, 1))
            gg = g - D1
            if g0 <= gg < n1:
                row = gg * GE
                r2[gg] = []
                for w, r in enumerate(r1.pop(gg)):
                    sm = pbuf[w, row:row + GE, :] + r
                    sbuf[w, row:row + GE, :] = sm
                    r2[gg].append(sm * 2.0 if E('NOROLL', '0') == '1' else pltpu.roll(sm, 32, 1))
            gg = g - D2
            if g0 <= gg < n1:
                row = gg * GE
                ls = []
                for w, r in enumerate(r2.pop(gg)):
                    l = sbuf[w, row:row + GE, :] + r
                    if row < HALO and w > 0:
                        t = b * T + row + jax.lax.broadcasted_iota(jnp.int32, (GE, 128), 0)
                        l = jnp.where(t >= 2 * w, l, MASKED)
                    if NOLBUF:
                        ls.append(l)
                    else:
                        lbuf[w, row:row + GE, :] = l
                if NOLBUF:
                    done[row // GR] = softmax_pv(vv, row, ob, ls)
            gg = g - D3
            if not NOLBUF and g0 <= gg < n1 and (gg + 1) % per == 0:
                row = (gg + 1 - per) * GE
                done[row // GR] = softmax_pv(vv, row, ob)

    def outproj(s, r0=0, n=T, ob=None):
        ob = op if ob is None else ob
        r = _dot(_bf(ob[r0 // 2:(r0 + n) // 2, :]), _bf(wop[...]))
        bres[s][r0:r0 + n, :] = r
        return [r[0:8, k * 128:(k + 1) * 128] * zvec[...] for k in range(ND)]

    def epilogue(b, s, mt=None, gs=range(NG)):
        r0 = pl.multiple_of(b * T, T)
        for g in gs:
            row = r0 + g * GR
            rowh = pl.multiple_of(b * (T // 2), T // 2) + g * (GR // 2)
            gl = glog[s][0, g * GR:(g + 1) * GR, :]
            if GLO:
                gl = gl + glog[s][1, g * GR:(g + 1) * GR, :]
            if mt is not None:
                gl = _badd(gl, mt[(g * EN) // NG])
            gt = jax.nn.sigmoid(gl)
            for j in range(ND):
                q = qbuf[j, pl.ds(row, GR), :].astype(F32)
                kv = _bf(kvp[j, pl.ds(rowh, GR // 2), :]).astype(F32)
                z = y2[0, j, pl.ds(row, GR), :] + y2[1, j, pl.ds(row, GR), :] + _bmul(kv, par[j, 4])
                bb = bres[s][g * GR:(g + 1) * GR, j * 128:(j + 1) * 128]
                o = bb + gt * (q * z - bb)
                obuf[b % NOB, j, g * GR:(g + 1) * GR, :] = o.astype(BF16)

    def region(k, f):
        pl.when(zsm[k % 64] == 0)(f)

    P = functools.partial

    wq_0, wq_1, wq_b = _Copies(wqkv_copy.cs[:WQ0]), _Copies(wqkv_copy.cs[WQ0:8]), _Copies(wqkv_copy.cs[8:])
    wq_a = _Copies(wqkv_copy.cs[:8])

    def x_dma(j):
        with _scope("waitX%d" % j):
            sk_copy(j + 1).wait()
            if j >= 1:
                kv_copy(j + 1).wait()
            if j == 2 and not WLATE:
                wq_a.wait()
            if j == 3 and not WLATE:
                wq_b.wait()
        if j == 0:
            kv_copy(2).start()
            sk_copy(2).start()
            if not WLATE:
                wq_0.start()
        if j == 1:
            kv_copy(3).start()
            sk_copy(3).start()
            if not WLATE:
                wq_1.start()
        if j == 2:
            kv_copy(4).start()
            sk_copy(4).start()
            (wq_0 if WLATE else wq_b).start()
        if j == 3 and WLATE:
            _Copies(wqkv_copy.cs[WQ0:]).start()
        if j == 3:
            q_copy(0).start()
            if not WLATE:
                wo_copy.start()
                q_copy(1).start()

    def block_x(j):
        s = j % 2
        with _scope("X%d" % j):
            if j >= 1:
                tk = kvprep(j + 1)
                aconv(s, toks=[tk] * 16 if KVFIRST2 else None)
            else:
                aconv(s)
            if j >= 1:
                idft(j - 1, 1 - s)
            dft_k(j + 1, 1 - s)
            if j == 2 and not WLATE:
                w_transpose(range(0, 8))
            if j == 3 and not WLATE:
                w_transpose(range(8, 15))
                if PERM_EARLY:
                    w_permute([0])
            if j >= 1:
                dft_u(j + 1, 1 - s)
        if j == 0:
            with _scope("waitK1"):
                kv_copy(1).wait()
            with _scope("Y0"):
                kvprep(1)
                dft_u(1, 1)

    def body_a(j, carry):
        return carry

    def b_dma(b, s):
        if ONLY == '':
            q_copy(b).wait()

        @pl.when(b - 2 >= NOB)
        def _():
            out_copy(b - 2 - NOB).wait()

    def epilogue_wait(t):
        if t >= NOB:
            out_copy(t - NOB).wait()

    def block_b(b, s, dma=True):
        if dma:
            b_dma(b, s)
        with _scope("B"):
            halo(1 - s)
            mt = qkv(b, s)
            if EPI == 'paced':
                epilogue(b - 2, s, mt)
            elif EPI == 'free':
                epilogue(b - 2, s)
            elif EPI == 'late':
                epilogue(b - 2, s, [mt[14]] * 15)
            if EPI != 'after':
                out_copy(b - 2).start()
            if E('NOATT', '0') != '1':
                attention(b - 1, 1 - s, mt)
            if E('NOGATE', '0') != '1':
                gate(b - 1, 1 - s, mt if GATEP else None)
            if EPI == 'after':
                ot = outproj(1 - s)
                epilogue(b - 2, s, [ot[(g * 5) // 15] for g in range(15)])
                out_copy(b - 2).start()
            else:
                outproj(1 - s)

    def body_b2(i, carry):
        b = 2 * i
        if ONLY == '':
            q_copy(b).wait()
            q_copy(b + 1).wait()

        @pl.when(b - 2 >= NOB)
        def _():
            out_copy(b - 2 - NOB).wait()
            out_copy(b - 1 - NOB).wait()
        block_b(b, 0, False)
        block_b(b + 1, 1, False)
        return carry

    def body_b(b, carry):
        if E('ONEPAR', '0') == '1':
            block_b(b, 0)
            return carry
        for s in range(2):
            pl.when(b % 2 == s)(functools.partial(block_b, b, s))
        return carry

    if ONLY != 'B':
        nb = NA // NCH
        for ch in range(NCH):
            with _scope("wait0"):
                first_copy(ch).wait()
            if ch == 1:
                sk_copy(1).start()
            if ch == NCH - 1:
                kv_copy(1).start()
            with _scope("pro"):
                blks = range(ch * nb, (ch + 1) * nb)
                kvprep(0, blks)
                dft_k(0, 0, blks)
                dft_u(0, 0, blks)

        for j in range(ND - 1):
            x_dma(j)
            region(2 * j, P(block_x, j))

    if ONLY == '':
        q_copy(0).wait()
        if WLATE:
            wqkv_copy.wait()
            wo_copy.start()
            q_copy(1).start()
        for b in range(2, NT):
            q_copy(b).start()

        def block_wlate():
            with _scope("Alast0"):
                aconv((ND - 1) % 2)
                idft(ND - 2, (ND - 2) % 2)
                w_transpose()
                if AMERGE >= 1:
                    w_permute([0] if AMERGE == 1 else [0, 1, 2])
                if AMERGE == 3:
                    qkv(0, 0)

        if WLATE:
            region(12, block_wlate)

        def block_alast():
            if WLATE:
                with _scope("Alast"):
                    if AMERGE == 3:
                        return
                    w_permute({0: [0, 1, 2], 1: [1, 2], 2: []}[AMERGE])
                    qkv(0, 0)
                return
            with _scope("Alast"):
                w_permute([1, 2] if PERM_EARLY else [0, 1, 2])
                if Q0 == 3:
                    idft(ND - 2, (ND - 2) % 2)
                    mt = qkv(0, 0, True)
                    wts = [sum(a + 1 for a in range(a0, a0 + LAB)) for a0 in range(0, NA, LAB)]
                    tot = 136 * 16
                    bt, cum = [], 0
                    for p in range(16):
                        row = []
                        for bi in range(len(wts)):
                            k = (cum * LN * len(mt)) // (tot * 16) - LOFF
                            row.append(mt[min(k, len(mt) - 1)] if k >= 0 else None)
                            cum += wts[bi]
                        bt.append(row)
                    aconv((ND - 1) % 2, range(16), btoks=bt, ab=LAB)
                elif Q0 == 2:
                    idft(ND - 2, (ND - 2) % 2)
                    mt = qkv(0, 0)
                    toks = [None] + [mt[min(14, ((p - 1) * LN) // 16)] for p in range(1, 16)]
                    aconv((ND - 1) % 2, range(16), toks, tz=False)
                else:
                    aconv((ND - 1) % 2)
                    idft(ND - 2, (ND - 2) % 2)
                    if Q0:
                        qkv(0, 0)

        region(10, block_alast)

        def block_b1():
            q_copy(1).wait()
            wo_copy.wait()
            with _scope("B1"):
                wo_permute()
                if not Q0:
                    qkv(0, 0)
                idft(ND - 1, (ND - 1) % 2)
                halo(0)
                mt = qkv(1, 1)
                attention(0, 0, mt)
                gate(0, 0, mt)
                outproj(0)

        region(11, block_b1)

    if ONLY != 'A':
        if PAIR:
            jax.lax.fori_loop(1, NT // 2, body_b2, 0)
        else:
            jax.lax.fori_loop(2, NT - 1 if (LASTB and ONLY == '') else NT, body_b, 0)

    if ONLY == '':
        if LASTB:
            def block_last():
                b, s = NT - 1, (NT - 1) % 2
                q_copy(b).wait()
                epilogue_wait(b - 2)
                with _scope("B7"):
                    halo(1 - s)
                    m1 = qkv_half(b, s, 0)
                    m2 = qkv_half(b, s, 1)
                    epilogue(b - 2, s, [m2[14]] * 15)
                    out_copy(b - 2).start()
                    attention(b - 1, 1 - s, m1 + m2, an=LAN1)
                    gate(b - 1, 1 - s, m1)
                    attention(b, s, m2, 0, T // 2, an=LAN2, ob=op2)
                    outproj(1 - s)

            region(13, block_last)
            with _scope("fin1"):
                epilogue_wait(NT - 2)
                epilogue_wait(NT - 1)
                epilogue(NT - 2, 0)
                out_copy(NT - 2).start()
                gate(NT - 1, 1)
                attention(NT - 1, 1, None, T // 2, T // 2, ob=op2)
                nh = T // FSPLIT
                for h in range(FSPLIT):
                    outproj(1, h * nh, nh, op2)
                for h in range(FSPLIT):
                    epilogue(NT - 1, 1, None, range(h * nh // GR, (h + 1) * nh // GR))
                    out_copy(NT - 1, h * nh, nh).start()
        elif FSPLIT:
            with _scope("fin1"):
                epilogue_wait(NT - 2)
                epilogue_wait(NT - 1)
                epilogue(NT - 2, 0)
                out_copy(NT - 2).start()
                gate(NT - 1, 1)
                attention(NT - 1, 1)
                nh = T // FSPLIT
                for h in range(FSPLIT):
                    outproj(1, h * nh, nh)
                for h in range(FSPLIT):
                    epilogue(NT - 1, 1, None, range(h * nh // GR, (h + 1) * nh // GR))
                    out_copy(NT - 1, h * nh, nh).start()
        else:
            with _scope("fin1"):
                epilogue_wait(NT - 2)
                epilogue(NT - 2, 0)
                out_copy(NT - 2).start()
                attention(NT - 1, 1)
                gate(NT - 1, 1)
                outproj(1)
            with _scope("fin2"):
                epilogue_wait(NT - 1)
                epilogue(NT - 1, 1)
                out_copy(NT - 1).start()
        with _scope("fin3"):
            for t in range(NT - NOB, NT):
                out_copy(t).wait()
    elif ONLY == 'B':
        for t in range(NT - 2 - NOB, NT - 2):
            out_copy(t).wait()
    else:
        for b in range(2):
            q_copy(b).wait()
        wo_copy.wait()


@jax.jit
def pallas_gated_mix__ssm_conv_h3__sliding_local_dilated__prompt_kernel(A_q, A_k, A_v, A_shift_k, A_ssm_k, A_ssm_D, B_x, B_wqkv, B_wo, gate_w):
    fwd, inv, eye = _dft_constants()
    hbm = pl.BlockSpec(memory_space=pl.ANY)
    vm = pl.BlockSpec(memory_space=pltpu.VMEM)
    two = lambda shape, dt: [pltpu.VMEM(shape, dt), pltpu.VMEM(shape, dt)]
    return pl.pallas_call(
        _kernel,
        out_shape=jax.ShapeDtypeStruct((1, S, D), BF16),
        in_specs=[hbm] * 12,
        out_specs=hbm,
        scratch_shapes=[
            pltpu.VMEM((4, D), BF16),
            pltpu.VMEM((D,), BF16),
            pltpu.VMEM((D,), BF16),
            pltpu.VMEM((384, 128), BF16),
            pltpu.VMEM((128, 256), BF16),
            pltpu.VMEM((128, 128), BF16),
            pltpu.VMEM((ND, 2 * KH + S, 128), BF16),
            pltpu.VMEM((ND, S, 128), BF16),
            pltpu.VMEM((ND, NA, 128, L), BF16),
            pltpu.VMEM((ND, S, 128), BF16),
            pltpu.VMEM((15, D, 128), BF16),
            pltpu.VMEM((ND, D, 128), BF16),
            pltpu.VMEM((ND, 6, 8, 128), F32),
            pltpu.VMEM((8, 128), F32),
            pltpu.SMEM((64,), jnp.int32),
            pltpu.VMEM((192, 128), U32),
            pltpu.VMEM((64, 256), U32),
            pltpu.VMEM((64, 128), U32),
            pltpu.VMEM((64, 128), U32),
            pltpu.VMEM((ND, S // 2, 128), U32),
            *two((3, NA, 128, 128), F32),
            *two((NA, 256, 128), F32),
            *two((NA, 128, 128), U32),
            *two((384, 128), F32),
            pltpu.VMEM((2, ND, S, 128), F32),
            pltpu.VMEM((ND, 3 * D, 128), F32),
            pltpu.VMEM((3 * D // 2, D), U32),
            pltpu.VMEM((D // 2, 3 * D), U32),
            pltpu.VMEM((ND, D, 128), F32),
            pltpu.VMEM((D // 2, D), U32),
            *two((ND, T, 128), F32),
            *two((ND, HALO + T, 128), F32),
            *two((ND, HALO + T, 128), F32),
            pltpu.VMEM((8, T, 128), F32),
            pltpu.VMEM((8, T, 128), F32),
            pltpu.VMEM((8, T, 128), F32),
            pltpu.VMEM((T // 2, D), U32),
            pltpu.VMEM((T // 2, D), U32),
            *two((T, D), F32),
            pltpu.VMEM((NOB, ND, T, 128), BF16),
            pltpu.VMEM((2, T // 2, 128), U32),
            *two((2, T, 128), F32),
            pltpu.SemaphoreType.DMA((3 * ND,)),
            pltpu.SemaphoreType.DMA((NT,)),
            pltpu.SemaphoreType.DMA((2,)),
            pltpu.SemaphoreType.DMA((NOB,)),
            pltpu.SemaphoreType.DMA((6,)),
            pltpu.SemaphoreType.DMA((NCH,)),
        ],
        compiler_params=pltpu.CompilerParams(vmem_limit_bytes=100 * 2 ** 20),
    )(A_q, A_k, A_v, A_shift_k.T, A_ssm_k, A_ssm_D, B_wqkv, B_wo, gate_w,
      jnp.asarray(fwd, BF16), jnp.asarray(inv, BF16), jnp.asarray(eye, BF16))
```

```python
import contextlib
import functools
import numpy as np
import jax
import jax.numpy as jnp
from jax.experimental import pallas as pl
from jax.experimental.pallas import tpu as pltpu


def E(key, default):
    return default


ONLY = E('ONLY', '')
SCOPES = int(E('SCOPES', '0'))
AN, EN, GN, PACE = int(E('AN', '13')), int(E('EN', '14')), int(E('GN', '10')), int(E('PACE', '4'))
D1, D2, D3 = int(E('D1', '2')), int(E('D2', '4')), int(E('D3', '5'))
DYNZ = int(E('DYNZ', '0'))
AB = int(E('AB', '4'))
ATOK = int(E('ATOK', '0'))
AOFF = int(E('AOFF', '1'))
ARATE = int(E('ARATE', '100'))
AORD = E('AORD', 'cf')
FR = int(E('FR', '100'))
USM = int(E('USM', '0'))
MERGE = int(E('MERGE', '0'))
KVFIRST = int(E('KVFIRST', '1'))
KSPLIT = int(E('KSPLIT', '8'))

WT_AT = int(E('WT_AT', '2'))
LN = int(E('LN', '15'))
EPI = E('EPI', 'late')
GATEP = int(E('GATEP', '1'))
NNW = int(E('NNW', '0'))
LOFF = int(E('LOFF', '0'))
LAB = int(E('LAB', '2'))
KVPOS = E('KVPOS', 'post')
TFIRST = int(E('TFIRST', '0'))
KVT = [int(x) for x in E('KVT', '-1,-1,-1').split(',')]
GATE = E('GATE', 'mem')
BIG = int(E('BIG', '0'))
KSPREAD = int(E('KSPREAD', '1'))
PAIR = int(E('PAIR', '0'))
NOB = 4
FSPLIT = int(E('FSPLIT', '4'))
PERM_EARLY = int(E('PERM_EARLY', '1'))
WQ0 = int(E('WQ0', '4'))
WLATE = int(E('WLATE', '1'))
KVFIRST2 = int(E('KVFIRST2', '0'))
NOLBUF = int(E('NOLBUF', '0'))
MSPLIT = int(E('MSPLIT', '1'))
AMERGE = int(E('AMERGE', '0'))
LASTB = int(E('LASTB', '1'))
LAN1 = int(E('LAN1', '20'))
LAN2 = int(E('LAN2', '13'))
GLO = int(E('GLO', '0'))
KVG = int(E('KVG', '4'))
STREAM = int(E('STREAM', '1'))
NCH = int(E('NCH', '4'))
Q0 = int(E('Q0', '1'))
S, D = 2048, 640
ND = 5
L = 128
NA = S // L
T = 256
NT = S // T
H, DH = 32, 20
HALO = 16
KH = 8
GR = 16
GE = int(E('GE', '8'))
NG = T // GR
LOG2E = 1.4426950408889634
QSCALE = float(DH ** -0.5) * LOG2E
MASKED = -1e9 * LOG2E
F32, BF16, U32 = jnp.float32, jnp.bfloat16, jnp.uint32


def _scope(name):
    return jax.named_scope(name) if SCOPES else contextlib.nullcontext()


def _dft_constants():
    forder = np.concatenate([np.arange(0, 128, 2), np.arange(1, 128, 2)])
    th = np.pi * (2 * forder + 1) / 256.0
    b = np.arange(128)
    fre, fim = np.cos(np.outer(th, b)), -np.sin(np.outer(th, b))
    fwd = np.concatenate([fre, fim, fre + fim], 0)
    gre = np.cos(np.outer(b, th)) / 128
    gim = -np.sin(np.outer(b, th)) / 128
    inv = np.stack([gre, gim], -1).reshape(128, 256)
    return fwd.astype(np.float32), inv.astype(np.float32), np.eye(128, dtype=np.float32)


def _bf(x):
    return pltpu.bitcast(x, BF16)


def _u32(x):
    return pltpu.bitcast(x, U32)


def _bmul(x, t8):
    return (x.reshape(-1, 8, 128) * t8).reshape(x.shape)


def _badd(x, t8):
    return (x.reshape(-1, 8, 128) + t8).reshape(x.shape)


def _dot(a, b):
    return jnp.dot(a, b, preferred_element_type=F32)


def _dot_nt(a, b):
    return jax.lax.dot_general(a, b, (((1,), (1,)), ((), ())), preferred_element_type=F32)


class _Copies:
    def __init__(self, cs):
        self.cs = list(cs)

    def start(self):
        for c in self.cs:
            c.start()

    def wait(self):
        for c in self.cs:
            c.wait()


def _kernel(q_hbm, k_hbm, v_hbm, shk_hbm, sk_hbm, dvec_hbm, wqkv_hbm, wo_hbm, gw_hbm,
            fwd_hbm, inv_hbm, eye_hbm,
            out_hbm,
            shk_ref, dvec_ref, gw_ref, fwd_ref, inv_ref, eye_ref,
            kbuf, vbuf, skbuf, qbuf, wqkv_v, wo_v, par, zvec, zsm, fwdp, invp, onesp, eyep,
            kvp, ubuf0, ubuf1, kpbuf0, kpbuf1, ybuf0, ybuf1, kst0, kst1, ksta, y2, wt, wtp, wnn, wof, wop,
            qp0, qp1, kp0, kp1, vp0, vp1, pbuf, sbuf, lbuf, op, op2, bres0, bres1, obuf, gsp, glog0, glog1,
            sem_a, sem_q, sem_w, sem_o, sem_s, sem_f):
    ubuf, kpbuf, ybuf, kstb = (ubuf0, ubuf1), (kpbuf0, kpbuf1), (ybuf0, ybuf1), (kst0, kst1)
    qp, kp, vp = (qp0, qp1), (kp0, kp1), (vp0, vp1)
    bres, glog = (bres0, bres1), (glog0, glog1)
    skw, qw, wqkvw = skbuf.bitcast(U32), qbuf.bitcast(U32), wqkv_v.bitcast(U32)
    kw, vw = kbuf.bitcast(U32), vbuf.bitcast(U32)

    def kv_copy(j):
        return _Copies(
            [pltpu.make_async_copy(k_hbm.at[0, :, pl.ds(j * 128, 128)], kbuf.at[j, pl.ds(2 * KH, S)], sem_a.at[3 * j]),
             pltpu.make_async_copy(v_hbm.at[0, :, pl.ds(j * 128, 128)], vbuf.at[j], sem_a.at[3 * j + 1])])

    def sk_copy(j):
        return _Copies(pltpu.make_async_copy(sk_hbm.at[pl.ds(j * 128, 128), pl.ds(m * L, L)], skbuf.at[j, m],
                                             sem_a.at[3 * j + 2]) for m in range(NA))

    def slab_copy(j):
        return _Copies(kv_copy(j).cs + sk_copy(j).cs)

    def first_copy(ch):
        rows = pl.ds(ch * (S // NCH), S // NCH)
        ms = range(ch * (NA // NCH), (ch + 1) * (NA // NCH))
        return _Copies(
            [pltpu.make_async_copy(k_hbm.at[0, rows, pl.ds(0, 128)],
                                   kbuf.at[0, pl.ds(2 * KH + ch * (S // NCH), S // NCH)], sem_f.at[ch]),
             pltpu.make_async_copy(v_hbm.at[0, rows, pl.ds(0, 128)], vbuf.at[0, rows], sem_f.at[ch])]
            + [pltpu.make_async_copy(sk_hbm.at[pl.ds(0, 128), pl.ds(m * L, L)], skbuf.at[0, m], sem_f.at[ch])
               for m in ms])

    small_copy = _Copies(pltpu.make_async_copy(a, b, sem_s.at[i]) for i, (a, b) in enumerate(
        [(shk_hbm, shk_ref), (dvec_hbm, dvec_ref), (gw_hbm, gw_ref), (fwd_hbm, fwd_ref), (inv_hbm, inv_ref),
         (eye_hbm, eye_ref)]))
    def q_copy(b):
        rows = pl.ds(b * T, T)
        return _Copies(pltpu.make_async_copy(q_hbm.at[0, rows, pl.ds(j * 128, 128)], qbuf.at[j, rows], sem_q.at[b])
                       for j in range(ND))

    wqkv_copy = _Copies(pltpu.make_async_copy(wqkv_hbm.at[:, pl.ds(n * 128, 128)], wqkv_v.at[n], sem_w.at[0])
                        for n in range(15))
    wo_copy = _Copies(pltpu.make_async_copy(wo_hbm.at[:, pl.ds(n * 128, 128)], wo_v.at[n], sem_w.at[1])
                      for n in range(ND))

    def out_copy(b, r0=0, n=T):
        return _Copies(pltpu.make_async_copy(obuf.at[b % NOB, j, pl.ds(r0, n)],
                                             out_hbm.at[0, pl.ds(b * T + r0, n), pl.ds(j * 128, 128)],
                                             sem_o.at[b % NOB]) for j in range(ND))

    for j in range(ND):
        kbuf[j, 0:2 * KH, :] = jnp.zeros((2 * KH, 128), BF16)
    with _scope("s_issue"):
        small_copy.start()
        if ONLY != 'B':
            first_copy(0).start()
    with _scope("s_wait"):
        small_copy.wait()
    if ONLY != 'B':
        for ch in range(1, NCH):
            first_copy(ch).start()

    with _scope("s_setup"):
        taps = shk_ref[...].astype(F32)
        dv = dvec_ref[...].astype(F32).reshape(1, D)
        gw = gw_ref[...].astype(F32).reshape(1, D)
        for j in range(ND):
            for i in range(4):
                par[j, i] = jnp.broadcast_to(taps[i:i + 1, j * 128:(j + 1) * 128], (8, 128))
            par[j, 4] = jnp.broadcast_to(dv[:, j * 128:(j + 1) * 128], (8, 128))
            par[j, 5] = jnp.broadcast_to(gw[:, j * 128:(j + 1) * 128], (8, 128))
        zvec[...] = jnp.zeros((8, 128), F32)
        for i in range(64):
            zsm[i] = 0
        fwdp[...] = _u32(fwd_ref[...])
        invp[...] = _u32(inv_ref[...])
        eyep[...] = _u32(eye_ref[...])
        onesp[...] = _u32(jnp.ones((128, 128), BF16))
        for j in range(ND):
            kp0[j, 0:HALO, :] = jnp.zeros((HALO, 128), F32)
            vp0[j, 0:HALO, :] = jnp.zeros((HALO, 128), F32)

    def fresh(i):
        return pl.multiple_of(zsm[i] * 8, 8)

    def gated(tok):
        i = tok[0, 0].astype(jnp.int32)
        return pl.multiple_of(jnp.minimum(jnp.maximum(i, zsm[62]), zsm[63]) * 8, 8)

    def kvprep(j, blks=range(NA), tok=None):
        t = [par[j, i] if tok is None else par[j, i] + tok * zvec[...] for i in range(4)]
        even = lambda w: pltpu.bitcast(w << 16, F32)
        odd = lambda w: pltpu.bitcast(w & jnp.uint32(0xFFFF0000), F32)
        for c in blks:
            for q in range(L // 32):
                r = c * (L // 2) + q * 16
                w0 = kw[j, KH + r:KH + r + 16, :]
                w1 = kw[j, KH + r - 1:KH + r + 15, :]
                w2 = kw[j, KH + r - 2:KH + r + 14, :]
                e0, o0, e1, o1, o2 = even(w0), odd(w0), even(w1), odd(w1), odd(w2)
                ks_e = _bmul(e0, t[0]) + _bmul(o1, t[1]) + _bmul(e1, t[2]) + _bmul(o2, t[3])
                ks_o = _bmul(o0, t[0]) + _bmul(e0, t[1]) + _bmul(o1, t[2]) + _bmul(e1, t[3])
                wv = vw[j, r:r + 16, :]
                pe = ks_e * even(wv)
                kvp[j, r:r + 16, :] = pltpu.pack_elementwise([pe, ks_o * odd(wv)], packed_dtype=BF16)
        return pe[0:8]

    def dft_u(j, s, cs=range(NA)):
        cs = list(cs)
        if BIG:
            f = _bf(fwdp[pl.ds(fresh(16), 192 if USM else 128), :])
            rhs = jnp.concatenate([_bf(kvp[j, c * 64:(c + 1) * 64, :]) for c in cs], axis=1)
            r = _dot(f, rhs)
            for n, c in enumerate(cs):
                for i in range(3 if USM else 2):
                    ubuf[s][i, c] = r[i * 128:(i + 1) * 128, n * 128:(n + 1) * 128]
            return [r[0:8, n * 128:(n + 1) * 128] for n in range(len(cs))]
        toks = []
        for c in cs:
            f = _bf(fwdp[pl.ds(fresh(16 + c), 192 if USM else 128), :])
            r = _dot(f, _bf(kvp[j, c * 64:(c + 1) * 64, :]))
            for i in range(3 if USM else 2):
                ubuf[s][i, c] = r[i * 128:(i + 1) * 128]
            toks.append(r[0:8])
        return toks

    def dft_k(j, s, ms=range(NA)):
        ms = list(ms)
        if BIG:
            f = _bf(fwdp[pl.ds(fresh(32), 128), :])
            rhs = jnp.concatenate([_bf(skw[j, m]) for m in ms], axis=0)
            r = _dot_nt(f, rhs)
            for n, m in enumerate(ms):
                kpbuf[s][m] = r[:, n * 128:(n + 1) * 128]
            return [r[0:8, n * 128:(n + 1) * 128] for n in range(len(ms))]
        toks = []
        for m in ms:
            f = _bf(fwdp[pl.ds(fresh(32 + m), 128), :])
            r = _dot_nt(f, _bf(skw[j, m]))
            kpbuf[s][m] = r
            toks.append(r[0:8])
        return toks

    def aconv(s, plist=range(16), toks=None, mode=None, tz=True, btoks=None, ab=AB):
        ub, kb, yb = ubuf[s], kpbuf[s], ybuf[s]

        def kprep(p, ms=range(NA)):
            r, im = p * 8, 128 + p * 8
            kst = kstb[p % 2]
            for m in ms:
                pr, pi = kb[m, r:r + 8, :], kb[m, im:im + 8, :]
                if m == 0:
                    kr, ki = pr, pi
                    if toks is not None and toks[p] is not None:
                        kr = kr + (toks[p] * zvec[...] if tz else toks[p])
                elif p < 8:
                    kr, ki = pr - kb[m - 1, im:im + 8, :], pi + kb[m - 1, r:r + 8, :]
                else:
                    kr, ki = pr + kb[m - 1, im:im + 8, :], pi - kb[m - 1, r:r + 8, :]
                kst[m * 8:m * 8 + 8, :] = kr
                kst[128 + m * 8:128 + m * 8 + 8, :] = kr + ki
                kst[256 + m * 8:256 + m * 8 + 8, :] = ki - kr

        def macs(p, nxt=None):
            r = p * 8
            kst = kstb[p % 2]
            nb = NA // ab
            for bi, a0 in enumerate(range(0, NA, ab)):
                z = fresh(bi)
                if btoks is not None and btoks[p][bi] is not None:
                    z = gated(btoks[p][bi])
                acc = [[None] * ab for _ in range(3)]
                ncs = a0 + ab
                todo = []
                if nxt is not None and KSPREAD:
                    if bi >= nb - 2:
                        half = bi - (nb - 2)
                        todo = list(range(half * 8, half * 8 + 8))
                for c in range(ncs):
                    if USM:
                        uu = [ub[i, c, pl.ds(z + r, 8), :] for i in (2, 1, 0)]
                    else:
                        u_i, u_r = ub[1, c, pl.ds(z + r, 8), :], ub[0, c, pl.ds(z + r, 8), :]
                        uu = [u_r + u_i, u_i, u_r]
                    for i in range(ab):
                        m = a0 + i - c
                        if m < 0:
                            continue
                        for t in range(3):
                            x = kst[pl.ds(z + t * 128 + m * 8, 8), :] * uu[t]
                            acc[t][i] = x if acc[t][i] is None else acc[t][i] + x
                    if todo and c < 8:
                        kprep(nxt, [todo[c]])
                for i in range(ab):
                    yb[a0 + i, r:r + 8, :] = pltpu.pack_elementwise(
                        [acc[0][i] - acc[1][i], acc[0][i] + acc[2][i]], packed_dtype=BF16)

        plist = list(plist)
        kprep(plist[0])
        for n, p in enumerate(plist):
            nxt = plist[n + 1] if n + 1 < len(plist) else None
            if nxt is not None and not KSPREAD:
                kprep(nxt)
            macs(p, nxt)

    def kprep_all(s, ms):
        kb = kpbuf[s]
        for p in range(16):
            r, im = p * 8, 128 + p * 8
            for m in ms:
                pr, pi = kb[m, r:r + 8, :], kb[m, im:im + 8, :]
                if m == 0:
                    kr, ki = pr, pi
                elif p < 8:
                    kr, ki = pr - kb[m - 1, im:im + 8, :], pi + kb[m - 1, r:r + 8, :]
                else:
                    kr, ki = pr + kb[m - 1, im:im + 8, :], pi - kb[m - 1, r:r + 8, :]
                ksta[p, m * 8:m * 8 + 8, :] = kr
                ksta[p, 128 + m * 8:128 + m * 8 + 8, :] = kr + ki
                ksta[p, 256 + m * 8:256 + m * 8 + 8, :] = ki - kr

    def macs_all(s, a0, ab):
        ub, yb = ubuf[s], ybuf[s]
        for p in range(16):
            r = p * 8
            acc = [[None] * ab for _ in range(3)]
            for c in range(a0 + ab):
                u_i, u_r = ub[1, c, r:r + 8, :], ub[0, c, r:r + 8, :]
                uu = [u_r + u_i, u_i, u_r]
                for i in range(ab):
                    m = a0 + i - c
                    if m < 0:
                        continue
                    for t in range(3):
                        x = ksta[p, t * 128 + m * 8:t * 128 + m * 8 + 8, :] * uu[t]
                        acc[t][i] = x if acc[t][i] is None else acc[t][i] + x
            for i in range(ab):
                yb[a0 + i, r:r + 8, :] = pltpu.pack_elementwise(
                    [acc[0][i] - acc[1][i], acc[0][i] + acc[2][i]], packed_dtype=BF16)

    def idft(j, s, as_=range(NA)):
        as_ = list(as_)
        if BIG:
            z = fresh(48)
            toks = []
            for h in range(2):
                g = _bf(invp[pl.ds(z, 64), h * 128:(h + 1) * 128])
                rhs = jnp.concatenate([_bf(ybuf[s][a, h * 64:(h + 1) * 64, :]) for a in as_], axis=1)
                r = _dot(g, rhs)
                for n, a in enumerate(as_):
                    y2[h, j, a * L:(a + 1) * L, :] = r[:, n * 128:(n + 1) * 128]
                toks += [r[0:8, n * 128:(n + 1) * 128] for n in range(len(as_))]
            return toks
        toks = []
        for a in as_:
            z = fresh(48 + a)
            g0 = _bf(invp[pl.ds(z, 64), 0:128])
            g1 = _bf(invp[pl.ds(z, 64), 128:256])
            r0 = _dot(g0, _bf(ybuf[s][a, 0:64, :]))
            r1 = _dot(g1, _bf(ybuf[s][a, 64:128, :]))
            y2[0, j, a * L:(a + 1) * L, :] = r0
            y2[1, j, a * L:(a + 1) * L, :] = r1
            toks.append(r1[0:8])
        return toks

    def w_transpose(ns=range(15)):
        toks = []
        for n in ns:
            eye = _bf(eyep[pl.ds(fresh(n), 64), :])
            r = _dot_nt(eye, _bf(wqkvw[n]))
            for kt in range(ND):
                wt[kt, n * 128:(n + 1) * 128, :] = r[:, kt * 128:(kt + 1) * 128]
            toks.append(r[0:8, 0:128])
        return toks

    def w_permute(parts=range(3)):
        for p in parts:
            for dh in range(DH):
                for kt in range(ND):
                    rows = wt[kt, pl.ds(p * D + dh, H, stride=DH), :]
                    r0 = (p * D + dh * H) // 2
                    wtp[r0:r0 + H // 2, kt * 128:(kt + 1) * 128] = _u32(rows.astype(BF16))

    def wo_permute():
        for j in range(ND):
            wof[j] = wo_v[j].astype(F32)
        for dh in range(DH):
            for j in range(ND):
                rows = wof[j, pl.ds(dh, H, stride=DH), :]
                r0 = dh * H // 2
                wop[r0:r0 + H // 2, j * 128:(j + 1) * 128] = _u32(rows.astype(BF16))

    def qkv(b, s, fine=False):
        r0 = pl.multiple_of(b * (T // 2), T // 2)
        if MSPLIT > 1:
            h = T // MSPLIT
            rs = []
            for i in range(MSPLIT):
                x = jnp.concatenate([_bf(qw[j, pl.ds(r0 + i * h // 2, h // 2), :]) for j in range(ND)], axis=1)
                r = _dot_nt(x, _bf(wtp[pl.ds(fresh(20 + i), 3 * D // 2), :]))
                for j in range(ND):
                    qp[s][j, i * h:(i + 1) * h, :] = r[:, j * 128:(j + 1) * 128]
                    kp[s][j, HALO + i * h:HALO + (i + 1) * h, :] = r[:, D + j * 128:D + (j + 1) * 128]
                    vp[s][j, HALO + i * h:HALO + (i + 1) * h, :] = r[:, 2 * D + j * 128:2 * D + (j + 1) * 128]
                rs.append(r)
            allt = [rs[i][0:8, n * 128:(n + 1) * 128] * zvec[...] for i in range(MSPLIT) for n in range(15)]
            return [allt[(k * len(allt)) // 15] for k in range(15)]
        x = jnp.concatenate([_bf(qw[j, pl.ds(r0, T // 2), :]) for j in range(ND)], axis=1)
        r = _dot(x, _bf(wnn[...])) if NNW else _dot_nt(x, _bf(wtp[...]))
        for j in range(ND):
            qp[s][j] = r[:, j * 128:(j + 1) * 128]
            kp[s][j, HALO:HALO + T, :] = r[:, D + j * 128:D + (j + 1) * 128]
            vp[s][j, HALO:HALO + T, :] = r[:, 2 * D + j * 128:2 * D + (j + 1) * 128]
        if fine:
            return [r[64 * i:64 * i + 8, n * 128:(n + 1) * 128] * zvec[...] for n in range(15) for i in range(4)]
        return [r[0:8, n * 128:(n + 1) * 128] * zvec[...] for n in range(15)]

    def qkv_half(b, s, i):
        h = T // 2
        r0 = b * (T // 2) + i * (h // 2)
        x = jnp.concatenate([_bf(qw[j, r0:r0 + h // 2, :]) for j in range(ND)], axis=1)
        r = _dot_nt(x, _bf(wtp[pl.ds(fresh(20 + i), 3 * D // 2), :]))
        for j in range(ND):
            qp[s][j, i * h:(i + 1) * h, :] = r[:, j * 128:(j + 1) * 128]
            kp[s][j, HALO + i * h:HALO + (i + 1) * h, :] = r[:, D + j * 128:D + (j + 1) * 128]
            vp[s][j, HALO + i * h:HALO + (i + 1) * h, :] = r[:, 2 * D + j * 128:2 * D + (j + 1) * 128]
        return [r[0:8, n * 128:(n + 1) * 128] * zvec[...] for n in range(15)]

    def gate(b, s, mt=None):
        r0 = pl.multiple_of(b * T, T)
        for g in range(NG):
            sm = None if mt is None else jnp.concatenate([mt[(g * GN) // NG]] * (GR // 8), axis=0)
            for j in range(ND):
                t = _bmul(qbuf[j, pl.ds(r0 + g * GR, GR), :].astype(F32), par[j, 5])
                sm = t if sm is None else sm + t
            hi = sm.astype(BF16)
            gsp[0, g * GR // 2:(g + 1) * GR // 2, :] = _u32(hi)
            if GLO:
                lo = (sm - hi.astype(F32)).astype(BF16)
                gsp[1, g * GR // 2:(g + 1) * GR // 2, :] = _u32(lo)
        ones = _bf(onesp[...])
        glog[s][0] = _dot(_bf(gsp[0]), ones)
        if GLO:
            glog[s][1] = _dot(_bf(gsp[1]), ones)

    def halo(s):
        for j in range(ND):
            kp[1 - s][j, 0:HALO, :] = kp[s][j, T:T + HALO, :]
            vp[1 - s][j, 0:HALO, :] = vp[s][j, T:T + HALO, :]

    def softmax_pv(vv, row, ob, lg=None):
        if lg is None:
            lg = [lbuf[w, row:row + GR, :] for w in range(8)]
        m = lg[0]
        for w in range(1, 8):
            m = jnp.maximum(m, lg[w])
        es = [(l - m) if E('NOEXP', '0') == '1' else jnp.exp2(l - m) for l in lg]
        sm = es[0]
        for w in range(1, 8):
            sm = sm + es[w]
        inv = 1.0 / sm
        for j in range(ND):
            acc = None
            for w in range(8):
                o = row + HALO - 2 * w
                t = es[w] * vv[j, o:o + GR, :]
                acc = t if acc is None else acc + t
            res = acc * inv
            ob[row // 2:(row + GR) // 2, j * 128:(j + 1) * 128] = _u32(res.astype(BF16))
        return res[0:8]

    def qk(qq, kk, row, tok):
        if tok is None:
            q = [qq[j, row:row + GE, :] * QSCALE for j in range(ND)]
        else:
            sc = tok + QSCALE
            q = [_bmul(qq[j, row:row + GE, :], sc) for j in range(ND)]
        out = []
        for w in range(8):
            p = None
            o = row + HALO - 2 * w
            for j in range(ND):
                t = q[j] * kk[j, o:o + GE, :]
                p = t if p is None else p + t
            out.append(p)
        return out

    def attention(b, s, mt=None, row0=0, nrows=T, an=AN, ob=None):
        qq, kk, vv = qp[s], kp[s], vp[s]
        ob = op if ob is None else ob
        g0 = row0 // GE
        n1 = g0 + nrows // GE
        per = GR // GE
        r1, r2, done = {}, {}, {}
        for g in range(g0, n1 + D3 + per):
            if g < n1:
                row = g * GE
                tok = None
                if mt is not None:
                    tok = mt[((g - g0) * an) // (n1 - g0)]
                    prev = done.get(row // GR - PACE) if PACE else None
                    if prev is not None:
                        tok = tok + prev * zvec[...]
                r1[g] = []
                for w, p in enumerate(qk(qq, kk, row, tok)):
                    pbuf[w, row:row + GE, :] = p
                    r1[g].append(p * 2.0 if E('NOROLL', '0') == '1' else pltpu.roll(p, 64, 1))
            gg = g - D1
            if g0 <= gg < n1:
                row = gg * GE
                r2[gg] = []
                for w, r in enumerate(r1.pop(gg)):
                    sm = pbuf[w, row:row + GE, :] + r
                    sbuf[w, row:row + GE, :] = sm
                    r2[gg].append(sm * 2.0 if E('NOROLL', '0') == '1' else pltpu.roll(sm, 32, 1))
            gg = g - D2
            if g0 <= gg < n1:
                row = gg * GE
                ls = []
                for w, r in enumerate(r2.pop(gg)):
                    l = sbuf[w, row:row + GE, :] + r
                    if row < HALO and w > 0:
                        t = b * T + row + jax.lax.broadcasted_iota(jnp.int32, (GE, 128), 0)
                        l = jnp.where(t >= 2 * w, l, MASKED)
                    if NOLBUF:
                        ls.append(l)
                    else:
                        lbuf[w, row:row + GE, :] = l
                if NOLBUF:
                    done[row // GR] = softmax_pv(vv, row, ob, ls)
            gg = g - D3
            if not NOLBUF and g0 <= gg < n1 and (gg + 1) % per == 0:
                row = (gg + 1 - per) * GE
                done[row // GR] = softmax_pv(vv, row, ob)

    def outproj(s, r0=0, n=T, ob=None):
        ob = op if ob is None else ob
        r = _dot(_bf(ob[r0 // 2:(r0 + n) // 2, :]), _bf(wop[...]))
        bres[s][r0:r0 + n, :] = r
        return [r[0:8, k * 128:(k + 1) * 128] * zvec[...] for k in range(ND)]

    def epilogue(b, s, mt=None, gs=range(NG)):
        r0 = pl.multiple_of(b * T, T)
        for g in gs:
            row = r0 + g * GR
            rowh = pl.multiple_of(b * (T // 2), T // 2) + g * (GR // 2)
            gl = glog[s][0, g * GR:(g + 1) * GR, :]
            if GLO:
                gl = gl + glog[s][1, g * GR:(g + 1) * GR, :]
            if mt is not None:
                gl = _badd(gl, mt[(g * EN) // NG])
            gt = jax.nn.sigmoid(gl)
            for j in range(ND):
                q = qbuf[j, pl.ds(row, GR), :].astype(F32)
                kv = _bf(kvp[j, pl.ds(rowh, GR // 2), :]).astype(F32)
                z = y2[0, j, pl.ds(row, GR), :] + y2[1, j, pl.ds(row, GR), :] + _bmul(kv, par[j, 4])
                bb = bres[s][g * GR:(g + 1) * GR, j * 128:(j + 1) * 128]
                o = bb + gt * (q * z - bb)
                obuf[b % NOB, j, g * GR:(g + 1) * GR, :] = o.astype(BF16)

    def region(k, f):
        pl.when(zsm[k % 64] == 0)(f)

    P = functools.partial

    wq_0, wq_1, wq_b = _Copies(wqkv_copy.cs[:WQ0]), _Copies(wqkv_copy.cs[WQ0:8]), _Copies(wqkv_copy.cs[8:])
    wq_a = _Copies(wqkv_copy.cs[:8])

    def x_dma(j):
        with _scope("waitX%d" % j):
            if STREAM and j == 0:
                kv_copy(1).wait()
            if not (STREAM and j == 0):
                sk_copy(j + 1).wait()
            if j >= 2 or (j == 1 and not STREAM):
                kv_copy(j + 1).wait()
        if j == 0:
            kv_copy(2).start()
            if not STREAM:
                sk_copy(2).start()
        if j == 1:
            kv_copy(3).start()
            sk_copy(3).start()
        if j == 2:
            kv_copy(4).start()
            sk_copy(4).start()
            wq_0.start()
        if j == 3:
            _Copies(wqkv_copy.cs[WQ0:]).start()
            q_copy(0).start()

    def block_x(j):
        s = j % 2
        late_kv = STREAM and j == 1
        if not (STREAM and j == 0):
            with _scope("X%d" % j):
                if j >= 1 and not late_kv:
                    kvprep(j + 1)
                aconv(s)
                if j >= 1:
                    idft(j - 1, 1 - s)
                dft_k(j + 1, 1 - s)
                if j >= 1 and not late_kv:
                    dft_u(j + 1, 1 - s)
        if j == 0 or late_kv:
            if not (STREAM and j == 0):
                with _scope("waitK%d" % (j + 1)):
                    kv_copy(j + 1).wait()
            with _scope("Y%d" % j):
                kvprep(j + 1)
                dft_u(j + 1, 1 - s)

    def body_a(j, carry):
        return carry

    def b_dma(b, s):
        if ONLY == '':
            q_copy(b).wait()

        @pl.when(b - 2 >= NOB)
        def _():
            out_copy(b - 2 - NOB).wait()

    def epilogue_wait(t):
        if t >= NOB:
            out_copy(t - NOB).wait()

    def block_b(b, s, dma=True):
        if dma:
            b_dma(b, s)
        with _scope("B"):
            halo(1 - s)
            mt = qkv(b, s)
            if EPI == 'paced':
                epilogue(b - 2, s, mt)
            elif EPI == 'free':
                epilogue(b - 2, s)
            elif EPI == 'late':
                epilogue(b - 2, s, [mt[14]] * 15)
            if EPI != 'after':
                out_copy(b - 2).start()
            if E('NOATT', '0') != '1':
                attention(b - 1, 1 - s, mt)
            if E('NOGATE', '0') != '1':
                gate(b - 1, 1 - s, mt if GATEP else None)
            if EPI == 'after':
                ot = outproj(1 - s)
                epilogue(b - 2, s, [ot[(g * 5) // 15] for g in range(15)])
                out_copy(b - 2).start()
            else:
                outproj(1 - s)

    def body_b2(i, carry):
        b = 2 * i
        if ONLY == '':
            q_copy(b).wait()
            q_copy(b + 1).wait()

        @pl.when(b - 2 >= NOB)
        def _():
            out_copy(b - 2 - NOB).wait()
            out_copy(b - 1 - NOB).wait()
        block_b(b, 0, False)
        block_b(b + 1, 1, False)
        return carry

    def body_b(b, carry):
        if E('ONEPAR', '0') == '1':
            block_b(b, 0)
            return carry
        for s in range(2):
            pl.when(b % 2 == s)(functools.partial(block_b, b, s))
        return carry

    if ONLY != 'B':
        nb = NA // NCH
        for ch in range(NCH):
            with _scope("wait0"):
                first_copy(ch).wait()
            if ch == 1:
                sk_copy(1).start()
            if ch == NCH - 1:
                kv_copy(1).start()
            with _scope("pro"):
                blks = range(ch * nb, (ch + 1) * nb)
                if STREAM and ch >= 1:
                    prev = range((ch - 1) * nb, ch * nb)
                    kprep_all(0, prev)
                    macs_all(0, (ch - 1) * nb, nb)
                kvprep(0, blks)
                dft_k(0, 0, blks)
                dft_u(0, 0, blks)
        if STREAM:
            with _scope("wait0"):
                sk_copy(1).wait()
            sk_copy(2).start()
            with _scope("pro2"):
                kprep_all(0, range((NCH - 1) * nb, NA))
                macs_all(0, (NCH - 1) * nb, nb)
                dft_k(1, 1)

        for j in range(ND - 1):
            x_dma(j)
            region(2 * j, P(block_x, j))

    if ONLY == '':
        q_copy(0).wait()
        if WLATE:
            wqkv_copy.wait()
            wo_copy.start()
            q_copy(1).start()
        for b in range(2, NT):
            q_copy(b).start()

        def block_wlate():
            with _scope("Alast0"):
                aconv((ND - 1) % 2)
                idft(ND - 2, (ND - 2) % 2)
                w_transpose()
                if AMERGE >= 1:
                    w_permute([0] if AMERGE == 1 else [0, 1, 2])
                if AMERGE == 3:
                    qkv(0, 0)

        if WLATE:
            region(12, block_wlate)

        def block_alast():
            if WLATE:
                with _scope("Alast"):
                    if AMERGE == 3:
                        return
                    w_permute({0: [0, 1, 2], 1: [1, 2], 2: []}[AMERGE])
                    qkv(0, 0)
                return
            with _scope("Alast"):
                w_permute([1, 2] if PERM_EARLY else [0, 1, 2])
                if Q0 == 3:
                    idft(ND - 2, (ND - 2) % 2)
                    mt = qkv(0, 0, True)
                    wts = [sum(a + 1 for a in range(a0, a0 + LAB)) for a0 in range(0, NA, LAB)]
                    tot = 136 * 16
                    bt, cum = [], 0
                    for p in range(16):
                        row = []
                        for bi in range(len(wts)):
                            k = (cum * LN * len(mt)) // (tot * 16) - LOFF
                            row.append(mt[min(k, len(mt) - 1)] if k >= 0 else None)
                            cum += wts[bi]
                        bt.append(row)
                    aconv((ND - 1) % 2, range(16), btoks=bt, ab=LAB)
                elif Q0 == 2:
                    idft(ND - 2, (ND - 2) % 2)
                    mt = qkv(0, 0)
                    toks = [None] + [mt[min(14, ((p - 1) * LN) // 16)] for p in range(1, 16)]
                    aconv((ND - 1) % 2, range(16), toks, tz=False)
                else:
                    aconv((ND - 1) % 2)
                    idft(ND - 2, (ND - 2) % 2)
                    if Q0:
                        qkv(0, 0)

        region(10, block_alast)

        def block_b1():
            q_copy(1).wait()
            wo_copy.wait()
            with _scope("B1"):
                wo_permute()
                if not Q0:
                    qkv(0, 0)
                idft(ND - 1, (ND - 1) % 2)
                halo(0)
                mt = qkv(1, 1)
                attention(0, 0, mt)
                gate(0, 0, mt)
                outproj(0)

        region(11, block_b1)

    if ONLY != 'A':
        if PAIR:
            jax.lax.fori_loop(1, NT // 2, body_b2, 0)
        else:
            jax.lax.fori_loop(2, NT - 1 if (LASTB and ONLY == '') else NT, body_b, 0)

    if ONLY == '':
        if LASTB:
            def block_last():
                b, s = NT - 1, (NT - 1) % 2
                q_copy(b).wait()
                epilogue_wait(b - 2)
                with _scope("B7"):
                    halo(1 - s)
                    m1 = qkv_half(b, s, 0)
                    m2 = qkv_half(b, s, 1)
                    epilogue(b - 2, s, [m2[14]] * 15)
                    out_copy(b - 2).start()
                    attention(b - 1, 1 - s, m1 + m2, an=LAN1)
                    gate(b - 1, 1 - s, m1)
                    attention(b, s, m2, 0, T // 2, an=LAN2, ob=op2)
                    outproj(1 - s)

            region(13, block_last)
            with _scope("fin1"):
                epilogue_wait(NT - 2)
                epilogue_wait(NT - 1)
                epilogue(NT - 2, 0)
                out_copy(NT - 2).start()
                gate(NT - 1, 1)
                attention(NT - 1, 1, None, T // 2, T // 2, ob=op2)
                nh = T // FSPLIT
                for h in range(FSPLIT):
                    outproj(1, h * nh, nh, op2)
                for h in range(FSPLIT):
                    epilogue(NT - 1, 1, None, range(h * nh // GR, (h + 1) * nh // GR))
                    out_copy(NT - 1, h * nh, nh).start()
        elif FSPLIT:
            with _scope("fin1"):
                epilogue_wait(NT - 2)
                epilogue_wait(NT - 1)
                epilogue(NT - 2, 0)
                out_copy(NT - 2).start()
                gate(NT - 1, 1)
                attention(NT - 1, 1)
                nh = T // FSPLIT
                for h in range(FSPLIT):
                    outproj(1, h * nh, nh)
                for h in range(FSPLIT):
                    epilogue(NT - 1, 1, None, range(h * nh // GR, (h + 1) * nh // GR))
                    out_copy(NT - 1, h * nh, nh).start()
        else:
            with _scope("fin1"):
                epilogue_wait(NT - 2)
                epilogue(NT - 2, 0)
                out_copy(NT - 2).start()
                attention(NT - 1, 1)
                gate(NT - 1, 1)
                outproj(1)
            with _scope("fin2"):
                epilogue_wait(NT - 1)
                epilogue(NT - 1, 1)
                out_copy(NT - 1).start()
        with _scope("fin3"):
            for t in range(NT - NOB, NT):
                out_copy(t).wait()
    elif ONLY == 'B':
        for t in range(NT - 2 - NOB, NT - 2):
            out_copy(t).wait()
    else:
        for b in range(2):
            q_copy(b).wait()
        wo_copy.wait()


@jax.jit
def pallas_gated_mix__ssm_conv_h3__sliding_local_dilated__prompt_kernel(A_q, A_k, A_v, A_shift_k, A_ssm_k, A_ssm_D, B_x, B_wqkv, B_wo, gate_w):
    fwd, inv, eye = _dft_constants()
    hbm = pl.BlockSpec(memory_space=pl.ANY)
    vm = pl.BlockSpec(memory_space=pltpu.VMEM)
    two = lambda shape, dt: [pltpu.VMEM(shape, dt), pltpu.VMEM(shape, dt)]
    return pl.pallas_call(
        _kernel,
        out_shape=jax.ShapeDtypeStruct((1, S, D), BF16),
        in_specs=[hbm] * 12,
        out_specs=hbm,
        scratch_shapes=[
            pltpu.VMEM((4, D), BF16),
            pltpu.VMEM((D,), BF16),
            pltpu.VMEM((D,), BF16),
            pltpu.VMEM((384, 128), BF16),
            pltpu.VMEM((128, 256), BF16),
            pltpu.VMEM((128, 128), BF16),
            pltpu.VMEM((ND, 2 * KH + S, 128), BF16),
            pltpu.VMEM((ND, S, 128), BF16),
            pltpu.VMEM((ND, NA, 128, L), BF16),
            pltpu.VMEM((ND, S, 128), BF16),
            pltpu.VMEM((15, D, 128), BF16),
            pltpu.VMEM((ND, D, 128), BF16),
            pltpu.VMEM((ND, 6, 8, 128), F32),
            pltpu.VMEM((8, 128), F32),
            pltpu.SMEM((64,), jnp.int32),
            pltpu.VMEM((192, 128), U32),
            pltpu.VMEM((64, 256), U32),
            pltpu.VMEM((64, 128), U32),
            pltpu.VMEM((64, 128), U32),
            pltpu.VMEM((ND, S // 2, 128), U32),
            *two((3, NA, 128, 128), F32),
            *two((NA, 256, 128), F32),
            *two((NA, 128, 128), U32),
            *two((384, 128), F32),
            pltpu.VMEM((16, 384, 128), F32),
            pltpu.VMEM((2, ND, S, 128), F32),
            pltpu.VMEM((ND, 3 * D, 128), F32),
            pltpu.VMEM((3 * D // 2, D), U32),
            pltpu.VMEM((D // 2, 3 * D), U32),
            pltpu.VMEM((ND, D, 128), F32),
            pltpu.VMEM((D // 2, D), U32),
            *two((ND, T, 128), F32),
            *two((ND, HALO + T, 128), F32),
            *two((ND, HALO + T, 128), F32),
            pltpu.VMEM((8, T, 128), F32),
            pltpu.VMEM((8, T, 128), F32),
            pltpu.VMEM((8, T, 128), F32),
            pltpu.VMEM((T // 2, D), U32),
            pltpu.VMEM((T // 2, D), U32),
            *two((T, D), F32),
            pltpu.VMEM((NOB, ND, T, 128), BF16),
            pltpu.VMEM((2, T // 2, 128), U32),
            *two((2, T, 128), F32),
            pltpu.SemaphoreType.DMA((3 * ND,)),
            pltpu.SemaphoreType.DMA((NT,)),
            pltpu.SemaphoreType.DMA((2,)),
            pltpu.SemaphoreType.DMA((NOB,)),
            pltpu.SemaphoreType.DMA((6,)),
            pltpu.SemaphoreType.DMA((NCH,)),
        ],
        compiler_params=pltpu.CompilerParams(vmem_limit_bytes=100 * 2 ** 20),
    )(A_q, A_k, A_v, A_shift_k.T, A_ssm_k, A_ssm_D, B_wqkv, B_wo, gate_w,
      jnp.asarray(fwd, BF16), jnp.asarray(inv, BF16), jnp.asarray(eye, BF16))
```

```python
import contextlib
import functools
import numpy as np
import jax
import jax.numpy as jnp
from jax.experimental import pallas as pl
from jax.experimental.pallas import tpu as pltpu


def E(key, default):
    return default


ONLY = E('ONLY', '')
SCOPES = int(E('SCOPES', '0'))
AN, EN, GN, PACE = int(E('AN', '13')), int(E('EN', '14')), int(E('GN', '10')), int(E('PACE', '4'))
D1, D2, D3 = int(E('D1', '2')), int(E('D2', '4')), int(E('D3', '5'))
DYNZ = int(E('DYNZ', '0'))
AB = int(E('AB', '4'))
ATOK = int(E('ATOK', '0'))
AOFF = int(E('AOFF', '1'))
ARATE = int(E('ARATE', '100'))
AORD = E('AORD', 'cf')
FR = int(E('FR', '100'))
USM = int(E('USM', '0'))
MERGE = int(E('MERGE', '0'))
KVFIRST = int(E('KVFIRST', '1'))
KSPLIT = int(E('KSPLIT', '8'))

WT_AT = int(E('WT_AT', '2'))
LN = int(E('LN', '15'))
EPI = E('EPI', 'late')
GATEP = int(E('GATEP', '1'))
NNW = int(E('NNW', '0'))
LOFF = int(E('LOFF', '0'))
LAB = int(E('LAB', '2'))
KVPOS = E('KVPOS', 'post')
TFIRST = int(E('TFIRST', '0'))
KVT = [int(x) for x in E('KVT', '-1,-1,-1').split(',')]
GATE = E('GATE', 'mem')
BIG = int(E('BIG', '0'))
KSPREAD = int(E('KSPREAD', '1'))
PAIR = int(E('PAIR', '0'))
NOB = 4
FSPLIT = int(E('FSPLIT', '4'))
PERM_EARLY = int(E('PERM_EARLY', '1'))
WQ0 = int(E('WQ0', '4'))
WLATE = int(E('WLATE', '1'))
KVFIRST2 = int(E('KVFIRST2', '0'))
NOLBUF = int(E('NOLBUF', '0'))
MSPLIT = int(E('MSPLIT', '1'))
AMERGE = int(E('AMERGE', '0'))
LASTB = int(E('LASTB', '1'))
LAN1 = int(E('LAN1', '24'))
LAN2 = int(E('LAN2', '14'))
GLO = int(E('GLO', '0'))
KVG = int(E('KVG', '4'))
STREAM = int(E('STREAM', '1'))
PROSPLIT = int(E('PROSPLIT', '1'))
XSPLIT = int(E('XSPLIT', '1'))
KVI = int(E('KVI', '8'))
DMAREG = int(E('DMAREG', '1'))
WSPLIT = int(E('WSPLIT', '0'))
NCH = int(E('NCH', '4'))
Q0 = int(E('Q0', '1'))
S, D = 2048, 640
ND = 5
L = 128
NA = S // L
T = 256
NT = S // T
H, DH = 32, 20
HALO = 16
KH = 8
GR = 16
GE = int(E('GE', '8'))
NG = T // GR
LOG2E = 1.4426950408889634
QSCALE = float(DH ** -0.5) * LOG2E
MASKED = -1e9 * LOG2E
F32, BF16, U32 = jnp.float32, jnp.bfloat16, jnp.uint32


def _scope(name):
    return jax.named_scope(name) if SCOPES else contextlib.nullcontext()


def _dft_constants():
    forder = np.concatenate([np.arange(0, 128, 2), np.arange(1, 128, 2)])
    th = np.pi * (2 * forder + 1) / 256.0
    b = np.arange(128)
    fre, fim = np.cos(np.outer(th, b)), -np.sin(np.outer(th, b))
    fwd = np.concatenate([fre, fim, fre + fim], 0)
    gre = np.cos(np.outer(b, th)) / 128
    gim = -np.sin(np.outer(b, th)) / 128
    inv = np.stack([gre, gim], -1).reshape(128, 256)
    return fwd.astype(np.float32), inv.astype(np.float32), np.eye(128, dtype=np.float32)


def _bf(x):
    return pltpu.bitcast(x, BF16)


def _u32(x):
    return pltpu.bitcast(x, U32)


def _bmul(x, t8):
    return (x.reshape(-1, 8, 128) * t8).reshape(x.shape)


def _badd(x, t8):
    return (x.reshape(-1, 8, 128) + t8).reshape(x.shape)


def _dot(a, b):
    return jnp.dot(a, b, preferred_element_type=F32)


def _dot_nt(a, b):
    return jax.lax.dot_general(a, b, (((1,), (1,)), ((), ())), preferred_element_type=F32)


class _Copies:
    def __init__(self, cs):
        self.cs = list(cs)

    def start(self):
        for c in self.cs:
            c.start()

    def wait(self):
        for c in self.cs:
            c.wait()


def _kernel(q_hbm, k_hbm, v_hbm, shk_hbm, sk_hbm, dvec_hbm, wqkv_hbm, wo_hbm, gw_hbm,
            fwd_hbm, inv_hbm, eye_hbm,
            out_hbm,
            shk_ref, dvec_ref, gw_ref, fwd_ref, inv_ref, eye_ref,
            kbuf, vbuf, skbuf, qbuf, wqkv_v, wo_v, par, zvec, zsm, fwdp, invp, onesp, eyep,
            kvp, ubuf0, ubuf1, kpbuf0, kpbuf1, ybuf0, ybuf1, kst0, kst1, ksta, y2, wt, wtp, wnn, wof, wop,
            qp0, qp1, kp0, kp1, vp0, vp1, pbuf, sbuf, lbuf, op, op2, bres0, bres1, obuf, gsp, glog0, glog1,
            sem_a, sem_q, sem_w, sem_o, sem_s, sem_f):
    ubuf, kpbuf, ybuf, kstb = (ubuf0, ubuf1), (kpbuf0, kpbuf1), (ybuf0, ybuf1), (kst0, kst1)
    qp, kp, vp = (qp0, qp1), (kp0, kp1), (vp0, vp1)
    bres, glog = (bres0, bres1), (glog0, glog1)
    skw, qw, wqkvw = skbuf.bitcast(U32), qbuf.bitcast(U32), wqkv_v.bitcast(U32)
    kw, vw = kbuf.bitcast(U32), vbuf.bitcast(U32)

    def kv_copy(j):
        return _Copies(
            [pltpu.make_async_copy(k_hbm.at[0, :, pl.ds(j * 128, 128)], kbuf.at[j, pl.ds(2 * KH, S)], sem_a.at[3 * j]),
             pltpu.make_async_copy(v_hbm.at[0, :, pl.ds(j * 128, 128)], vbuf.at[j], sem_a.at[3 * j + 1])])

    def sk_copy(j):
        return _Copies(pltpu.make_async_copy(sk_hbm.at[pl.ds(j * 128, 128), pl.ds(m * L, L)], skbuf.at[j, m],
                                             sem_a.at[3 * j + 2]) for m in range(NA))

    def slab_copy(j):
        return _Copies(kv_copy(j).cs + sk_copy(j).cs)

    def first_copy(ch):
        rows = pl.ds(ch * (S // NCH), S // NCH)
        ms = range(ch * (NA // NCH), (ch + 1) * (NA // NCH))
        return _Copies(
            [pltpu.make_async_copy(k_hbm.at[0, rows, pl.ds(0, 128)],
                                   kbuf.at[0, pl.ds(2 * KH + ch * (S // NCH), S // NCH)], sem_f.at[ch]),
             pltpu.make_async_copy(v_hbm.at[0, rows, pl.ds(0, 128)], vbuf.at[0, rows], sem_f.at[ch])]
            + [pltpu.make_async_copy(sk_hbm.at[pl.ds(0, 128), pl.ds(m * L, L)], skbuf.at[0, m], sem_f.at[ch])
               for m in ms])

    small_copy = _Copies(pltpu.make_async_copy(a, b, sem_s.at[i]) for i, (a, b) in enumerate(
        [(shk_hbm, shk_ref), (dvec_hbm, dvec_ref), (gw_hbm, gw_ref), (fwd_hbm, fwd_ref), (inv_hbm, inv_ref),
         (eye_hbm, eye_ref)]))
    def q_copy(b):
        rows = pl.ds(b * T, T)
        return _Copies(pltpu.make_async_copy(q_hbm.at[0, rows, pl.ds(j * 128, 128)], qbuf.at[j, rows], sem_q.at[b])
                       for j in range(ND))

    wqkv_copy = _Copies(pltpu.make_async_copy(wqkv_hbm.at[:, pl.ds(n * 128, 128)], wqkv_v.at[n], sem_w.at[0])
                        for n in range(15))
    wo_copy = _Copies(pltpu.make_async_copy(wo_hbm.at[:, pl.ds(n * 128, 128)], wo_v.at[n], sem_w.at[1])
                      for n in range(ND))

    def out_copy(b, r0=0, n=T):
        return _Copies(pltpu.make_async_copy(obuf.at[b % NOB, j, pl.ds(r0, n)],
                                             out_hbm.at[0, pl.ds(b * T + r0, n), pl.ds(j * 128, 128)],
                                             sem_o.at[b % NOB]) for j in range(ND))

    for j in range(ND):
        kbuf[j, 0:2 * KH, :] = jnp.zeros((2 * KH, 128), BF16)
    with _scope("s_issue"):
        small_copy.start()
        if ONLY != 'B':
            first_copy(0).start()
    with _scope("s_wait"):
        small_copy.wait()
    if ONLY != 'B':
        for ch in range(1, NCH):
            first_copy(ch).start()

    with _scope("s_setup"):
        taps = shk_ref[...].astype(F32)
        dv = dvec_ref[...].astype(F32).reshape(1, D)
        gw = gw_ref[...].astype(F32).reshape(1, D)
        for j in range(ND):
            for i in range(4):
                par[j, i] = jnp.broadcast_to(taps[i:i + 1, j * 128:(j + 1) * 128], (8, 128))
            par[j, 4] = jnp.broadcast_to(dv[:, j * 128:(j + 1) * 128], (8, 128))
            par[j, 5] = jnp.broadcast_to(gw[:, j * 128:(j + 1) * 128], (8, 128))
        zvec[...] = jnp.zeros((8, 128), F32)
        for i in range(64):
            zsm[i] = 0
        fwdp[...] = _u32(fwd_ref[...])
        invp[...] = _u32(inv_ref[...])
        eyep[...] = _u32(eye_ref[...])
        onesp[...] = _u32(jnp.ones((128, 128), BF16))
        for j in range(ND):
            kp0[j, 0:HALO, :] = jnp.zeros((HALO, 128), F32)
            vp0[j, 0:HALO, :] = jnp.zeros((HALO, 128), F32)

    def fresh(i):
        return pl.multiple_of(zsm[i] * 8, 8)

    def gated(tok):
        i = tok[0, 0].astype(jnp.int32)
        return pl.multiple_of(jnp.minimum(jnp.maximum(i, zsm[62]), zsm[63]) * 8, 8)

    def kvprep(j, blks=range(NA), tok=None):
        t = [par[j, i] if tok is None else par[j, i] + tok * zvec[...] for i in range(4)]
        even = lambda w: pltpu.bitcast(w << 16, F32)
        odd = lambda w: pltpu.bitcast(w & jnp.uint32(0xFFFF0000), F32)
        for c in blks:
            for q in range(L // 32):
                r = c * (L // 2) + q * 16
                w0 = kw[j, KH + r:KH + r + 16, :]
                w1 = kw[j, KH + r - 1:KH + r + 15, :]
                w2 = kw[j, KH + r - 2:KH + r + 14, :]
                e0, o0, e1, o1, o2 = even(w0), odd(w0), even(w1), odd(w1), odd(w2)
                ks_e = _bmul(e0, t[0]) + _bmul(o1, t[1]) + _bmul(e1, t[2]) + _bmul(o2, t[3])
                ks_o = _bmul(o0, t[0]) + _bmul(e0, t[1]) + _bmul(o1, t[2]) + _bmul(e1, t[3])
                wv = vw[j, r:r + 16, :]
                pe = ks_e * even(wv)
                kvp[j, r:r + 16, :] = pltpu.pack_elementwise([pe, ks_o * odd(wv)], packed_dtype=BF16)
        return pe[0:8]

    def dft_u(j, s, cs=range(NA)):
        cs = list(cs)
        if BIG:
            f = _bf(fwdp[pl.ds(fresh(16), 192 if USM else 128), :])
            rhs = jnp.concatenate([_bf(kvp[j, c * 64:(c + 1) * 64, :]) for c in cs], axis=1)
            r = _dot(f, rhs)
            for n, c in enumerate(cs):
                for i in range(3 if USM else 2):
                    ubuf[s][i, c] = r[i * 128:(i + 1) * 128, n * 128:(n + 1) * 128]
            return [r[0:8, n * 128:(n + 1) * 128] for n in range(len(cs))]
        toks = []
        for c in cs:
            f = _bf(fwdp[pl.ds(fresh(16 + c), 192 if USM else 128), :])
            r = _dot(f, _bf(kvp[j, c * 64:(c + 1) * 64, :]))
            for i in range(3 if USM else 2):
                ubuf[s][i, c] = r[i * 128:(i + 1) * 128]
            toks.append(r[0:8])
        return toks

    def dft_k(j, s, ms=range(NA)):
        ms = list(ms)
        if BIG:
            f = _bf(fwdp[pl.ds(fresh(32), 128), :])
            rhs = jnp.concatenate([_bf(skw[j, m]) for m in ms], axis=0)
            r = _dot_nt(f, rhs)
            for n, m in enumerate(ms):
                kpbuf[s][m] = r[:, n * 128:(n + 1) * 128]
            return [r[0:8, n * 128:(n + 1) * 128] for n in range(len(ms))]
        toks = []
        for m in ms:
            f = _bf(fwdp[pl.ds(fresh(32 + m), 128), :])
            r = _dot_nt(f, _bf(skw[j, m]))
            kpbuf[s][m] = r
            toks.append(r[0:8])
        return toks

    def aconv(s, plist=range(16), toks=None, mode=None, tz=True, btoks=None, ab=AB):
        ub, kb, yb = ubuf[s], kpbuf[s], ybuf[s]

        def kprep(p, ms=range(NA)):
            r, im = p * 8, 128 + p * 8
            kst = kstb[p % 2]
            for m in ms:
                pr, pi = kb[m, r:r + 8, :], kb[m, im:im + 8, :]
                if m == 0:
                    kr, ki = pr, pi
                    if toks is not None and toks[p] is not None:
                        kr = kr + (toks[p] * zvec[...] if tz else toks[p])
                elif p < 8:
                    kr, ki = pr - kb[m - 1, im:im + 8, :], pi + kb[m - 1, r:r + 8, :]
                else:
                    kr, ki = pr + kb[m - 1, im:im + 8, :], pi - kb[m - 1, r:r + 8, :]
                kst[m * 8:m * 8 + 8, :] = kr
                kst[128 + m * 8:128 + m * 8 + 8, :] = kr + ki
                kst[256 + m * 8:256 + m * 8 + 8, :] = ki - kr

        def macs(p, nxt=None):
            r = p * 8
            kst = kstb[p % 2]
            nb = NA // ab
            for bi, a0 in enumerate(range(0, NA, ab)):
                z = fresh(bi)
                if btoks is not None and btoks[p][bi] is not None:
                    z = gated(btoks[p][bi])
                acc = [[None] * ab for _ in range(3)]
                ncs = a0 + ab
                todo = []
                if nxt is not None and KSPREAD:
                    if bi >= nb - 2:
                        half = bi - (nb - 2)
                        todo = list(range(half * 8, half * 8 + 8))
                for c in range(ncs):
                    if USM:
                        uu = [ub[i, c, pl.ds(z + r, 8), :] for i in (2, 1, 0)]
                    else:
                        u_i, u_r = ub[1, c, pl.ds(z + r, 8), :], ub[0, c, pl.ds(z + r, 8), :]
                        uu = [u_r + u_i, u_i, u_r]
                    for i in range(ab):
                        m = a0 + i - c
                        if m < 0:
                            continue
                        for t in range(3):
                            x = kst[pl.ds(z + t * 128 + m * 8, 8), :] * uu[t]
                            acc[t][i] = x if acc[t][i] is None else acc[t][i] + x
                    if todo and c < 8:
                        kprep(nxt, [todo[c]])
                for i in range(ab):
                    yb[a0 + i, r:r + 8, :] = pltpu.pack_elementwise(
                        [acc[0][i] - acc[1][i], acc[0][i] + acc[2][i]], packed_dtype=BF16)

        plist = list(plist)
        kprep(plist[0])
        for n, p in enumerate(plist):
            nxt = plist[n + 1] if n + 1 < len(plist) else None
            if nxt is not None and not KSPREAD:
                kprep(nxt)
            macs(p, nxt)

    def kprep_all(s, ms):
        kb = kpbuf[s]
        for p in range(16):
            r, im = p * 8, 128 + p * 8
            for m in ms:
                pr, pi = kb[m, r:r + 8, :], kb[m, im:im + 8, :]
                if m == 0:
                    kr, ki = pr, pi
                elif p < 8:
                    kr, ki = pr - kb[m - 1, im:im + 8, :], pi + kb[m - 1, r:r + 8, :]
                else:
                    kr, ki = pr + kb[m - 1, im:im + 8, :], pi - kb[m - 1, r:r + 8, :]
                ksta[p, m * 8:m * 8 + 8, :] = kr
                ksta[p, 128 + m * 8:128 + m * 8 + 8, :] = kr + ki
                ksta[p, 256 + m * 8:256 + m * 8 + 8, :] = ki - kr

    def macs_all(s, a0, ab):
        ub, yb = ubuf[s], ybuf[s]
        for p in range(16):
            r = p * 8
            acc = [[None] * ab for _ in range(3)]
            for c in range(a0 + ab):
                u_i, u_r = ub[1, c, r:r + 8, :], ub[0, c, r:r + 8, :]
                uu = [u_r + u_i, u_i, u_r]
                for i in range(ab):
                    m = a0 + i - c
                    if m < 0:
                        continue
                    for t in range(3):
                        x = ksta[p, t * 128 + m * 8:t * 128 + m * 8 + 8, :] * uu[t]
                        acc[t][i] = x if acc[t][i] is None else acc[t][i] + x
            for i in range(ab):
                yb[a0 + i, r:r + 8, :] = pltpu.pack_elementwise(
                    [acc[0][i] - acc[1][i], acc[0][i] + acc[2][i]], packed_dtype=BF16)

    def idft(j, s, as_=range(NA)):
        as_ = list(as_)
        if BIG:
            z = fresh(48)
            toks = []
            for h in range(2):
                g = _bf(invp[pl.ds(z, 64), h * 128:(h + 1) * 128])
                rhs = jnp.concatenate([_bf(ybuf[s][a, h * 64:(h + 1) * 64, :]) for a in as_], axis=1)
                r = _dot(g, rhs)
                for n, a in enumerate(as_):
                    y2[h, j, a * L:(a + 1) * L, :] = r[:, n * 128:(n + 1) * 128]
                toks += [r[0:8, n * 128:(n + 1) * 128] for n in range(len(as_))]
            return toks
        toks = []
        for a in as_:
            z = fresh(48 + a)
            g0 = _bf(invp[pl.ds(z, 64), 0:128])
            g1 = _bf(invp[pl.ds(z, 64), 128:256])
            r0 = _dot(g0, _bf(ybuf[s][a, 0:64, :]))
            r1 = _dot(g1, _bf(ybuf[s][a, 64:128, :]))
            y2[0, j, a * L:(a + 1) * L, :] = r0
            y2[1, j, a * L:(a + 1) * L, :] = r1
            toks.append(r1[0:8])
        return toks

    def w_transpose(ns=range(15)):
        toks = []
        for n in ns:
            eye = _bf(eyep[pl.ds(fresh(n), 64), :])
            r = _dot_nt(eye, _bf(wqkvw[n]))
            for kt in range(ND):
                wt[kt, n * 128:(n + 1) * 128, :] = r[:, kt * 128:(kt + 1) * 128]
            toks.append(r[0:8, 0:128])
        return toks

    def w_permute(parts=range(3)):
        for p in parts:
            for dh in range(DH):
                for kt in range(ND):
                    rows = wt[kt, pl.ds(p * D + dh, H, stride=DH), :]
                    r0 = (p * D + dh * H) // 2
                    wtp[r0:r0 + H // 2, kt * 128:(kt + 1) * 128] = _u32(rows.astype(BF16))

    def wo_permute():
        for j in range(ND):
            wof[j] = wo_v[j].astype(F32)
        for dh in range(DH):
            for j in range(ND):
                rows = wof[j, pl.ds(dh, H, stride=DH), :]
                r0 = dh * H // 2
                wop[r0:r0 + H // 2, j * 128:(j + 1) * 128] = _u32(rows.astype(BF16))

    def qkv(b, s, fine=False):
        r0 = pl.multiple_of(b * (T // 2), T // 2)
        if MSPLIT > 1:
            h = T // MSPLIT
            rs = []
            for i in range(MSPLIT):
                x = jnp.concatenate([_bf(qw[j, pl.ds(r0 + i * h // 2, h // 2), :]) for j in range(ND)], axis=1)
                r = _dot_nt(x, _bf(wtp[pl.ds(fresh(20 + i), 3 * D // 2), :]))
                for j in range(ND):
                    qp[s][j, i * h:(i + 1) * h, :] = r[:, j * 128:(j + 1) * 128]
                    kp[s][j, HALO + i * h:HALO + (i + 1) * h, :] = r[:, D + j * 128:D + (j + 1) * 128]
                    vp[s][j, HALO + i * h:HALO + (i + 1) * h, :] = r[:, 2 * D + j * 128:2 * D + (j + 1) * 128]
                rs.append(r)
            allt = [rs[i][0:8, n * 128:(n + 1) * 128] * zvec[...] for i in range(MSPLIT) for n in range(15)]
            return [allt[(k * len(allt)) // 15] for k in range(15)]
        x = jnp.concatenate([_bf(qw[j, pl.ds(r0, T // 2), :]) for j in range(ND)], axis=1)
        r = _dot(x, _bf(wnn[...])) if NNW else _dot_nt(x, _bf(wtp[...]))
        for j in range(ND):
            qp[s][j] = r[:, j * 128:(j + 1) * 128]
            kp[s][j, HALO:HALO + T, :] = r[:, D + j * 128:D + (j + 1) * 128]
            vp[s][j, HALO:HALO + T, :] = r[:, 2 * D + j * 128:2 * D + (j + 1) * 128]
        if fine:
            return [r[64 * i:64 * i + 8, n * 128:(n + 1) * 128] * zvec[...] for n in range(15) for i in range(4)]
        return [r[0:8, n * 128:(n + 1) * 128] * zvec[...] for n in range(15)]

    def qkv_half(b, s, i):
        h = T // 2
        r0 = b * (T // 2) + i * (h // 2)
        x = jnp.concatenate([_bf(qw[j, r0:r0 + h // 2, :]) for j in range(ND)], axis=1)
        r = _dot_nt(x, _bf(wtp[pl.ds(fresh(20 + i), 3 * D // 2), :]))
        for j in range(ND):
            qp[s][j, i * h:(i + 1) * h, :] = r[:, j * 128:(j + 1) * 128]
            kp[s][j, HALO + i * h:HALO + (i + 1) * h, :] = r[:, D + j * 128:D + (j + 1) * 128]
            vp[s][j, HALO + i * h:HALO + (i + 1) * h, :] = r[:, 2 * D + j * 128:2 * D + (j + 1) * 128]
        return [r[0:8, n * 128:(n + 1) * 128] * zvec[...] for n in range(15)]

    def gate(b, s, mt=None):
        r0 = pl.multiple_of(b * T, T)
        for g in range(NG):
            sm = None if mt is None else jnp.concatenate([mt[(g * GN) // NG]] * (GR // 8), axis=0)
            for j in range(ND):
                t = _bmul(qbuf[j, pl.ds(r0 + g * GR, GR), :].astype(F32), par[j, 5])
                sm = t if sm is None else sm + t
            hi = sm.astype(BF16)
            gsp[0, g * GR // 2:(g + 1) * GR // 2, :] = _u32(hi)
            if GLO:
                lo = (sm - hi.astype(F32)).astype(BF16)
                gsp[1, g * GR // 2:(g + 1) * GR // 2, :] = _u32(lo)
        ones = _bf(onesp[...])
        glog[s][0] = _dot(_bf(gsp[0]), ones)
        if GLO:
            glog[s][1] = _dot(_bf(gsp[1]), ones)

    def halo(s):
        for j in range(ND):
            kp[1 - s][j, 0:HALO, :] = kp[s][j, T:T + HALO, :]
            vp[1 - s][j, 0:HALO, :] = vp[s][j, T:T + HALO, :]

    def softmax_pv(vv, row, ob, lg=None):
        if lg is None:
            lg = [lbuf[w, row:row + GR, :] for w in range(8)]
        m = lg[0]
        for w in range(1, 8):
            m = jnp.maximum(m, lg[w])
        es = [(l - m) if E('NOEXP', '0') == '1' else jnp.exp2(l - m) for l in lg]
        sm = es[0]
        for w in range(1, 8):
            sm = sm + es[w]
        inv = 1.0 / sm
        for j in range(ND):
            acc = None
            for w in range(8):
                o = row + HALO - 2 * w
                t = es[w] * vv[j, o:o + GR, :]
                acc = t if acc is None else acc + t
            res = acc * inv
            ob[row // 2:(row + GR) // 2, j * 128:(j + 1) * 128] = _u32(res.astype(BF16))
        return res[0:8]

    def qk(qq, kk, row, tok):
        if tok is None:
            q = [qq[j, row:row + GE, :] * QSCALE for j in range(ND)]
        else:
            sc = tok + QSCALE
            q = [_bmul(qq[j, row:row + GE, :], sc) for j in range(ND)]
        out = []
        for w in range(8):
            p = None
            o = row + HALO - 2 * w
            for j in range(ND):
                t = q[j] * kk[j, o:o + GE, :]
                p = t if p is None else p + t
            out.append(p)
        return out

    def attention(b, s, mt=None, row0=0, nrows=T, an=AN, ob=None):
        qq, kk, vv = qp[s], kp[s], vp[s]
        ob = op if ob is None else ob
        g0 = row0 // GE
        n1 = g0 + nrows // GE
        per = GR // GE
        r1, r2, done = {}, {}, {}
        for g in range(g0, n1 + D3 + per):
            if g < n1:
                row = g * GE
                tok = None
                if mt is not None:
                    tok = mt[((g - g0) * an) // (n1 - g0)]
                    prev = done.get(row // GR - PACE) if PACE else None
                    if prev is not None:
                        tok = tok + prev * zvec[...]
                r1[g] = []
                for w, p in enumerate(qk(qq, kk, row, tok)):
                    pbuf[w, row:row + GE, :] = p
                    r1[g].append(p * 2.0 if E('NOROLL', '0') == '1' else pltpu.roll(p, 64, 1))
            gg = g - D1
            if g0 <= gg < n1:
                row = gg * GE
                r2[gg] = []
                for w, r in enumerate(r1.pop(gg)):
                    sm = pbuf[w, row:row + GE, :] + r
                    sbuf[w, row:row + GE, :] = sm
                    r2[gg].append(sm * 2.0 if E('NOROLL', '0') == '1' else pltpu.roll(sm, 32, 1))
            gg = g - D2
            if g0 <= gg < n1:
                row = gg * GE
                ls = []
                for w, r in enumerate(r2.pop(gg)):
                    l = sbuf[w, row:row + GE, :] + r
                    if row < HALO and w > 0:
                        t = b * T + row + jax.lax.broadcasted_iota(jnp.int32, (GE, 128), 0)
                        l = jnp.where(t >= 2 * w, l, MASKED)
                    if NOLBUF:
                        ls.append(l)
                    else:
                        lbuf[w, row:row + GE, :] = l
                if NOLBUF:
                    done[row // GR] = softmax_pv(vv, row, ob, ls)
            gg = g - D3
            if not NOLBUF and g0 <= gg < n1 and (gg + 1) % per == 0:
                row = (gg + 1 - per) * GE
                done[row // GR] = softmax_pv(vv, row, ob)

    def outproj(s, r0=0, n=T, ob=None):
        ob = op if ob is None else ob
        r = _dot(_bf(ob[r0 // 2:(r0 + n) // 2, :]), _bf(wop[...]))
        bres[s][r0:r0 + n, :] = r
        return [r[0:8, k * 128:(k + 1) * 128] * zvec[...] for k in range(ND)]

    def epilogue(b, s, mt=None, gs=range(NG)):
        r0 = pl.multiple_of(b * T, T)
        for g in gs:
            row = r0 + g * GR
            rowh = pl.multiple_of(b * (T // 2), T // 2) + g * (GR // 2)
            gl = glog[s][0, g * GR:(g + 1) * GR, :]
            if GLO:
                gl = gl + glog[s][1, g * GR:(g + 1) * GR, :]
            if mt is not None:
                gl = _badd(gl, mt[(g * EN) // NG])
            gt = jax.nn.sigmoid(gl)
            for j in range(ND):
                q = qbuf[j, pl.ds(row, GR), :].astype(F32)
                kv = _bf(kvp[j, pl.ds(rowh, GR // 2), :]).astype(F32)
                z = y2[0, j, pl.ds(row, GR), :] + y2[1, j, pl.ds(row, GR), :] + _bmul(kv, par[j, 4])
                bb = bres[s][g * GR:(g + 1) * GR, j * 128:(j + 1) * 128]
                o = bb + gt * (q * z - bb)
                obuf[b % NOB, j, g * GR:(g + 1) * GR, :] = o.astype(BF16)

    def region(k, f):
        pl.when(zsm[k % 64] == 0)(f)

    P = functools.partial

    wq_0, wq_1, wq_b = _Copies(wqkv_copy.cs[:WQ0]), _Copies(wqkv_copy.cs[WQ0:8]), _Copies(wqkv_copy.cs[8:])
    wq_a = _Copies(wqkv_copy.cs[:8])

    def x_dma(j):
        with _scope("waitX%d" % j):
            if STREAM and j == 0:
                kv_copy(1).wait()
            if not (STREAM and j == 0):
                sk_copy(j + 1).wait()
            if j >= 2 or (j == 1 and not STREAM):
                kv_copy(j + 1).wait()

        def starts():
            if j == 0:
                kv_copy(2).start()
                if not STREAM:
                    sk_copy(2).start()
            if j == 1:
                kv_copy(3).start()
                sk_copy(3).start()
            if j == 2:
                kv_copy(4).start()
                sk_copy(4).start()
                wq_0.start()
            if j == 3:
                _Copies(wqkv_copy.cs[WQ0:]).start()
                q_copy(0).start()

        if DMAREG:
            region(40 + j, starts)
        else:
            starts()

    def block_x(j):
        s = j % 2
        late_kv = STREAM and j == 1
        if not (STREAM and j == 0):
            with _scope("X%d" % j):
                if j >= 1 and not late_kv and not XSPLIT:
                    kvprep(j + 1)
                aconv(s)
                if j >= 1:
                    idft(j - 1, 1 - s, range(KVI if (XSPLIT and not late_kv) else 0, NA))
                dft_k(j + 1, 1 - s)
                if j >= 1 and not late_kv:
                    dft_u(j + 1, 1 - s)
        if j == 0 or late_kv:
            if not (STREAM and j == 0):
                with _scope("waitK%d" % (j + 1)):
                    kv_copy(j + 1).wait()
            with _scope("Y%d" % j):
                kvprep(j + 1)
                dft_u(j + 1, 1 - s)

    def body_a(j, carry):
        return carry

    def b_dma(b, s):
        if ONLY == '':
            q_copy(b).wait()

        @pl.when(b - 2 >= NOB)
        def _():
            out_copy(b - 2 - NOB).wait()

    def epilogue_wait(t):
        if t >= NOB:
            out_copy(t - NOB).wait()

    def block_b(b, s, dma=True):
        if dma:
            b_dma(b, s)
        with _scope("B"):
            halo(1 - s)
            mt = qkv(b, s)
            if EPI == 'paced':
                epilogue(b - 2, s, mt)
            elif EPI == 'free':
                epilogue(b - 2, s)
            elif EPI == 'late':
                epilogue(b - 2, s, [mt[14]] * 15)
            if EPI != 'after':
                out_copy(b - 2).start()
            if E('NOATT', '0') != '1':
                attention(b - 1, 1 - s, mt)
            if E('NOGATE', '0') != '1':
                gate(b - 1, 1 - s, mt if GATEP else None)
            if EPI == 'after':
                ot = outproj(1 - s)
                epilogue(b - 2, s, [ot[(g * 5) // 15] for g in range(15)])
                out_copy(b - 2).start()
            else:
                outproj(1 - s)

    def body_b2(i, carry):
        b = 2 * i
        if ONLY == '':
            q_copy(b).wait()
            q_copy(b + 1).wait()

        @pl.when(b - 2 >= NOB)
        def _():
            out_copy(b - 2 - NOB).wait()
            out_copy(b - 1 - NOB).wait()
        block_b(b, 0, False)
        block_b(b + 1, 1, False)
        return carry

    def body_b(b, carry):
        if E('ONEPAR', '0') == '1':
            block_b(b, 0)
            return carry
        for s in range(2):
            pl.when(b % 2 == s)(functools.partial(block_b, b, s))
        return carry

    if ONLY != 'B':
        nb = NA // NCH
        for ch in range(NCH):
            with _scope("wait0"):
                first_copy(ch).wait()
            if ch == 1:
                sk_copy(1).start()
            if ch == NCH - 1:
                kv_copy(1).start()
            blks = range(ch * nb, (ch + 1) * nb)

            def seg(ch=ch, blks=blks):
                if STREAM and ch >= 1:
                    kprep_all(0, range((ch - 1) * nb, ch * nb))
                    macs_all(0, (ch - 1) * nb, nb)
                if not PROSPLIT:
                    kvprep(0, blks)
                dft_k(0, 0, blks)
                dft_u(0, 0, blks)

            with _scope("pro"):
                if PROSPLIT:
                    kvprep(0, blks)
                    region(30 + ch, seg)
                else:
                    seg()
        if STREAM:
            with _scope("wait0"):
                sk_copy(1).wait()
            sk_copy(2).start()
            with _scope("pro2"):
                kprep_all(0, range((NCH - 1) * nb, NA))
                macs_all(0, (NCH - 1) * nb, nb)
                dft_k(1, 1)

        for j in range(ND - 1):
            x_dma(j)
            if XSPLIT and j >= 1 and not (STREAM and j == 1):
                with _scope("KV%d" % (j + 1)):
                    kvprep(j + 1)
                    if KVI:
                        idft(j - 1, 1 - j % 2, range(0, KVI))
            region(2 * j, P(block_x, j))

    if ONLY == '':
        def block_wlate0():
            with _scope("Alast00"):
                aconv((ND - 1) % 2, range(0, WSPLIT))
                idft(ND - 2, (ND - 2) % 2)

        if WSPLIT:
            region(14, block_wlate0)
        with _scope("waitW"):
            wqkv_copy.wait()
        wo_copy.start()
        q_copy(1).start()

        def block_wlate():
            with _scope("Alast0"):
                aconv((ND - 1) % 2, range(WSPLIT, 16))
                if not WSPLIT:
                    idft(ND - 2, (ND - 2) % 2)
                w_transpose()

        region(12, block_wlate)
        with _scope("waitQ"):
            q_copy(0).wait()
        for b in range(2, NT):
            q_copy(b).start()

        def block_alast():
            if WLATE:
                with _scope("Alast"):
                    if AMERGE == 3:
                        return
                    w_permute({0: [0, 1, 2], 1: [1, 2], 2: []}[AMERGE])
                    qkv(0, 0)
                return
            with _scope("Alast"):
                w_permute([1, 2] if PERM_EARLY else [0, 1, 2])
                if Q0 == 3:
                    idft(ND - 2, (ND - 2) % 2)
                    mt = qkv(0, 0, True)
                    wts = [sum(a + 1 for a in range(a0, a0 + LAB)) for a0 in range(0, NA, LAB)]
                    tot = 136 * 16
                    bt, cum = [], 0
                    for p in range(16):
                        row = []
                        for bi in range(len(wts)):
                            k = (cum * LN * len(mt)) // (tot * 16) - LOFF
                            row.append(mt[min(k, len(mt) - 1)] if k >= 0 else None)
                            cum += wts[bi]
                        bt.append(row)
                    aconv((ND - 1) % 2, range(16), btoks=bt, ab=LAB)
                elif Q0 == 2:
                    idft(ND - 2, (ND - 2) % 2)
                    mt = qkv(0, 0)
                    toks = [None] + [mt[min(14, ((p - 1) * LN) // 16)] for p in range(1, 16)]
                    aconv((ND - 1) % 2, range(16), toks, tz=False)
                else:
                    aconv((ND - 1) % 2)
                    idft(ND - 2, (ND - 2) % 2)
                    if Q0:
                        qkv(0, 0)

        region(10, block_alast)

        def block_b1():
            q_copy(1).wait()
            wo_copy.wait()
            with _scope("B1"):
                wo_permute()
                if not Q0:
                    qkv(0, 0)
                idft(ND - 1, (ND - 1) % 2)
                halo(0)
                mt = qkv(1, 1)
                attention(0, 0, mt)
                gate(0, 0, mt)
                outproj(0)

        region(11, block_b1)

    if ONLY != 'A':
        if PAIR:
            jax.lax.fori_loop(1, NT // 2, body_b2, 0)
        else:
            jax.lax.fori_loop(2, NT - 1 if (LASTB and ONLY == '') else NT, body_b, 0)

    if ONLY == '':
        if LASTB:
            def block_last():
                b, s = NT - 1, (NT - 1) % 2
                q_copy(b).wait()
                epilogue_wait(b - 2)
                with _scope("B7"):
                    halo(1 - s)
                    m1 = qkv_half(b, s, 0)
                    m2 = qkv_half(b, s, 1)
                    epilogue(b - 2, s, [m2[14]] * 15)
                    out_copy(b - 2).start()
                    attention(b - 1, 1 - s, m1 + m2, an=LAN1)
                    gate(b - 1, 1 - s, m1)
                    attention(b, s, m2, 0, T // 2, an=LAN2, ob=op2)
                    outproj(1 - s)

            region(13, block_last)
            with _scope("fin1"):
                epilogue_wait(NT - 2)
                epilogue_wait(NT - 1)
                epilogue(NT - 2, 0)
                out_copy(NT - 2).start()
                gate(NT - 1, 1)
                attention(NT - 1, 1, None, T // 2, T // 2, ob=op2)
                nh = T // FSPLIT
                for h in range(FSPLIT):
                    outproj(1, h * nh, nh, op2)
                for h in range(FSPLIT):
                    epilogue(NT - 1, 1, None, range(h * nh // GR, (h + 1) * nh // GR))
                    out_copy(NT - 1, h * nh, nh).start()
        elif FSPLIT:
            with _scope("fin1"):
                epilogue_wait(NT - 2)
                epilogue_wait(NT - 1)
                epilogue(NT - 2, 0)
                out_copy(NT - 2).start()
                gate(NT - 1, 1)
                attention(NT - 1, 1)
                nh = T // FSPLIT
                for h in range(FSPLIT):
                    outproj(1, h * nh, nh)
                for h in range(FSPLIT):
                    epilogue(NT - 1, 1, None, range(h * nh // GR, (h + 1) * nh // GR))
                    out_copy(NT - 1, h * nh, nh).start()
        else:
            with _scope("fin1"):
                epilogue_wait(NT - 2)
                epilogue(NT - 2, 0)
                out_copy(NT - 2).start()
                attention(NT - 1, 1)
                gate(NT - 1, 1)
                outproj(1)
            with _scope("fin2"):
                epilogue_wait(NT - 1)
                epilogue(NT - 1, 1)
                out_copy(NT - 1).start()
        with _scope("fin3"):
            for t in range(NT - NOB, NT):
                out_copy(t).wait()
    elif ONLY == 'B':
        for t in range(NT - 2 - NOB, NT - 2):
            out_copy(t).wait()
    else:
        for b in range(2):
            q_copy(b).wait()
        wo_copy.wait()


@jax.jit
def pallas_gated_mix__ssm_conv_h3__sliding_local_dilated__prompt_kernel(A_q, A_k, A_v, A_shift_k, A_ssm_k, A_ssm_D, B_x, B_wqkv, B_wo, gate_w):
    fwd, inv, eye = _dft_constants()
    hbm = pl.BlockSpec(memory_space=pl.ANY)
    vm = pl.BlockSpec(memory_space=pltpu.VMEM)
    two = lambda shape, dt: [pltpu.VMEM(shape, dt), pltpu.VMEM(shape, dt)]
    return pl.pallas_call(
        _kernel,
        out_shape=jax.ShapeDtypeStruct((1, S, D), BF16),
        in_specs=[hbm] * 12,
        out_specs=hbm,
        scratch_shapes=[
            pltpu.VMEM((4, D), BF16),
            pltpu.VMEM((D,), BF16),
            pltpu.VMEM((D,), BF16),
            pltpu.VMEM((384, 128), BF16),
            pltpu.VMEM((128, 256), BF16),
            pltpu.VMEM((128, 128), BF16),
            pltpu.VMEM((ND, 2 * KH + S, 128), BF16),
            pltpu.VMEM((ND, S, 128), BF16),
            pltpu.VMEM((ND, NA, 128, L), BF16),
            pltpu.VMEM((ND, S, 128), BF16),
            pltpu.VMEM((15, D, 128), BF16),
            pltpu.VMEM((ND, D, 128), BF16),
            pltpu.VMEM((ND, 6, 8, 128), F32),
            pltpu.VMEM((8, 128), F32),
            pltpu.SMEM((64,), jnp.int32),
            pltpu.VMEM((192, 128), U32),
            pltpu.VMEM((64, 256), U32),
            pltpu.VMEM((64, 128), U32),
            pltpu.VMEM((64, 128), U32),
            pltpu.VMEM((ND, S // 2, 128), U32),
            *two((3, NA, 128, 128), F32),
            *two((NA, 256, 128), F32),
            *two((NA, 128, 128), U32),
            *two((384, 128), F32),
            pltpu.VMEM((16, 384, 128), F32),
            pltpu.VMEM((2, ND, S, 128), F32),
            pltpu.VMEM((ND, 3 * D, 128), F32),
            pltpu.VMEM((3 * D // 2, D), U32),
            pltpu.VMEM((D // 2, 3 * D), U32),
            pltpu.VMEM((ND, D, 128), F32),
            pltpu.VMEM((D // 2, D), U32),
            *two((ND, T, 128), F32),
            *two((ND, HALO + T, 128), F32),
            *two((ND, HALO + T, 128), F32),
            pltpu.VMEM((8, T, 128), F32),
            pltpu.VMEM((8, T, 128), F32),
            pltpu.VMEM((8, T, 128), F32),
            pltpu.VMEM((T // 2, D), U32),
            pltpu.VMEM((T // 2, D), U32),
            *two((T, D), F32),
            pltpu.VMEM((NOB, ND, T, 128), BF16),
            pltpu.VMEM((2, T // 2, 128), U32),
            *two((2, T, 128), F32),
            pltpu.SemaphoreType.DMA((3 * ND,)),
            pltpu.SemaphoreType.DMA((NT,)),
            pltpu.SemaphoreType.DMA((2,)),
            pltpu.SemaphoreType.DMA((NOB,)),
            pltpu.SemaphoreType.DMA((6,)),
            pltpu.SemaphoreType.DMA((NCH,)),
        ],
        compiler_params=pltpu.CompilerParams(vmem_limit_bytes=100 * 2 ** 20),
    )(A_q, A_k, A_v, A_shift_k.T, A_ssm_k, A_ssm_D, B_wqkv, B_wo, gate_w,
      jnp.asarray(fwd, BF16), jnp.asarray(inv, BF16), jnp.asarray(eye, BF16))
```

```python
import functools

import numpy as np
import jax
import jax.numpy as jnp
from jax.experimental import pallas as pl
from jax.experimental.pallas import tpu as pltpu

S, D = 2048, 640
ND = 5
L = 128
NA = S // L
AB = 4
NCH = 4
T = 256
NT = S // T
H, DH = 32, 20
HALO = 16
KH = 8
GR = 16
GE = 8
NG = T // GR
NOB = 4
WQ0 = 4
KVI = 8
D1, D2, D3 = 2, 4, 5
PACE = 4
LOG2E = 1.4426950408889634
QSCALE = float(DH ** -0.5) * LOG2E
MASKED = -1e9 * LOG2E
F32, BF16, U32 = jnp.float32, jnp.bfloat16, jnp.uint32


def _dft_constants():
    forder = np.concatenate([np.arange(0, 128, 2), np.arange(1, 128, 2)])
    th = np.pi * (2 * forder + 1) / 256.0
    b = np.arange(128)
    fwd = np.concatenate([np.cos(np.outer(th, b)), -np.sin(np.outer(th, b))], 0)
    gre = np.cos(np.outer(b, th)) / 128
    gim = -np.sin(np.outer(b, th)) / 128
    inv = np.stack([gre, gim], -1).reshape(128, 256)
    return fwd.astype(np.float32), inv.astype(np.float32), np.eye(128, dtype=np.float32)


def _bf(x):
    return pltpu.bitcast(x, BF16)


def _u32(x):
    return pltpu.bitcast(x, U32)


def _bmul(x, t8):
    return (x.reshape(-1, 8, 128) * t8).reshape(x.shape)


def _badd(x, t8):
    return (x.reshape(-1, 8, 128) + t8).reshape(x.shape)


def _dot(a, b):
    return jnp.dot(a, b, preferred_element_type=F32)


def _dot_nt(a, b):
    return jax.lax.dot_general(a, b, (((1,), (1,)), ((), ())), preferred_element_type=F32)


class _Copies:
    def __init__(self, cs):
        self.cs = list(cs)

    def start(self):
        for c in self.cs:
            c.start()

    def wait(self):
        for c in self.cs:
            c.wait()


def _kernel(q_hbm, k_hbm, v_hbm, shk_hbm, sk_hbm, dvec_hbm, wqkv_hbm, wo_hbm, gw_hbm,
            fwd_hbm, inv_hbm, eye_hbm,
            out_hbm,
            shk_ref, dvec_ref, gw_ref, fwd_ref, inv_ref, eye_ref,
            kbuf, vbuf, skbuf, qbuf, wqkv_v, wo_v, par, zvec, zsm, fwdp, invp, onesp, eyep,
            kvp, ubuf0, ubuf1, kpbuf0, kpbuf1, ybuf0, ybuf1, kst0, kst1, ksta, y2, wt, wtp, wof, wop,
            qp0, qp1, kp0, kp1, vp0, vp1, pbuf, sbuf, lbuf, op, op2, bres0, bres1, obuf, gsp, glog0, glog1,
            sem_a, sem_q, sem_w, sem_o, sem_s, sem_f):
    ubuf, kpbuf, ybuf, kstb = (ubuf0, ubuf1), (kpbuf0, kpbuf1), (ybuf0, ybuf1), (kst0, kst1)
    qp, kp, vp = (qp0, qp1), (kp0, kp1), (vp0, vp1)
    bres, glog = (bres0, bres1), (glog0, glog1)
    skw, qw, wqkvw = skbuf.bitcast(U32), qbuf.bitcast(U32), wqkv_v.bitcast(U32)
    kw, vw = kbuf.bitcast(U32), vbuf.bitcast(U32)
    P = functools.partial

    def kv_copy(j):
        return _Copies(
            [pltpu.make_async_copy(k_hbm.at[0, :, pl.ds(j * 128, 128)], kbuf.at[j, pl.ds(2 * KH, S)],
                                   sem_a.at[2 * j]),
             pltpu.make_async_copy(v_hbm.at[0, :, pl.ds(j * 128, 128)], vbuf.at[j], sem_a.at[2 * j])])

    def sk_copy(j):
        return _Copies(pltpu.make_async_copy(sk_hbm.at[pl.ds(j * 128, 128), pl.ds(m * L, L)], skbuf.at[j, m],
                                             sem_a.at[2 * j + 1]) for m in range(NA))

    def first_copy(ch):
        n = S // NCH
        rows = pl.ds(ch * n, n)
        ms = range(ch * (NA // NCH), (ch + 1) * (NA // NCH))
        return _Copies(
            [pltpu.make_async_copy(k_hbm.at[0, rows, pl.ds(0, 128)], kbuf.at[0, pl.ds(2 * KH + ch * n, n)],
                                   sem_f.at[ch]),
             pltpu.make_async_copy(v_hbm.at[0, rows, pl.ds(0, 128)], vbuf.at[0, rows], sem_f.at[ch])]
            + [pltpu.make_async_copy(sk_hbm.at[pl.ds(0, 128), pl.ds(m * L, L)], skbuf.at[0, m], sem_f.at[ch])
               for m in ms])

    small_copy = _Copies(pltpu.make_async_copy(a, b, sem_s.at[i]) for i, (a, b) in enumerate(
        [(shk_hbm, shk_ref), (dvec_hbm, dvec_ref), (gw_hbm, gw_ref), (fwd_hbm, fwd_ref), (inv_hbm, inv_ref),
         (eye_hbm, eye_ref)]))

    def q_copy(b):
        rows = pl.ds(b * T, T)
        return _Copies(pltpu.make_async_copy(q_hbm.at[0, rows, pl.ds(j * 128, 128)], qbuf.at[j, rows], sem_q.at[b])
                       for j in range(ND))

    wqkv_copy = _Copies(pltpu.make_async_copy(wqkv_hbm.at[:, pl.ds(n * 128, 128)], wqkv_v.at[n], sem_w.at[0])
                        for n in range(15))
    wo_copy = _Copies(pltpu.make_async_copy(wo_hbm.at[:, pl.ds(n * 128, 128)], wo_v.at[n], sem_w.at[1])
                      for n in range(ND))

    def out_copy(b, r0=0, n=T):
        return _Copies(pltpu.make_async_copy(obuf.at[b % NOB, j, pl.ds(r0, n)],
                                             out_hbm.at[0, pl.ds(b * T + r0, n), pl.ds(j * 128, 128)],
                                             sem_o.at[b % NOB]) for j in range(ND))

    for j in range(ND):
        kbuf[j, 0:2 * KH, :] = jnp.zeros((2 * KH, 128), BF16)
    small_copy.start()
    first_copy(0).start()
    small_copy.wait()
    for ch in range(1, NCH):
        first_copy(ch).start()

    taps = shk_ref[...].astype(F32)
    dv = dvec_ref[...].astype(F32).reshape(1, D)
    gw = gw_ref[...].astype(F32).reshape(1, D)
    for j in range(ND):
        for i in range(4):
            par[j, i] = jnp.broadcast_to(taps[i:i + 1, j * 128:(j + 1) * 128], (8, 128))
        par[j, 4] = jnp.broadcast_to(dv[:, j * 128:(j + 1) * 128], (8, 128))
        par[j, 5] = jnp.broadcast_to(gw[:, j * 128:(j + 1) * 128], (8, 128))
    zvec[...] = jnp.zeros((8, 128), F32)
    for i in range(64):
        zsm[i] = 0
    fwdp[...] = _u32(fwd_ref[...])
    invp[...] = _u32(inv_ref[...])
    eyep[...] = _u32(eye_ref[...])
    onesp[...] = _u32(jnp.ones((128, 128), BF16))
    for j in range(ND):
        kp0[j, 0:HALO, :] = jnp.zeros((HALO, 128), F32)
        vp0[j, 0:HALO, :] = jnp.zeros((HALO, 128), F32)

    def fresh(i):
        return pl.multiple_of(zsm[i] * 8, 8)

    def region(k, f):
        pl.when(zsm[k] == 0)(f)

    def kvprep(j, blks=range(NA)):
        t = [par[j, i] for i in range(4)]
        even = lambda w: pltpu.bitcast(w << 16, F32)
        odd = lambda w: pltpu.bitcast(w & jnp.uint32(0xFFFF0000), F32)
        for c in blks:
            for q in range(L // 32):
                r = c * (L // 2) + q * 16
                w0 = kw[j, KH + r:KH + r + 16, :]
                w1 = kw[j, KH + r - 1:KH + r + 15, :]
                w2 = kw[j, KH + r - 2:KH + r + 14, :]
                e0, o0, e1, o1, o2 = even(w0), odd(w0), even(w1), odd(w1), odd(w2)
                ks_e = _bmul(e0, t[0]) + _bmul(o1, t[1]) + _bmul(e1, t[2]) + _bmul(o2, t[3])
                ks_o = _bmul(o0, t[0]) + _bmul(e0, t[1]) + _bmul(o1, t[2]) + _bmul(e1, t[3])
                wv = vw[j, r:r + 16, :]
                kvp[j, r:r + 16, :] = pltpu.pack_elementwise([ks_e * even(wv), ks_o * odd(wv)], packed_dtype=BF16)

    def dft_u(j, s, cs=range(NA)):
        for c in cs:
            f = _bf(fwdp[pl.ds(fresh(16 + c), 128), :])
            r = _dot(f, _bf(kvp[j, c * 64:(c + 1) * 64, :]))
            ubuf[s][0, c] = r[0:128]
            ubuf[s][1, c] = r[128:256]

    def dft_k(j, s, ms=range(NA)):
        for m in ms:
            f = _bf(fwdp[pl.ds(fresh(32 + m), 128), :])
            kpbuf[s][m] = _dot_nt(f, _bf(skw[j, m]))

    def filter_prep(kb, p, m):
        r, im = p * 8, 128 + p * 8
        pr, pi = kb[m, r:r + 8, :], kb[m, im:im + 8, :]
        if m == 0:
            kr, ki = pr, pi
        elif p < 8:
            kr, ki = pr - kb[m - 1, im:im + 8, :], pi + kb[m - 1, r:r + 8, :]
        else:
            kr, ki = pr + kb[m - 1, im:im + 8, :], pi - kb[m - 1, r:r + 8, :]
        return kr, kr + ki, ki - kr

    def mac_group(ub, yb, p, a0, z, kload, between=None):
        r = p * 8
        acc = [[None] * AB for _ in range(3)]
        for c in range(a0 + AB):
            rows = pl.ds(r if z is None else z + r, 8)
            u_i, u_r = ub[1, c, rows, :], ub[0, c, rows, :]
            uu = [u_r + u_i, u_i, u_r]
            for i in range(AB):
                m = a0 + i - c
                if m < 0:
                    continue
                for t in range(3):
                    x = kload(t, m) * uu[t]
                    acc[t][i] = x if acc[t][i] is None else acc[t][i] + x
            if between is not None:
                between(c)
        for i in range(AB):
            yb[a0 + i, r:r + 8, :] = pltpu.pack_elementwise(
                [acc[0][i] - acc[1][i], acc[0][i] + acc[2][i]], packed_dtype=BF16)

    def aconv(s):
        ub, kb, yb = ubuf[s], kpbuf[s], ybuf[s]

        def kprep(p, ms):
            for m in ms:
                for t, x in enumerate(filter_prep(kb, p, m)):
                    kstb[p % 2][t * 128 + m * 8:t * 128 + m * 8 + 8, :] = x

        kprep(0, range(NA))
        nb = NA // AB
        for p in range(16):
            kst = kstb[p % 2]
            for bi in range(nb):
                z = fresh(bi)
                between = None
                if p + 1 < 16 and bi >= nb - 2:
                    first = (bi - (nb - 2)) * 8
                    between = lambda c, first=first: kprep(p + 1, [first + c]) if c < 8 else None
                mac_group(ub, yb, p, bi * AB, z, lambda t, m: kst[pl.ds(z + t * 128 + m * 8, 8), :], between)

    def kprep_all(s, ms):
        for p in range(16):
            for m in ms:
                for t, x in enumerate(filter_prep(kpbuf[s], p, m)):
                    ksta[p, t * 128 + m * 8:t * 128 + m * 8 + 8, :] = x

    def macs_all(s, a0):
        for p in range(16):
            mac_group(ubuf[s], ybuf[s], p, a0, None, lambda t, m: ksta[p, t * 128 + m * 8:t * 128 + m * 8 + 8, :])

    def idft(j, s, as_=range(NA)):
        for a in as_:
            z = fresh(48 + a)
            g0 = _bf(invp[pl.ds(z, 64), 0:128])
            g1 = _bf(invp[pl.ds(z, 64), 128:256])
            y2[0, j, a * L:(a + 1) * L, :] = _dot(g0, _bf(ybuf[s][a, 0:64, :]))
            y2[1, j, a * L:(a + 1) * L, :] = _dot(g1, _bf(ybuf[s][a, 64:128, :]))

    def w_transpose():
        for n in range(15):
            eye = _bf(eyep[pl.ds(fresh(n), 64), :])
            r = _dot_nt(eye, _bf(wqkvw[n]))
            for kt in range(ND):
                wt[kt, n * 128:(n + 1) * 128, :] = r[:, kt * 128:(kt + 1) * 128]

    def w_permute():
        for p in range(3):
            for dh in range(DH):
                for kt in range(ND):
                    rows = wt[kt, pl.ds(p * D + dh, H, stride=DH), :]
                    r0 = (p * D + dh * H) // 2
                    wtp[r0:r0 + H // 2, kt * 128:(kt + 1) * 128] = _u32(rows.astype(BF16))

    def wo_permute():
        for j in range(ND):
            wof[j] = wo_v[j].astype(F32)
        for dh in range(DH):
            for j in range(ND):
                rows = wof[j, pl.ds(dh, H, stride=DH), :]
                r0 = dh * H // 2
                wop[r0:r0 + H // 2, j * 128:(j + 1) * 128] = _u32(rows.astype(BF16))

    def qkv(b, s):
        r0 = pl.multiple_of(b * (T // 2), T // 2)
        x = jnp.concatenate([_bf(qw[j, pl.ds(r0, T // 2), :]) for j in range(ND)], axis=1)
        r = _dot_nt(x, _bf(wtp[...]))
        for j in range(ND):
            qp[s][j] = r[:, j * 128:(j + 1) * 128]
            kp[s][j, HALO:HALO + T, :] = r[:, D + j * 128:D + (j + 1) * 128]
            vp[s][j, HALO:HALO + T, :] = r[:, 2 * D + j * 128:2 * D + (j + 1) * 128]
        return [r[0:8, n * 128:(n + 1) * 128] * zvec[...] for n in range(15)]

    def qkv_half(b, s, i):
        h = T // 2
        r0 = b * (T // 2) + i * (h // 2)
        x = jnp.concatenate([_bf(qw[j, r0:r0 + h // 2, :]) for j in range(ND)], axis=1)
        r = _dot_nt(x, _bf(wtp[pl.ds(fresh(20 + i), 3 * D // 2), :]))
        for j in range(ND):
            qp[s][j, i * h:(i + 1) * h, :] = r[:, j * 128:(j + 1) * 128]
            kp[s][j, HALO + i * h:HALO + (i + 1) * h, :] = r[:, D + j * 128:D + (j + 1) * 128]
            vp[s][j, HALO + i * h:HALO + (i + 1) * h, :] = r[:, 2 * D + j * 128:2 * D + (j + 1) * 128]
        return [r[0:8, n * 128:(n + 1) * 128] * zvec[...] for n in range(15)]

    def gate(b, s, mt=None):
        r0 = pl.multiple_of(b * T, T)
        for g in range(NG):
            sm = None if mt is None else jnp.concatenate([mt[(g * 10) // NG]] * (GR // 8), axis=0)
            for j in range(ND):
                t = _bmul(qbuf[j, pl.ds(r0 + g * GR, GR), :].astype(F32), par[j, 5])
                sm = t if sm is None else sm + t
            gsp[g * GR // 2:(g + 1) * GR // 2, :] = _u32(sm.astype(BF16))
        glog[s][...] = _dot(_bf(gsp[...]), _bf(onesp[...]))

    def halo(s):
        for j in range(ND):
            kp[1 - s][j, 0:HALO, :] = kp[s][j, T:T + HALO, :]
            vp[1 - s][j, 0:HALO, :] = vp[s][j, T:T + HALO, :]

    def softmax_pv(vv, row, ob):
        lg = [lbuf[w, row:row + GR, :] for w in range(8)]
        m = lg[0]
        for w in range(1, 8):
            m = jnp.maximum(m, lg[w])
        es = [jnp.exp2(l - m) for l in lg]
        sm = es[0]
        for w in range(1, 8):
            sm = sm + es[w]
        inv = 1.0 / sm
        for j in range(ND):
            acc = None
            for w in range(8):
                o = row + HALO - 2 * w
                t = es[w] * vv[j, o:o + GR, :]
                acc = t if acc is None else acc + t
            res = acc * inv
            ob[row // 2:(row + GR) // 2, j * 128:(j + 1) * 128] = _u32(res.astype(BF16))
        return res[0:8]

    def qk(qq, kk, row, tok):
        if tok is None:
            q = [qq[j, row:row + GE, :] * QSCALE for j in range(ND)]
        else:
            sc = tok + QSCALE
            q = [_bmul(qq[j, row:row + GE, :], sc) for j in range(ND)]
        out = []
        for w in range(8):
            p = None
            o = row + HALO - 2 * w
            for j in range(ND):
                t = q[j] * kk[j, o:o + GE, :]
                p = t if p is None else p + t
            out.append(p)
        return out

    def attention(b, s, mt=None, row0=0, nrows=T, an=13, ob=op):
        qq, kk, vv = qp[s], kp[s], vp[s]
        g0 = row0 // GE
        n1 = g0 + nrows // GE
        per = GR // GE
        r1, r2, done = {}, {}, {}
        for g in range(g0, n1 + D3 + per):
            if g < n1:
                row = g * GE
                tok = None
                if mt is not None:
                    tok = mt[((g - g0) * an) // (n1 - g0)]
                    prev = done.get(row // GR - PACE)
                    if prev is not None:
                        tok = tok + prev * zvec[...]
                r1[g] = []
                for w, p in enumerate(qk(qq, kk, row, tok)):
                    pbuf[w, row:row + GE, :] = p
                    r1[g].append(pltpu.roll(p, 64, 1))
            gg = g - D1
            if g0 <= gg < n1:
                row = gg * GE
                r2[gg] = []
                for w, r in enumerate(r1.pop(gg)):
                    sm = pbuf[w, row:row + GE, :] + r
                    sbuf[w, row:row + GE, :] = sm
                    r2[gg].append(pltpu.roll(sm, 32, 1))
            gg = g - D2
            if g0 <= gg < n1:
                row = gg * GE
                for w, r in enumerate(r2.pop(gg)):
                    l = sbuf[w, row:row + GE, :] + r
                    if row < HALO and w > 0:
                        t = b * T + row + jax.lax.broadcasted_iota(jnp.int32, (GE, 128), 0)
                        l = jnp.where(t >= 2 * w, l, MASKED)
                    lbuf[w, row:row + GE, :] = l
            gg = g - D3
            if g0 <= gg < n1 and (gg + 1) % per == 0:
                row = (gg + 1 - per) * GE
                done[row // GR] = softmax_pv(vv, row, ob)

    def outproj(s, r0=0, n=T, ob=op):
        bres[s][r0:r0 + n, :] = _dot(_bf(ob[r0 // 2:(r0 + n) // 2, :]), _bf(wop[...]))

    def epilogue(b, s, tok=None, gs=range(NG)):
        r0 = pl.multiple_of(b * T, T)
        for g in gs:
            row = r0 + g * GR
            rowh = pl.multiple_of(b * (T // 2), T // 2) + g * (GR // 2)
            gl = glog[s][g * GR:(g + 1) * GR, :]
            if tok is not None:
                gl = _badd(gl, tok)
            gt = jax.nn.sigmoid(gl)
            for j in range(ND):
                q = qbuf[j, pl.ds(row, GR), :].astype(F32)
                kv = _bf(kvp[j, pl.ds(rowh, GR // 2), :]).astype(F32)
                z = y2[0, j, pl.ds(row, GR), :] + y2[1, j, pl.ds(row, GR), :] + _bmul(kv, par[j, 4])
                bb = bres[s][g * GR:(g + 1) * GR, j * 128:(j + 1) * 128]
                o = bb + gt * (q * z - bb)
                obuf[b % NOB, j, g * GR:(g + 1) * GR, :] = o.astype(BF16)

    nb = NA // NCH
    for ch in range(NCH):
        first_copy(ch).wait()
        if ch == 1:
            sk_copy(1).start()
        if ch == NCH - 1:
            kv_copy(1).start()
        blks = range(ch * nb, (ch + 1) * nb)
        kvprep(0, blks)

        def seg(ch=ch, blks=blks):
            if ch >= 1:
                kprep_all(0, range((ch - 1) * nb, ch * nb))
                macs_all(0, (ch - 1) * nb)
            dft_k(0, 0, blks)
            dft_u(0, 0, blks)

        region(30 + ch, seg)
    sk_copy(1).wait()
    sk_copy(2).start()
    kprep_all(0, range((NCH - 1) * nb, NA))
    macs_all(0, (NCH - 1) * nb)
    dft_k(1, 1)

    kv_copy(1).wait()
    region(40, lambda: kv_copy(2).start())

    def block_y0():
        kvprep(1)
        dft_u(1, 1)

    region(0, block_y0)

    sk_copy(2).wait()

    def starts1():
        kv_copy(3).start()
        sk_copy(3).start()

    region(41, starts1)

    def block_x1():
        aconv(1)
        idft(0, 0)
        dft_k(2, 0)
        kv_copy(2).wait()
        kvprep(2)
        dft_u(2, 0)

    region(2, block_x1)

    def block_x(j):
        s = j % 2
        aconv(s)
        dft_u(j + 1, 1 - s)
        dft_k(j + 1, 1 - s)
        idft(j - 1, 1 - s, range(KVI, NA))

    def starts2():
        kv_copy(4).start()
        sk_copy(4).start()
        _Copies(wqkv_copy.cs[:WQ0]).start()

    def starts3():
        _Copies(wqkv_copy.cs[WQ0:]).start()
        q_copy(0).start()

    for j, starts in ((2, starts2), (3, starts3)):
        sk_copy(j + 1).wait()
        kv_copy(j + 1).wait()
        region(40 + j, starts)
        kvprep(j + 1)
        idft(j - 1, 1 - j % 2, range(0, KVI))
        region(2 * j, P(block_x, j))

    wqkv_copy.wait()
    wo_copy.start()
    q_copy(1).start()

    def block_last_conv():
        aconv((ND - 1) % 2)
        idft(ND - 2, (ND - 2) % 2)
        w_transpose()

    region(12, block_last_conv)
    q_copy(0).wait()
    for b in range(2, NT):
        q_copy(b).start()

    def block_b0():
        w_permute()
        qkv(0, 0)

    region(10, block_b0)

    def block_b1():
        q_copy(1).wait()
        wo_copy.wait()
        wo_permute()
        idft(ND - 1, (ND - 1) % 2)
        halo(0)
        mt = qkv(1, 1)
        attention(0, 0, mt)
        gate(0, 0, mt)
        outproj(0)

    region(11, block_b1)

    def epilogue_wait(t):
        if t >= NOB:
            out_copy(t - NOB).wait()

    def block_b(b, s):
        q_copy(b).wait()

        @pl.when(b - 2 >= NOB)
        def _():
            out_copy(b - 2 - NOB).wait()

        halo(1 - s)
        mt = qkv(b, s)
        epilogue(b - 2, s, mt[14])
        out_copy(b - 2).start()
        gate(b - 1, 1 - s, mt)
        attention(b - 1, 1 - s, mt)
        outproj(1 - s)

    def body_b(b, carry):
        for s in range(2):
            pl.when(b % 2 == s)(P(block_b, b, s))
        return carry

    jax.lax.fori_loop(2, NT - 1, body_b, 0)

    def block_last():
        b, s = NT - 1, (NT - 1) % 2
        q_copy(b).wait()
        epilogue_wait(b - 2)
        halo(1 - s)
        m1 = qkv_half(b, s, 0)
        m2 = qkv_half(b, s, 1)
        epilogue(b - 2, s, m2[14])
        out_copy(b - 2).start()
        attention(b - 1, 1 - s, m1 + m2, an=24)
        gate(b - 1, 1 - s, m1)
        attention(b, s, m2, 0, T // 2, an=14, ob=op2)
        outproj(1 - s)

    region(13, block_last)

    epilogue_wait(NT - 2)
    epilogue_wait(NT - 1)
    epilogue(NT - 2, 0)
    out_copy(NT - 2).start()
    gate(NT - 1, 1)
    attention(NT - 1, 1, None, T // 2, T // 2, ob=op2)
    nh = T // 4
    for h in range(4):
        outproj(1, h * nh, nh, op2)
    for h in range(4):
        epilogue(NT - 1, 1, None, range(h * nh // GR, (h + 1) * nh // GR))
        out_copy(NT - 1, h * nh, nh).start()
    for t in range(NT - NOB, NT - 1):
        out_copy(t).wait()
    for h in range(4):
        out_copy(NT - 1, h * nh, nh).wait()


@jax.jit
def pallas_gated_mix__ssm_conv_h3__sliding_local_dilated__prompt_kernel(A_q, A_k, A_v, A_shift_k, A_ssm_k, A_ssm_D, B_x, B_wqkv, B_wo, gate_w):
    fwd, inv, eye = _dft_constants()
    hbm = pl.BlockSpec(memory_space=pl.ANY)
    two = lambda shape, dt: [pltpu.VMEM(shape, dt), pltpu.VMEM(shape, dt)]
    return pl.pallas_call(
        _kernel,
        out_shape=jax.ShapeDtypeStruct((1, S, D), BF16),
        in_specs=[hbm] * 12,
        out_specs=hbm,
        scratch_shapes=[
            pltpu.VMEM((4, D), BF16),
            pltpu.VMEM((D,), BF16),
            pltpu.VMEM((D,), BF16),
            pltpu.VMEM((256, 128), BF16),
            pltpu.VMEM((128, 256), BF16),
            pltpu.VMEM((128, 128), BF16),
            pltpu.VMEM((ND, 2 * KH + S, 128), BF16),
            pltpu.VMEM((ND, S, 128), BF16),
            pltpu.VMEM((ND, NA, 128, L), BF16),
            pltpu.VMEM((ND, S, 128), BF16),
            pltpu.VMEM((15, D, 128), BF16),
            pltpu.VMEM((ND, D, 128), BF16),
            pltpu.VMEM((ND, 6, 8, 128), F32),
            pltpu.VMEM((8, 128), F32),
            pltpu.SMEM((64,), jnp.int32),
            pltpu.VMEM((128, 128), U32),
            pltpu.VMEM((64, 256), U32),
            pltpu.VMEM((64, 128), U32),
            pltpu.VMEM((64, 128), U32),
            pltpu.VMEM((ND, S // 2, 128), U32),
            *two((2, NA, 128, 128), F32),
            *two((NA, 256, 128), F32),
            *two((NA, 128, 128), U32),
            *two((384, 128), F32),
            pltpu.VMEM((16, 384, 128), F32),
            pltpu.VMEM((2, ND, S, 128), F32),
            pltpu.VMEM((ND, 3 * D, 128), F32),
            pltpu.VMEM((3 * D // 2, D), U32),
            pltpu.VMEM((ND, D, 128), F32),
            pltpu.VMEM((D // 2, D), U32),
            *two((ND, T, 128), F32),
            *two((ND, HALO + T, 128), F32),
            *two((ND, HALO + T, 128), F32),
            pltpu.VMEM((8, T, 128), F32),
            pltpu.VMEM((8, T, 128), F32),
            pltpu.VMEM((8, T, 128), F32),
            pltpu.VMEM((T // 2, D), U32),
            pltpu.VMEM((T // 2, D), U32),
            *two((T, D), F32),
            pltpu.VMEM((NOB, ND, T, 128), BF16),
            pltpu.VMEM((T // 2, 128), U32),
            *two((T, 128), F32),
            pltpu.SemaphoreType.DMA((2 * ND,)),
            pltpu.SemaphoreType.DMA((NT,)),
            pltpu.SemaphoreType.DMA((2,)),
            pltpu.SemaphoreType.DMA((NOB,)),
            pltpu.SemaphoreType.DMA((6,)),
            pltpu.SemaphoreType.DMA((NCH,)),
        ],
        compiler_params=pltpu.CompilerParams(vmem_limit_bytes=100 * 2 ** 20),
    )(A_q, A_k, A_v, A_shift_k.T, A_ssm_k, A_ssm_D, B_wqkv, B_wo, gate_w,
      jnp.asarray(fwd, BF16), jnp.asarray(inv, BF16), jnp.asarray(eye, BF16))
```
